```python
import jax
import jax.numpy as jnp

def _softmax(x, axis=-1):
    return jax.nn.softmax(x, axis=axis)

def _gelu(x):
    return jax.nn.gelu(x, approximate=True)

def _silu(x):
    return jax.nn.silu(x)

def _sigmoid(x):
    return jax.nn.sigmoid(x)

def _layernorm(x, axis=-1, eps=1e-05):
    m = jnp.mean(x, axis=axis, keepdims=True)
    v = jnp.var(x, axis=axis, keepdims=True)
    return (x - m) / jnp.sqrt(v + eps)

def _scatter_add(tgt, idx, src, axis=0):
    return tgt.at[idx].add(src)

def _segment_sum(src, seg, n):
    return jax.ops.segment_sum(src, seg, n)

class _Rng:

    def __init__(self, key):
        self._k = key

    def _next(self):
        self._k, sub = jax.random.split(self._k)
        return sub

    def normal(self, shape):
        return jax.random.normal(self._next(), shape, dtype=jnp.bfloat16)

    def randint(self, lo, hi, shape):
        return jax.random.randint(self._next(), shape, lo, hi, dtype=jnp.int32)

    def uniform(self, shape, lo=0.0, hi=1.0):
        return jax.random.uniform(self._next(), shape, jnp.bfloat16, lo, hi)

    def permutation(self, n):
        return jax.random.permutation(self._next(), n)
kernel_name = 'adaLN_cond__sliding_local_dilated__glu_gated_swiglu__prompt'

def setup_inputs():
    _rng = _Rng(jax.random.key(int.from_bytes(__import__("os").urandom(4), "little")))
    _w = lambda a: (lambda t: t.astype(jnp.bfloat16) if jnp.issubdtype(t.dtype, jnp.floating) else t)(jnp.asarray(a))

    def _A_setup():
        B, S, D = (1, 2048, 1024)
        return {'x': _w((lambda *s: _rng.normal(s) * 0.05)(B, S, D)), 'wqkv': _w((lambda *s: _rng.normal(s) * 0.05)(D, 3 * D)), 'wo': _w((lambda *s: _rng.normal(s) * 0.05)(D, D))}
    _A_in = _A_setup()

    def _B_setup():
        B, S, D, F = (1, 2048, 1024, 3584)
        return {'x': _w((lambda *s: _rng.normal(s) * 0.05)(B, S, D)), 'w1': _w((lambda *s: _rng.normal(s) * 0.05)(D, F) * (2.0 / D) ** 0.5), 'w3': _w((lambda *s: _rng.normal(s) * 0.05)(D, F) * (2.0 / D) ** 0.5), 'w2': _w((lambda *s: _rng.normal(s) * 0.05)(F, D) * (2.0 / F) ** 0.5)}
    _B_in = _B_setup()
    return {'A_x': _A_in['x'], 'A_wqkv': _A_in['wqkv'], 'A_wo': _A_in['wo'], 'B_x': _B_in['x'], 'B_w1': _B_in['w1'], 'B_w3': _B_in['w3'], 'B_w2': _B_in['w2'], 'c': _w((lambda *s: _rng.normal(s) * 0.05)(1, 1024)), 'w_mod': _w((lambda *s: _rng.normal(s) * 0.05)(1024, 6 * 1024) * 1024 ** (-0.5))}

def reference(A_x, A_wqkv, A_wo, B_x, B_w1, B_w3, B_w2, c, w_mod):

    def _A_ref(x, wqkv, wo):
        B, S, D = x.shape
        H = 32
        Dh = D // H
        W, dil = (8, 2)
        qkv = (lambda x, *d: x.transpose(*d))((x @ wqkv).reshape(B, S, 3, H, Dh), 2, 0, 3, 1, 4)
        q, k, v = (qkv[0], qkv[1], qkv[2])
        scale = Dh ** (-0.5)
        pos = jnp.arange(S)
        off = jnp.arange(W) * dil
        idx = pos[:, None] - off[None, :]
        mask = idx >= 0
        idx_c = jnp.where(mask, idx, 0).reshape(-1)
        kg = k[:, :, idx_c, :].reshape(B, H, S, W, Dh)
        vg = v[:, :, idx_c, :].reshape(B, H, S, W, Dh)
        logits = jnp.einsum('bhsd,bhswd->bhsw', q, kg) * scale
        logits = jnp.where(mask[None, None, :, :], logits, -1000000000.0)
        attn = _softmax(logits, axis=-1)
        o = jnp.einsum('bhsw,bhswd->bhsd', attn, vg)
        return (lambda x, *d: x.transpose(*d))(o, 0, 2, 1, 3).reshape(B, S, D) @ wo

    def _B_ref(x, w1, w3, w2):
        gate = jnp.einsum('bsd,df->bsf', x, w1)
        up = jnp.einsum('bsd,df->bsf', x, w3)
        h = _silu(gate) * up
        out = jnp.einsum('bsf,fd->bsd', h, w2)
        return out
    x = A_x
    mod = (_silu(c) @ w_mod).reshape(c.shape[0], 6, 1, -1)
    sa, ca, ga, sb, cb, gb = (mod[:, 0].copy(), mod[:, 1].copy(), mod[:, 2].copy(), mod[:, 3].copy(), mod[:, 4].copy(), mod[:, 5].copy())
    h = _layernorm(x, axis=-1) * (1 + ca) + sa
    x = x + ga * _A_ref(h, A_wqkv, A_wo)
    h = _layernorm(x, axis=-1) * (1 + cb) + sb
    x = x + gb * _B_ref(h, B_w1, B_w3, B_w2)
    return x
```

```python
import contextlib
import functools
import math

import jax
import jax.numpy as jnp
import jax.experimental.pallas as pl
import jax.experimental.pallas.tpu as pltpu

S, D, F = 2048, 1024, 3584
H, DH, WIN, DIL = 32, 32, 8, 2
NC = D // 128
PAD = 16
EPS = 1e-5
SCALE = DH ** -0.5
EXP2_C = SCALE * math.log2(math.e)
MASKED = -1e9 / SCALE
F32, BF16, U32 = jnp.float32, jnp.bfloat16, jnp.uint32
TM = 256
NT = S // TM
G = 16
NG = TM // G
HK = D // 2
SA = 2 * TM
SB = S - SA


def _xor_network(xs):
    lane = jax.lax.broadcasted_iota(jnp.int32, xs[0].shape, 1)
    for b in range(3):
        m = ((lane >> (2 + b)) & 1) == 1
        xs = [jnp.where(m, xs[i ^ (1 << b)], xs[i]) for i in range(NC)]
    return xs


def _gather_fwd(z, j):
    lane = jax.lax.broadcasted_iota(jnp.int32, z.shape, 1)
    e, g, p = lane >> 5, (lane >> 3) & 3, lane & 7
    return jnp.take_along_axis(z, g * 32 + (p ^ j) * 4 + e, axis=1)


def _gather_inv(y, j):
    lane = jax.lax.broadcasted_iota(jnp.int32, y.shape, 1)
    g, q, e = lane >> 5, (lane >> 2) & 7, lane & 3
    return jnp.take_along_axis(y, e * 32 + g * 8 + (q ^ j), axis=1)


def _unpack(w):
    return (pltpu.unpack_elementwise(w, index=0, packed_dtype=BF16, unpacked_dtype=F32),
            pltpu.unpack_elementwise(w, index=1, packed_dtype=BF16, unpacked_dtype=F32))


def _pack(a, b):
    return pltpu.pack_elementwise([a, b], packed_dtype=BF16)


def _or_all(vs):
    parts = []
    for v in vs:
        for r in range(0, v.shape[0], 8):
            for c in range(0, v.shape[1], 128):
                parts.append(v[r:r + 8, c:c + 128])
    while len(parts) > 1:
        parts = [parts[i] | parts[i + 1] if i + 1 < len(parts) else parts[i] for i in range(0, len(parts), 2)]
    return parts[0]


def _gate(x, g):
    if g is None:
        return x
    xb = x if x.dtype == U32 else pltpu.bitcast(x, U32)
    y = xb | jnp.tile(g, (x.shape[0] // 8, x.shape[1] // 128))
    return y if x.dtype == U32 else pltpu.bitcast(y, x.dtype)


def _rows(start, n, mult):
    if isinstance(start, int):
        return pl.ds(start, n)
    return pl.ds(pl.multiple_of(start, mult), n)


def make_kernel(NREL=4, QKG=2, PVG=2, SKIP=8, DL=4, PRIO=0, BQKG=2, BPVG=2, BSKIP=8, BDL=4, NAT=False, HSTAT=False, BATT=True, BLN=True,
                scopes=False, only=None):

    def scope(name):
        return jax.named_scope(name) if scopes else contextlib.nullcontext()

    def kernel(x_hbm, wqkv_hbm, wo_hbm, w1_hbm, w3_hbm, w2_hbm, c_hbm, wm_hbm, out_hbm,
               x_v, wraw_v, wp_v, wo_v, w1_v, w3_v, w2_v, wm_v,
               mod_v, scol_v, st_v, h1_v, qa_v, ka_v, va_v, qb_v, kb_v, vb_v, o_v, x1_v, h2_v, out_v, hc_v, z_v, c_v,
               sems, sem_out, bar):
        cp = pltpu.make_async_copy
        dmas = {}

        def add(name, src, dst):
            dmas[name] = cp(src, dst, sems.at[len(dmas)])

        def wm_part(m, lo, n):
            return wm_hbm.at[:, pl.ds(m * D + lo, n)], wm_v.at[:, pl.ds(m * D + lo, n)]

        def w_part(m, r0, n):
            return wqkv_hbm.at[pl.ds(r0, n), pl.ds(m * D, D)], wraw_v.at[pl.ds(r0, n), pl.ds(m * D, D)]

        def x_part(t0, n):
            return x_hbm.at[pl.ds(t0 * TM, n * TM), :], x_v.at[pl.ds(t0 * TM, n * TM), :]

        for j in range(NC):
            ka_v[j, 0:PAD, :] = jnp.zeros((PAD, 128), F32)
            va_v[j, 0:PAD, :] = jnp.zeros((PAD, 128), F32)
        add("c", c_hbm, c_v)
        add("z", ka_v.at[0, pl.ds(0, 8), :], z_v.at[pl.ds(0, 8), :])
        add("ca_lo", *wm_part(1, 0, HK))
        add("x0", *x_part(0, 1))
        add("sa_lo", *wm_part(0, 0, HK))
        add("q_lo_a", *w_part(0, 0, HK // 2))
        add("q_lo_b", *w_part(0, HK // 2, HK // 2))
        add("x1", *x_part(1, 1))
        add("k_lo", *w_part(1, 0, HK))
        add("v_lo", *w_part(2, 0, HK))
        add("ca_hi", *wm_part(1, HK, HK))
        add("sa_hi", *wm_part(0, HK, HK))
        add("q_hi", *w_part(0, HK, HK))
        add("k_hi", *w_part(1, HK, HK))
        add("v_hi", *w_part(2, HK, HK))
        add("x2", *x_part(2, 1))
        add("xr", *x_part(3, NT - 3))
        add("wmr", *wm_part(2, 0, 4 * D))
        add("wo", wo_hbm, wo_v)
        add("w1", w1_hbm, w1_v)
        add("w3", w3_hbm, w3_v)
        add("w2", w2_hbm, w2_v)
        for name, d in dmas.items():
            d.start(priority=0 if name in ("c", "z") else PRIO)
            pl.semaphore_signal(bar, 1)
            pl.semaphore_wait(bar, 1)

        def wait(*names):
            with scope("w_" + names[0]):
                for n in names:
                    dmas[n].wait()

        def zero():
            return pltpu.bitcast(z_v[0:8, :], U32)

        def mod_task(m, j, add_one):
            acc = None
            for kb in range(D // 128):
                if kb % 2 == 0:
                    rel = yield
                w = wm_v[kb * 128:(kb + 1) * 128, m * D + j * 128:m * D + (j + 1) * 128].astype(F32)
                p = w * scol_v[kb * 128:(kb + 1) * 128, :]
                parts = [p[r:r + 8] for r in range(0, 128, 8)]
                a0, a1 = parts[0], parts[1]
                if kb % 2 == 0:
                    a0, a1 = _gate(a0, rel), _gate(a1, rel)
                for r in range(2, 16, 2):
                    a0, a1 = a0 + parts[r], a1 + parts[r + 1]
                a0 = a0 + a1
                acc = a0 if acc is None else acc + a0
            r = jnp.sum(acc, axis=0, keepdims=True)
            if add_one:
                r = r + 1.0
            mod_v[m:m + 1, j * 128:(j + 1) * 128] = r
            return pltpu.bitcast(jnp.broadcast_to(r, (8, 128)), U32)

        def stats(x):
            mu = jnp.mean(x, axis=-1, keepdims=True)
            xc = x - mu
            var = jnp.mean(xc * xc, axis=-1, keepdims=True)
            return mu, xc, jax.lax.rsqrt(var + EPS)

        def finish_ln(xn, ms, mb, dst, t, g, c0, c1):
            h = xn * mod_v[ms:ms + 1, c0:c1] + mod_v[mb:mb + 1, c0:c1]
            hb = _pack(h[0:8], h[8:16])

            def commit():
                dst.at[_rows(t * (TM // 2), TM // 2, TM // 2), :][g * 8:(g + 1) * 8, c0:c1] = hb

            if isinstance(t, int):
                commit()
                return _or_all([hb])
            return commit

        def ln1_task(t, g, part="full"):
            rel = yield
            xt = x_v.at[_rows(t * TM, TM, TM), :]
            rows = slice(g * G, (g + 1) * G)
            if part == "hi":
                xb = _gate(pltpu.bitcast(xt[rows, HK:], U32), rel)
                x = jnp.concatenate(_unpack(xb), axis=0)
                mu = jnp.tile(st_v[2 * t, rows, :], (1, HK // 128))
                rs = jnp.tile(st_v[2 * t + 1, rows, :], (1, HK // 128))
                return finish_ln((x - mu) * rs, 1, 0, h1_v, t, g, HK, D)
            xb = _gate(pltpu.bitcast(xt[rows, :], U32), rel)
            x = jnp.concatenate(_unpack(xb), axis=0)
            mu, xc, rs = stats(x)
            if part == "lo":
                st_v[2 * t, rows, :] = jnp.broadcast_to(mu, (G, 128))
                st_v[2 * t + 1, rows, :] = jnp.broadcast_to(rs, (G, 128))
                return finish_ln(xc[:, :HK] * rs, 1, 0, h1_v, t, g, 0, HK)
            return finish_ln(xc * rs, 1, 0, h1_v, t, g, 0, D)

        def ln2_task(t, g):
            rel = yield
            xv = x1_v.at[:, _rows(t * TM, TM, TM), :]
            x = jnp.concatenate(
                [jnp.concatenate([_gate(xv[j, pl.ds(g * G + par, 8, stride=2), :], rel) for j in range(NC)], axis=1)
                 for par in range(2)], axis=0)
            mu, xc, rs = stats(x)
            return finish_ln(xc * rs, 4, 3, h2_v, t, g, 0, D)

        def permA_task(m, r0, n):
            rel = yield
            xs = [_gate(pltpu.bitcast(wraw_v[r0:r0 + n, m * D + j * 128:m * D + (j + 1) * 128], U32), rel) for j in range(NC)]
            zs = _xor_network(xs)
            for j in range(NC):
                wp_v[r0 // 2:(r0 + n) // 2, m * D + j * 128:m * D + (j + 1) * 128] = zs[j]
            return None

        def permB_task(m, j, r0, n):
            rel = yield
            sl = (slice(r0 // 2, (r0 + n) // 2), slice(m * D + j * 128, m * D + (j + 1) * 128))
            wp_v[sl] = _gather_fwd(_gate(wp_v[sl], rel), j)
            return None

        def perm_tasks(m, r0, n):
            return [permA_task(m, r, 32) for r in range(r0, r0 + n, 32)] + [permB_task(m, j, r0, n) for j in range(NC)]

        def halo_task():
            rel = yield
            for j in range(NC):
                kb_v[j, 0:PAD, :] = ka_v[j, SA:SA + PAD, :]
                vb_v[j, 0:PAD, :] = va_v[j, SA:SA + PAD, :]
            return None

        def attn_task(first, base, span, g, qkg, pvg, skip):
            q_v, k_v, v_v = (qa_v, ka_v, va_v) if first else (qb_v, kb_v, vb_v)
            qv = q_v.at[:, _rows(base, span, 32), :]
            kv = k_v.at[:, _rows(base, span + PAD, 32), :]
            vv = v_v.at[:, _rows(base, span + PAD, 32), :]

            def ld(ref, j, a):
                if NAT:
                    return ref[j, pl.ds(g * G + a, G), :]
                return jnp.concatenate([ref[j, pl.ds(g * G + a + par, 8, stride=2), :] for par in range(2)], axis=0)

            q = [ld(qv, j, 0) for j in range(NC)]
            ls = []
            for w in range(WIN):
                if w % qkg == 0:
                    rel = yield
                a = PAD - DIL * w
                acc = _gate(q[0], rel) * ld(kv, 0, a)
                for j in range(1, NC):
                    acc = acc + q[j] * ld(kv, j, a)
                ls.append(acc)
            ls = [l + pltpu.roll(l, 64, 1) for l in ls]
            ls = [l + pltpu.roll(l, 32, 1) for l in ls]
            if first and isinstance(base, int) and base + g * G < DIL * (WIN - 1):
                i = jax.lax.broadcasted_iota(jnp.int32, (G, 128), 0)
                rows = base + g * G + (i if NAT else 2 * (i & 7) + (i >> 3))
                ls = [ls[0]] + [jnp.where(rows >= DIL * w, ls[w], MASKED) for w in range(1, WIN)]
            mx = ls[0]
            for w in range(1, WIN):
                mx = jnp.maximum(mx, ls[w])
            ps = [jnp.exp2((l - mx) * EXP2_C) for l in ls]
            den = ps[0]
            for w in range(1, WIN):
                den = den + ps[w]
            inv = 1.0 / den
            ps = [pw * inv for pw in ps]
            for _ in range(skip):
                rel = yield
            zs = []
            for j in range(NC):
                if j % pvg == 0:
                    rel = yield
                acc = None
                for w in range(WIN):
                    pw = _gate(ps[w], rel) if w == 0 else ps[w]
                    pv = pw * ld(vv, j, PAD - DIL * w)
                    acc = pv if acc is None else acc + pv
                pk = pltpu.bitcast(acc.astype(BF16), U32) if NAT else _pack(acc[0:8], acc[8:16])
                zs.append(_gather_inv(pk, j))
            xs = _xor_network(zs)
            hb = base // 2 if isinstance(base, int) else jax.lax.shift_right_logical(base, 1)
            ov = o_v.at[_rows(hb + (0 if first else SA // 2), span // 2, 16), :]
            for j in range(NC):
                ov[g * 8:(g + 1) * 8, j * 128:(j + 1) * 128] = xs[j]
            return _or_all(xs)

        def run_now(tasks):
            for tk in tasks:
                try:
                    next(tk)
                    while True:
                        tk.send(None)
                except StopIteration:
                    pass

        def inject(h, tok):
            if tok is not None:
                h00 = h[0:8, 0:128] | (tok & zero())
                h = jnp.concatenate([jnp.concatenate([h00, h[0:8, 128:]], axis=1), h[8:]], axis=0)
            return pltpu.bitcast(h, BF16)

        def rels_of(res):
            n = res.shape[0]
            return [pltpu.bitcast(res[r:r + 8, :], U32) & zero() for r in range(0, n, n // NREL)]

        def qkv_pass(t, m, j, hf, st, tok):
            first = isinstance(t, int) and t < 2
            dst = ((qa_v, ka_v, va_v) if first else (qb_v, kb_v, vb_v))[m]
            dst = dst.at[:, _rows((t if first else t - 2) * TM, TM + (PAD if m else 0), TM), :]
            rows = slice(PAD, PAD + TM) if m else slice(0, TM)
            h = inject(h1_v[_rows(t * (TM // 2), TM // 2, TM // 2), hf * HK:(hf + 1) * HK], tok)
            w = pltpu.bitcast(wp_v[hf * HK // 2:(hf + 1) * HK // 2, m * D + j * 128:m * D + (j + 1) * 128], BF16)
            res = jnp.dot(h, w, preferred_element_type=F32)
            if hf == 1:
                res = (dst[j, rows, :] if st is None else st.pop("a")) + res
            if hf == 1 or st is None:
                dst[j, rows, :] = res
            else:
                st["a"] = res
            return rels_of(res)

        def wo_pass(t, j, hf, st, tok):
            rows = _rows(t * TM, TM, TM)
            h = inject(o_v[_rows(t * (TM // 2), TM // 2, TM // 2), hf * HK:(hf + 1) * HK], tok)
            res = jnp.dot(h, wo_v[hf * HK:(hf + 1) * HK, j * 128:(j + 1) * 128], preferred_element_type=F32)
            if hf == 1:
                y = st.pop("a") + res
                res = x_v[rows, j * 128:(j + 1) * 128].astype(F32) + mod_v[2:3, j * 128:(j + 1) * 128] * y
                x1_v[j, rows, :] = res
            else:
                st["a"] = res
            return rels_of(res)

        def P(t, m, hf):
            return [functools.partial(qkv_pass, t, m, j, hf, None) for j in range(NC)]

        def QKV(t):
            st = {}
            return [functools.partial(qkv_pass, t, m, j, hf, st) for m in range(3) for j in range(NC) for hf in range(2)]

        def WO(t):
            st = {}
            return [functools.partial(wo_pass, t, j, hf, st) for j in range(NC) for hf in range(2)]

        def FFN(i):
            st = {"acc": [None] * NC}
            hrows = _rows(i * (TM // 2), TM // 2, TM // 2)
            rows = _rows(i * TM, TM, TM)

            def gu_pass(which, n, hf, tok):
                wref = (w1_v, w3_v)[which]
                if HSTAT:
                    h = inject(hc_v[:, hf * HK:(hf + 1) * HK], tok)
                else:
                    h = inject(h2_v[hrows, hf * HK:(hf + 1) * HK], tok)
                res = jnp.dot(h, wref[hf * HK:(hf + 1) * HK, n * 128:(n + 1) * 128], preferred_element_type=F32)
                if hf == 1:
                    res = st.pop("a") + res
                    if which == 0:
                        hg = 0.5 * res
                        st["g"] = hg + hg * jnp.tanh(hg)
                    else:
                        st.setdefault("act", []).append((st.pop("g") * res).astype(BF16))
                else:
                    st["a"] = res
                return rels_of(res)

            def down_pass(cidx, j, last, tok):
                if j == 0:
                    st["lhs"] = jnp.concatenate(st.pop("act"), axis=1)
                h = st["lhs"]
                if tok is not None:
                    w = pltpu.bitcast(w2_v[cidx * HK:(cidx + 1) * HK, j * 128:(j + 1) * 128], U32)
                    w = pltpu.bitcast(jnp.concatenate([w[0:8] | (tok & zero()), w[8:]], axis=0), BF16)
                else:
                    w = w2_v[cidx * HK:(cidx + 1) * HK, j * 128:(j + 1) * 128]
                res = jnp.dot(h, w, preferred_element_type=F32)
                if st["acc"][j] is not None:
                    res = st["acc"][j] + res
                st["acc"][j] = res
                if last:
                    cs = slice(j * 128, (j + 1) * 128)
                    out_v[rows, cs] = (x1_v[j, rows, :] + mod_v[5:6, cs] * res).astype(BF16)
                return rels_of(res)

            out = []
            nch = F // HK
            for cidx in range(nch):
                for n in range(cidx * 4, cidx * 4 + 4):
                    out += [functools.partial(gu_pass, which, n, hf) for which in range(2) for hf in range(2)]
                out += [functools.partial(down_pass, cidx, j, cidx == nch - 1) for j in range(NC)]
            return out

        def segment(name, passes, groups, dl=DL):
            if only is not None and name not in only:
                return
            with scope(name):
                n = len(passes)
                active = []
                for tasks, lo, hi in groups:
                    for k, tk in enumerate(tasks):
                        active.append((int((lo + k * (hi - lo) / len(tasks)) * NREL), tk))
                        next(tk)
                deadlines = [[] for _ in range(n + dl + 1)]

                def feed(rel, slot, i):
                    for ent in list(active):
                        if ent[0] <= slot:
                            try:
                                ent[1].send(rel)
                            except StopIteration as e:
                                if e.value is not None:
                                    deadlines[i + dl].append(e.value)
                                active.remove(ent)

                feed(None, 0, 0)
                slot = 1
                for i, ps in enumerate(passes):
                    toks = []
                    for dlv in deadlines[i]:
                        if callable(dlv):
                            dlv()
                        else:
                            toks.append(dlv)
                    tok = _or_all(toks) if toks else None
                    for rel in ps(tok):
                        feed(rel, slot, i)
                        slot += 1
                while active:
                    feed(None, 1 << 30, n)
                for rest in deadlines[n:]:
                    for dlv in rest:
                        if callable(dlv):
                            dlv()

        def LN1(t, part="full"):
            return [ln1_task(t, g, part) for g in range(NG)]

        def LN2(t):
            return [ln2_task(t, g) for g in range(NG)]

        def MOD(m, j0, j1, add_one=False):
            return [mod_task(m, j, add_one) for j in range(j0, j1)]

        with scope("S0"):
            wait("c", "z")
            c = c_v[...].astype(F32)
            s = (c * jax.nn.sigmoid(c)).astype(BF16).astype(F32)
            row = jax.lax.broadcasted_iota(jnp.int32, (128, 128), 0)
            lane = jax.lax.broadcasted_iota(jnp.int32, (128, 128), 1)
            ones = jnp.ones((128, 128), BF16)
            for j in range(NC):
                dg = jnp.where(row == lane, jnp.broadcast_to(s[:, j * 128:(j + 1) * 128], (128, 128)), 0.0).astype(BF16)
                scol_v[j * 128:(j + 1) * 128, :] = jnp.dot(dg, ones, preferred_element_type=F32)
            wait("ca_lo")
            run_now(MOD(1, 0, 4, True))
            wait("x0", "sa_lo")
            run_now(MOD(0, 0, 4))
            run_now(LN1(0, "lo"))
            wait("q_lo_a")
            run_now(perm_tasks(0, 0, HK // 2))
            wait("q_lo_b")
            run_now(perm_tasks(0, HK // 2, HK // 2))
        wait("x1")
        segment("S1", P(0, 0, 0), [(LN1(1, "lo"), 0, 5)])
        wait("k_lo")
        segment("S2", P(1, 0, 0), [(perm_tasks(1, 0, HK), 0, 6)])
        wait("v_lo")
        segment("S3", P(0, 1, 0), [(perm_tasks(2, 0, HK), 0, 6)])
        wait("ca_hi")
        segment("S3b", P(1, 1, 0), [(MOD(1, 4, 8, True), 0, 4)])
        wait("sa_hi")
        segment("S4", P(0, 2, 0), [(MOD(0, 4, 8), 0, 4)])
        wait("q_hi")
        segment("S5", P(1, 2, 0), [(perm_tasks(0, HK, HK), 0, 6), (LN1(0, "hi"), 0, 4)])
        wait("k_hi")
        segment("S6", P(0, 0, 1) + P(1, 0, 1), [(LN1(1, "hi"), 0, 4), (perm_tasks(1, HK, HK), 2, 13)])
        wait("v_hi", "x2")
        segment("S7", P(0, 1, 1) + P(0, 2, 1) + P(1, 1, 1) + P(1, 2, 1),
                [(perm_tasks(2, HK, HK), 0, 6), (LN1(2), 4, 26),
                 ([attn_task(True, 0, 32, g, QKG, PVG, SKIP) for g in range(2)], 17, 24)])
        wait("xr")

        def a_step(npc, p0, t0, t, carry):
            base = jnp.minimum(p0 // 2 + (t - t0) * (npc // 2), NG - npc // 2) * (2 * G)
            att = [attn_task(True, base, npc * G, g, QKG, PVG, SKIP) for g in range(npc)]
            segment("A", QKV(t), [(att, 0, 44), (LN1(jnp.minimum(t + 1, NT - 1)), 1, 43)])
            return carry

        with scope("loopA1"):
            jax.lax.fori_loop(2, 4, functools.partial(a_step, 8, 2, 2), 0)
        wait("wmr", "wo")
        q4 = QKV(4)
        segment("AF", q4[:16] + WO(0) + q4[16:],
                [(MOD(2, 0, 8), 0, 10), (MOD(3, 0, 8) + MOD(4, 0, 8, True), 10, 30), (LN2(0), 34, 58),
                 (MOD(5, 0, 8), 34, 58), (LN1(5), 0, 58), ([halo_task()], 1, 2)])
        with scope("loopA2"):
            jax.lax.fori_loop(5, NT, functools.partial(a_step, 6, 18, 5), 0)
        wait("w1", "w3", "w2")

        def b_step(i, carry):
            @pl.when(i < NT - 1)
            def _():
                segment("W", WO(i + 1), [])

            if HSTAT:
                hc_v[...] = h2_v[_rows(i * (TM // 2), TM // 2, TM // 2), :]
                pl.semaphore_signal(bar, 1)
                pl.semaphore_wait(bar, 1)
            ta = jnp.minimum(i, NT - 3)
            tl = jnp.minimum(i + 1, NT - 1)
            att = [attn_task(False, ta * TM, TM, g, BQKG, BPVG, BSKIP) for g in range(NG)]
            grp = ([(att, 0, 158)] if BATT else []) + ([(LN2(tl), 5, 163)] if BLN else [])
            segment("F", FFN(i), grp, dl=BDL)
            r0 = pl.multiple_of(i * TM, TM)
            cp(out_v.at[pl.ds(r0, TM), :], out_hbm.at[pl.ds(r0, TM), :], sem_out.at[i]).start()
            return carry

        with scope("B"):
            jax.lax.fori_loop(0, NT, b_step, 0)
        for t in range(NT):
            cp(out_v.at[pl.ds(t * TM, TM), :], out_hbm.at[pl.ds(t * TM, TM), :], sem_out.at[t]).wait()

    @jax.jit
    def fn(A_x, A_wqkv, A_wo, B_x, B_w1, B_w3, B_w2, c, w_mod):
        x = A_x.reshape(S, D)
        V = pltpu.VMEM
        out = pl.pallas_call(
            kernel,
            in_specs=[pl.BlockSpec(memory_space=pl.ANY)] * 8,
            out_specs=pl.BlockSpec(memory_space=pl.ANY),
            out_shape=jax.ShapeDtypeStruct((S, D), BF16),
            scratch_shapes=[
                V((S, D), BF16), V((D, 3 * D), BF16), V((D // 2, 3 * D), U32), V((D, D), BF16),
                V((D, F), BF16), V((D, F), BF16), V((F, D), BF16), V((D, 6 * D), BF16),
                V((8, D), F32), V((D, 128), F32), V((4, TM, 128), F32), V((S // 2, D), U32),
                V((NC, SA, 128), F32), V((NC, PAD + SA, 128), F32), V((NC, PAD + SA, 128), F32),
                V((NC, SB, 128), F32), V((NC, PAD + SB, 128), F32), V((NC, PAD + SB, 128), F32),
                V((S // 2, D), U32), V((NC, S, 128), F32), V((S // 2, D), U32), V((S, D), BF16), V((TM // 2, D), U32), V((32, 128), F32), V((1, D), BF16),
                pltpu.SemaphoreType.DMA((32,)), pltpu.SemaphoreType.DMA((NT,)), pltpu.SemaphoreType.REGULAR,
            ],
            compiler_params=pltpu.CompilerParams(vmem_limit_bytes=124 * 1024 * 1024),
        )(x, A_wqkv, A_wo, B_w1, B_w3, B_w2, c, w_mod)
        return out.reshape(1, S, D)

    return fn


_impl = make_kernel()


@jax.jit
def pallas_adaLN_cond__sliding_local_dilated__glu_gated_swiglu__prompt_kernel(A_x, A_wqkv, A_wo, B_x, B_w1, B_w3, B_w2, c, w_mod):
    return _impl(A_x, A_wqkv, A_wo, B_x, B_w1, B_w3, B_w2, c, w_mod)
```

```python
import contextlib
import functools
import math

import jax
import jax.numpy as jnp
import jax.experimental.pallas as pl
import jax.experimental.pallas.tpu as pltpu

S, D, F = 2048, 1024, 3584
H, DH, WIN, DIL = 32, 32, 8, 2
NC = D // 128
PAD = 16
EPS = 1e-5
SCALE = DH ** -0.5
EXP2_C = SCALE * math.log2(math.e)
MASKED = -1e9 / SCALE
F32, BF16, U32 = jnp.float32, jnp.bfloat16, jnp.uint32
TM = 256
NT = S // TM
G = 16
NG = TM // G
HK = D // 2
SA = 2 * TM
SB = S - SA


def _xor_network(xs):
    lane = jax.lax.broadcasted_iota(jnp.int32, xs[0].shape, 1)
    for b in range(3):
        m = ((lane >> (2 + b)) & 1) == 1
        xs = [jnp.where(m, xs[i ^ (1 << b)], xs[i]) for i in range(NC)]
    return xs


def _gather_fwd(z, j):
    lane = jax.lax.broadcasted_iota(jnp.int32, z.shape, 1)
    e, g, p = lane >> 5, (lane >> 3) & 3, lane & 7
    return jnp.take_along_axis(z, g * 32 + (p ^ j) * 4 + e, axis=1)


def _gather_inv(y, j):
    lane = jax.lax.broadcasted_iota(jnp.int32, y.shape, 1)
    g, q, e = lane >> 5, (lane >> 2) & 7, lane & 3
    return jnp.take_along_axis(y, e * 32 + g * 8 + (q ^ j), axis=1)


def _unpack(w):
    return (pltpu.unpack_elementwise(w, index=0, packed_dtype=BF16, unpacked_dtype=F32),
            pltpu.unpack_elementwise(w, index=1, packed_dtype=BF16, unpacked_dtype=F32))


def _pack(a, b):
    return pltpu.pack_elementwise([a, b], packed_dtype=BF16)


def _or_all(vs):
    parts = []
    for v in vs:
        for r in range(0, v.shape[0], 8):
            for c in range(0, v.shape[1], 128):
                parts.append(v[r:r + 8, c:c + 128])
    while len(parts) > 1:
        parts = [parts[i] | parts[i + 1] if i + 1 < len(parts) else parts[i] for i in range(0, len(parts), 2)]
    return parts[0]


def _gate(x, g):
    if g is None:
        return x
    xb = x if x.dtype == U32 else pltpu.bitcast(x, U32)
    y = xb | jnp.tile(g, (x.shape[0] // 8, x.shape[1] // 128))
    return y if x.dtype == U32 else pltpu.bitcast(y, x.dtype)


def _rows(start, n, mult):
    if isinstance(start, int):
        return pl.ds(start, n)
    return pl.ds(pl.multiple_of(start, mult), n)


def make_kernel(NREL=2, QKG=2, PVG=2, SKIP=4, DL=4, PRIO=0, BQKG=1, BPVG=2, BSKIP=3, BDL=4, NAT=False, AFP=(16, 10, 30, 34, 58, 34, 58, 0, 58), AFDL=4, T7L=(7, 14), AA=(0, 44), AL=(1, 42), PEEL=False, W0=(3, 9, 1), WA=(9, 9, 7, 6, 6, 6, 6), WP=(3.5, 1.5, 0.5, 1.5, 2, 5), X2AT=6, OSPLIT=1, BA=(0, 158), BL=(5, 155), CPH=0.5, BATT=True, BLN=True,
                scopes=False, only=None):

    def scope(name):
        return jax.named_scope(name) if scopes else contextlib.nullcontext()

    def kernel(x_hbm, wqkv_hbm, wo_hbm, w1_hbm, w3_hbm, w2_hbm, c_hbm, wm_hbm, out_hbm,
               x_v, wraw_v, wp_v, wo_v, w1_v, w3_v, w2_v, wm_v,
               mod_v, scol_v, st_v, h1_v, qa_v, ka_v, va_v, qb_v, kb_v, vb_v, o_v, x1_v, h2_v, out_v, hc_v, hn_v, z_v, c_v,
               sems, sem_out, bar):
        cp = pltpu.make_async_copy
        dmas = {}

        def add(name, src, dst):
            dmas[name] = cp(src, dst, sems.at[len(dmas)])

        def wm_part(m, lo, n):
            return wm_hbm.at[:, pl.ds(m * D + lo, n)], wm_v.at[:, pl.ds(m * D + lo, n)]

        def w_part(m, r0, n):
            return wqkv_hbm.at[pl.ds(r0, n), pl.ds(m * D, D)], wraw_v.at[pl.ds(r0, n), pl.ds(m * D, D)]

        def x_part(t0, n):
            return x_hbm.at[pl.ds(t0 * TM, n * TM), :], x_v.at[pl.ds(t0 * TM, n * TM), :]

        add("c", c_hbm, c_v)
        def wq_rows(k, c0, n):
            return wqkv_hbm.at[pl.ds(k * 128, 128), pl.ds(c0, n)], wraw_v.at[pl.ds(k * 128, 128), pl.ds(c0, n)]

        add("x0", *x_part(0, 1))
        for k in range(NC):
            add(f"ca{k}", *wm_part(1, k * 128, 128))
            add(f"sa{k}", *wm_part(0, k * 128, 128))
            if k == 1:
                add("w1", *wq_rows(k, 0, D))
                add("w1kv", *wq_rows(k, D, 2 * D))
            else:
                add(f"w{k}", *wq_rows(k, 0, 3 * D))
            if k == 0:
                add("x1", *x_part(1, 1))
            if k == X2AT:
                add("x2", *x_part(2, 1))
        add("xr", *x_part(3, NT - 3))
        add("wmr", *wm_part(2, 0, 4 * D))
        add("wo", wo_hbm, wo_v)
        add("fw1", w1_hbm, w1_v)
        add("fw3", w3_hbm, w3_v)
        add("fw2", w2_hbm, w2_v)
        for name, d in dmas.items():
            d.start(priority=0 if name == "c" else PRIO)
            pl.semaphore_signal(bar, 1)
            pl.semaphore_wait(bar, 1)
        for j in range(NC):
            ka_v[j, 0:PAD, :] = jnp.zeros((PAD, 128), F32)
            va_v[j, 0:PAD, :] = jnp.zeros((PAD, 128), F32)
        add("z", ka_v.at[0, pl.ds(0, 8), :], z_v.at[pl.ds(0, 8), :])
        dmas["z"].start()

        def wait(*names):
            with scope("w_" + names[0]):
                for n in names:
                    dmas[n].wait()

        def zero():
            return pltpu.bitcast(z_v[0:8, :], U32)

        def mod_task(m, j, add_one):
            acc = None
            for kb in range(D // 128):
                if kb % 2 == 0:
                    rel = yield
                w = wm_v[kb * 128:(kb + 1) * 128, m * D + j * 128:m * D + (j + 1) * 128].astype(F32)
                p = w * scol_v[kb * 128:(kb + 1) * 128, :]
                parts = [p[r:r + 8] for r in range(0, 128, 8)]
                a0, a1 = parts[0], parts[1]
                if kb % 2 == 0:
                    a0, a1 = _gate(a0, rel), _gate(a1, rel)
                for r in range(2, 16, 2):
                    a0, a1 = a0 + parts[r], a1 + parts[r + 1]
                a0 = a0 + a1
                acc = a0 if acc is None else acc + a0
            r = jnp.sum(acc, axis=0, keepdims=True)
            if add_one:
                r = r + 1.0
            mod_v[m:m + 1, j * 128:(j + 1) * 128] = r
            return pltpu.bitcast(jnp.broadcast_to(r, (8, 128)), U32)

        def stats(x):
            mu = jnp.mean(x, axis=-1, keepdims=True)
            xc = x - mu
            var = jnp.mean(xc * xc, axis=-1, keepdims=True)
            return mu, xc, jax.lax.rsqrt(var + EPS)

        def finish_ln(xn, ms, mb, dst, g, c0, c1):
            h = xn * mod_v[ms:ms + 1, c0:c1] + mod_v[mb:mb + 1, c0:c1]
            hb = _pack(h[0:8], h[8:16])

            dst[g * 8:(g + 1) * 8, c0:c1] = hb
            return _or_all([hb])

        def ln1_task(t, g, dst):
            rel = yield
            xt = x_v.at[_rows(t * TM, TM, TM), :]
            xb = _gate(pltpu.bitcast(xt[g * G:(g + 1) * G, :], U32), rel)
            x = jnp.concatenate(_unpack(xb), axis=0)
            mu, xc, rs = stats(x)
            return finish_ln(xc * rs, 1, 0, dst, g, 0, D)

        def stats_task(t, g):
            rel = yield
            rows = slice(t * TM + g * G, t * TM + (g + 1) * G)
            x = jnp.concatenate(_unpack(_gate(pltpu.bitcast(x_v[rows, :], U32), rel)), axis=0)
            mu, xc, rs = stats(x)
            st_v[0, rows, :] = jnp.broadcast_to(mu, (G, 128))
            st_v[1, rows, :] = jnp.broadcast_to(rs, (G, 128))
            return None

        def fin_task(t, k, g0, ng):
            rel = yield
            cs = slice(k * 128, (k + 1) * 128)
            for g in range(g0, g0 + ng):
                rows = slice(t * TM + g * G, t * TM + (g + 1) * G)
                x = jnp.concatenate(_unpack(_gate(pltpu.bitcast(x_v[rows, cs], U32), rel)), axis=0)
                finish_ln((x - st_v[0, rows, :]) * st_v[1, rows, :], 1, 0, h1_v.at[t], g, k * 128, (k + 1) * 128)
            return None

        def ln2_task(t, g, dst):
            rel = yield
            xv = x1_v.at[:, _rows(t * TM, TM, TM), :]
            x = jnp.concatenate(
                [jnp.concatenate([_gate(xv[j, pl.ds(g * G + par, 8, stride=2), :], rel) for j in range(NC)], axis=1)
                 for par in range(2)], axis=0)
            mu, xc, rs = stats(x)
            return finish_ln(xc * rs, 4, 3, dst, g, 0, D)

        def permA_task(m, r0, n):
            rel = yield
            xs = [_gate(pltpu.bitcast(wraw_v[r0:r0 + n, m * D + j * 128:m * D + (j + 1) * 128], U32), rel) for j in range(NC)]
            zs = _xor_network(xs)
            for j in range(NC):
                wp_v[r0 // 2:(r0 + n) // 2, m * D + j * 128:m * D + (j + 1) * 128] = zs[j]
            return None

        def permB_task(m, j, r0, n):
            rel = yield
            sl = (slice(r0 // 2, (r0 + n) // 2), slice(m * D + j * 128, m * D + (j + 1) * 128))
            wp_v[sl] = _gather_fwd(_gate(wp_v[sl], rel), j)
            return None

        def perm_tasks(m, r0, n):
            return [permA_task(m, r, 32) for r in range(r0, r0 + n, 32)] + [permB_task(m, j, r0, n) for j in range(NC)]

        def copy_task(src, dst, hf):
            rel = yield
            dst[:, hf * HK:(hf + 1) * HK] = _gate(src[:, hf * HK:(hf + 1) * HK], rel)
            return None

        def COPY(src, dst, n):
            return [([copy_task(src, dst, 0)], n - 1, n), ([copy_task(src, dst, 1)], n - 1 + CPH, n)]

        def halo_task():
            rel = yield
            for j in range(NC):
                kb_v[j, 0:PAD, :] = ka_v[j, SA:SA + PAD, :]
                vb_v[j, 0:PAD, :] = va_v[j, SA:SA + PAD, :]
            return None

        def attn_task(first, base, span, g, qkg, pvg, skip, masked=False):
            q_v, k_v, v_v = (qa_v, ka_v, va_v) if first else (qb_v, kb_v, vb_v)
            qv = q_v.at[:, _rows(base, span, 32), :]
            kv = k_v.at[:, _rows(base, span + PAD, 32), :]
            vv = v_v.at[:, _rows(base, span + PAD, 32), :]

            def ld(ref, j, a):
                if NAT:
                    return ref[j, pl.ds(g * G + a, G), :]
                return jnp.concatenate([ref[j, pl.ds(g * G + a + par, 8, stride=2), :] for par in range(2)], axis=0)

            q = [ld(qv, j, 0) for j in range(NC)]
            ls = []
            for w in range(WIN):
                if w % qkg == 0:
                    rel = yield
                a = PAD - DIL * w
                acc = _gate(q[0], rel) * ld(kv, 0, a)
                for j in range(1, NC):
                    acc = acc + q[j] * ld(kv, j, a)
                ls.append(acc)
            ls = [l + pltpu.roll(l, 64, 1) for l in ls]
            ls = [l + pltpu.roll(l, 32, 1) for l in ls]
            if masked and g == 0:
                i = jax.lax.broadcasted_iota(jnp.int32, (G, 128), 0)
                rows = base + g * G + (i if NAT else 2 * (i & 7) + (i >> 3))
                ls = [ls[0]] + [jnp.where(rows >= DIL * w, ls[w], MASKED) for w in range(1, WIN)]
            mx = ls[0]
            for w in range(1, WIN):
                mx = jnp.maximum(mx, ls[w])
            ps = [jnp.exp2((l - mx) * EXP2_C) for l in ls]
            den = ps[0]
            for w in range(1, WIN):
                den = den + ps[w]
            inv = 1.0 / den
            ps = [pw * inv for pw in ps]
            for _ in range(skip):
                rel = yield
            zs = []
            for j in range(NC):
                if j % pvg == 0:
                    rel = yield
                acc = None
                for w in range(WIN):
                    pw = _gate(ps[w], rel) if w == 0 else ps[w]
                    pv = pw * ld(vv, j, PAD - DIL * w)
                    acc = pv if acc is None else acc + pv
                pk = pltpu.bitcast(acc.astype(BF16), U32) if NAT else _pack(acc[0:8], acc[8:16])
                zs.append(_gather_inv(pk, j))
            xs = _xor_network(zs)
            hb = base // 2 if isinstance(base, int) else jax.lax.shift_right_logical(base, 1)
            ov = o_v.at[_rows(hb + (0 if first else SA // 2), span // 2, 16), :]
            for j in range(NC):
                ov[g * 8:(g + 1) * 8, j * 128:(j + 1) * 128] = xs[j]
            return _or_all(xs)

        def run_now(tasks):
            for tk in tasks:
                try:
                    next(tk)
                    while True:
                        tk.send(None)
                except StopIteration:
                    pass

        def inject(h, tok):
            if tok is not None:
                h00 = h[0:8, 0:128] | (tok & zero())
                h = jnp.concatenate([jnp.concatenate([h00, h[0:8, 128:]], axis=1), h[8:]], axis=0)
            return pltpu.bitcast(h, BF16)

        def rels_of(res):
            n = res.shape[0]
            return [pltpu.bitcast(res[r:r + 8, :], U32) & zero() for r in range(0, n, n // NREL)]

        def qkv_pass(t, m, j, hf, st, tok):
            first = isinstance(t, int) and t < 2
            dst = ((qa_v, ka_v, va_v) if first else (qb_v, kb_v, vb_v))[m]
            dst = dst.at[:, _rows((t if first else t - 2) * TM, TM + (PAD if m else 0), TM), :]
            rows = slice(PAD, PAD + TM) if m else slice(0, TM)
            h = inject((h1_v.at[t] if first else hc_v)[:, hf * HK:(hf + 1) * HK], tok)
            w = pltpu.bitcast(wp_v[hf * HK // 2:(hf + 1) * HK // 2, m * D + j * 128:m * D + (j + 1) * 128], BF16)
            res = jnp.dot(h, w, preferred_element_type=F32)
            if hf == 1:
                res = (dst[j, rows, :] if st is None else st.pop("a")) + res
            if hf == 1 or st is None:
                dst[j, rows, :] = res
            else:
                st["a"] = res
            return rels_of(res)

        def wo_pass(t, j, hf, st, tok):
            rows = _rows(t * TM, TM, TM)
            h = inject(o_v[_rows(t * (TM // 2), TM // 2, TM // 2), hf * HK:(hf + 1) * HK], tok)
            res = jnp.dot(h, wo_v[hf * HK:(hf + 1) * HK, j * 128:(j + 1) * 128], preferred_element_type=F32)
            if hf == 1:
                y = st.pop("a") + res
                res = x_v[rows, j * 128:(j + 1) * 128].astype(F32) + mod_v[2:3, j * 128:(j + 1) * 128] * y
                x1_v[j, rows, :] = res
            else:
                st["a"] = res
            return rels_of(res)

        def wave_pass(k, t, nb, tok):
            m, j0 = nb // 2, (nb % 2) * 4
            dst = (qa_v, ka_v, va_v)[m]
            rows = slice(t * TM + (PAD if m else 0), (t + 1) * TM + (PAD if m else 0))
            h = h1_v[t, :, k * 128:(k + 1) * 128]
            if tok is not None:
                h = jnp.concatenate([h[0:8] | (tok & zero()), h[8:]], axis=0)
            w = pltpu.bitcast(wp_v[k * 64:(k + 1) * 64, nb * 512:(nb + 1) * 512], BF16)
            res = jnp.dot(pltpu.bitcast(h, BF16), w, preferred_element_type=F32)
            for jj in range(4):
                r = res[:, jj * 128:(jj + 1) * 128]
                if k > 0:
                    r = dst[j0 + jj, rows, :] + r
                dst[j0 + jj, rows, :] = r
            return rels_of(res[:, 0:128])

        def WAVE(k):
            return [functools.partial(wave_pass, k, t, nb) for m in range(3) for t in range(2) for nb in (2 * m, 2 * m + 1)]

        def QKV(t):
            st = {}
            return [functools.partial(qkv_pass, t, m, j, hf, st) for m in range(3) for j in range(NC) for hf in range(2)]

        def WO(t):
            st = {}
            return [functools.partial(wo_pass, t, j, hf, st) for j in range(NC) for hf in range(2)]

        def FFN(i):
            st = {"acc": [None] * NC}
            rows = _rows(i * TM, TM, TM)

            def gu_pass(which, n, hf, tok):
                wref = (w1_v, w3_v)[which]
                h = inject(h2_v[:, hf * HK:(hf + 1) * HK], tok)
                res = jnp.dot(h, wref[hf * HK:(hf + 1) * HK, n * 128:(n + 1) * 128], preferred_element_type=F32)
                if hf == 1:
                    res = st.pop("a") + res
                    if which == 0:
                        hg = 0.5 * res
                        st["g"] = hg + hg * jnp.tanh(hg)
                    else:
                        st.setdefault("act", []).append((st.pop("g") * res).astype(BF16))
                else:
                    st["a"] = res
                return rels_of(res)

            def down_pass(cidx, j, last, tok):
                if j == 0:
                    st["lhs"] = jnp.concatenate(st.pop("act"), axis=1)
                h = st["lhs"]
                if tok is not None:
                    w = pltpu.bitcast(w2_v[cidx * HK:(cidx + 1) * HK, j * 128:(j + 1) * 128], U32)
                    w = pltpu.bitcast(jnp.concatenate([w[0:8] | (tok & zero()), w[8:]], axis=0), BF16)
                else:
                    w = w2_v[cidx * HK:(cidx + 1) * HK, j * 128:(j + 1) * 128]
                res = jnp.dot(h, w, preferred_element_type=F32)
                if st["acc"][j] is not None:
                    res = st["acc"][j] + res
                st["acc"][j] = res
                if last:
                    cs = slice(j * 128, (j + 1) * 128)
                    out_v[rows, cs] = (x1_v[j, rows, :] + mod_v[5:6, cs] * res).astype(BF16)
                    if OSPLIT and (j + 1) % OSPLIT == 0:
                        cols = pl.ds((j + 1 - OSPLIT) * 128, OSPLIT * 128)
                        cp(out_v.at[rows, cols], out_hbm.at[rows, cols], sem_out.at[i]).start()
                return rels_of(res)

            out = []
            nch = F // HK
            for cidx in range(nch):
                for n in range(cidx * 4, cidx * 4 + 4):
                    out += [functools.partial(gu_pass, which, n, hf) for which in range(2) for hf in range(2)]
                out += [functools.partial(down_pass, cidx, j, cidx == nch - 1) for j in range(NC)]
            return out

        def segment(name, passes, groups, dl=DL, need=None):
            if only is not None and name not in only:
                return
            with scope(name):
                n = len(passes)
                active = []
                for tasks, lo, hi in groups:
                    for k, tk in enumerate(tasks):
                        active.append((int((lo + k * (hi - lo) / len(tasks)) * NREL), tk))
                        next(tk)
                deadlines = [[] for _ in range(n + dl + 1)]

                def feed(rel, slot, i):
                    for ent in list(active):
                        if ent[0] <= slot:
                            try:
                                ent[1].send(rel)
                            except StopIteration as e:
                                if e.value is not None:
                                    deadlines[i + dl].append(e.value)
                                active.remove(ent)

                feed(None, 0, 0)
                slot = 1
                for i, ps in enumerate(passes):
                    for tk in (need or {}).get(i, ()):
                        assert all(ent[1] is not tk for ent in active), (name, i)
                    toks = []
                    for dlv in deadlines[i]:
                        if callable(dlv):
                            dlv()
                        else:
                            toks.append(dlv)
                    tok = _or_all(toks) if toks else None
                    for rel in ps(tok):
                        feed(rel, slot, i)
                        slot += 1
                while active:
                    feed(None, 1 << 30, n)
                for rest in deadlines[n:]:
                    for dlv in rest:
                        if callable(dlv):
                            dlv()

        def LN1(t, dst):
            return [ln1_task(t, g, dst) for g in range(NG)]

        def LN2(t, dst):
            return [ln2_task(t, g, dst) for g in range(NG)]

        def MOD(m, j0, j1, add_one=False):
            return [mod_task(m, j, add_one) for j in range(j0, j1)]

        with scope("S0"):
            wait("c", "z")
            c = c_v[...].astype(F32)
            s = (c * jax.nn.sigmoid(c)).astype(BF16).astype(F32)
            row = jax.lax.broadcasted_iota(jnp.int32, (128, 128), 0)
            lane = jax.lax.broadcasted_iota(jnp.int32, (128, 128), 1)
            ones = jnp.ones((128, 128), BF16)
            for j in range(NC):
                dg = jnp.where(row == lane, jnp.broadcast_to(s[:, j * 128:(j + 1) * 128], (128, 128)), 0.0).astype(BF16)
                scol_v[j * 128:(j + 1) * 128, :] = jnp.dot(dg, ones, preferred_element_type=F32)
            wait("x0")
            run_now([stats_task(0, g) for g in range(NG)])
            wait("ca0", "sa0")
            run_now(MOD(1, 0, 1, True) + MOD(0, 0, 1) + [fin_task(0, 0, 0, NG)])
            wait("w0")
            run_now(perm_tasks(0, 0, 128))

        def WP_(k, t, nb):
            return functools.partial(wave_pass, k, t, nb)

        def FIN(t, k):
            return [fin_task(t, k, g0, 4) for g0 in range(0, NG, 4)]

        m0 = [WP_(0, 0, nb) for nb in range(6)] + [WP_(0, 1, nb) for nb in range(6)]
        m1 = WAVE(1)
        n0, n1, n2 = W0
        p1, p2 = perm_tasks(1, 0, 128), perm_tasks(2, 0, 128)
        segment("T0a", m0[:n0], [(p1, 0, 1), (p2, 1, n0 - 0.5)], need={2: p1})
        wait("x1")
        s1, f1 = [stats_task(1, g) for g in range(NG)], FIN(1, 0)
        segment("T0b", m0[n0:n1], [(s1, 0, 6 - n0 - 1), (f1, 6 - n0 - 1, 6 - n0 - 0.5)], need={6 - n0: s1 + f1})
        wait("ca1", "sa1", "w1")
        mods, f0, f1, pq = MOD(1, 1, 2, True) + MOD(0, 1, 2), FIN(0, 1), FIN(1, 1), perm_tasks(0, 128, 128)
        u = 12 - n1
        segment("T0c", m0[n1:] + m1[:n2], [(mods, 0, 0.5), (f0, u - 1, u - 0.5), (f1, u - 0.5, u + 0.5), (pq, 0, u - 1)],
                need={u: mods + f0 + pq, u + 2: f1})
        wait("w1kv")
        p1, p2 = perm_tasks(1, 128, 128), perm_tasks(2, 128, 128)
        segment("T1", m1[n2:WA[1]], [(p1, 0, 4 - n2 - 1), (p2, 4 - n2 - 1, 8 - n2 - 1.5)], need={4 - n2: p1, 8 - n2: p2})
        for k in range(2, NC):
            wait(f"ca{k}", f"sa{k}", f"w{k}", *(["x2"] if k == NC - 1 else []))
            u = 12 - WA[k - 1]
            mods = MOD(1, k, k + 1, True) + MOD(0, k, k + 1)
            fins = [FIN(t, k) for t in range(2)]
            perms = [perm_tasks(m, k * 128, 128) for m in range(3)]
            nxt = WAVE(k) if k == NC - 1 else WAVE(k)[:WA[k]]
            mend = max(0.5, u - WP[0])
            groups = [(mods[:1], 0, 1), (mods[1:], mend - 0.5 if mend > 2 else 0, mend),
                      (fins[0], u - WP[1], u - WP[2]), (fins[1], u - WP[2], u + 1),
                      (perms[0], 0, u - WP[3]), (perms[1], u - WP[3], u + WP[4]), (perms[2], u + WP[4], u + WP[5])]
            if k == NC - 1:
                groups.append((LN1(2, hc_v), T7L[0], T7L[1]))
            segment(f"T{k}", WAVE(k - 1)[WA[k - 1]:] + nxt, groups,
                    need={u: mods + fins[0] + perms[0], u + 2: fins[1], u + 4: perms[1], u + 8: perms[2]})
        wait("xr")

        def a_step(npc, p0, t0, t, carry):
            base = jnp.minimum(p0 // 2 + (t - t0) * (npc // 2), NG - npc // 2) * (2 * G)
            att = [attn_task(True, base, npc * G, g, QKG, PVG, SKIP, p0 == 0) for g in range(npc)]
            segment("A", QKV(t), [(att, *AA), (LN1(jnp.minimum(t + 1, NT - 1), hn_v), *AL)] + COPY(hn_v, hc_v, 48))
            return carry

        with scope("loopA1"):
            jax.lax.fori_loop(2, 4, functools.partial(a_step, 8, 0, 2), 0)
        wait("wmr", "wo")
        q4 = QKV(4)
        n1 = AFP[0]
        mg, msc, l2 = MOD(2, 0, 8), MOD(3, 0, 8) + MOD(4, 0, 8, True), LN2(0, h2_v)
        segment("AF", q4[:n1] + WO(0) + q4[n1:],
                [(mg, 0, AFP[1]), (msc, AFP[1], AFP[2]), (l2, AFP[3], AFP[4]),
                 (MOD(5, 0, 8), AFP[5], AFP[6]), (LN1(5, hn_v), AFP[7], AFP[8]), ([halo_task()], 1, 2)] + COPY(hn_v, hc_v, 64),
                need={n1: mg, int(AFP[3]): msc}, dl=AFDL)
        with scope("loopA2"):
            jax.lax.fori_loop(5, NT, functools.partial(a_step, 6, 16, 5), 0)
        wait("fw1", "fw3", "fw2")

        def b_step(i, carry):
            ta = jnp.minimum(i, NT - 3)
            tl = jnp.minimum(i + 1, NT - 1)
            att = [attn_task(False, ta * TM, TM, g, BQKG, BPVG, BSKIP) for g in range(NG)]
            if PEEL:
                off = 16
                passes = WO(i + 1) + FFN(i)
            else:
                off = 0
                passes = FFN(i)

                @pl.when(i < NT - 1)
                def _():
                    segment("W", WO(i + 1), [])

            grp = ([(att, BA[0], BA[1] + off)] if BATT else []) + (
                [(LN2(tl, hn_v), BL[0] + off, BL[1] + off), ([copy_task(hn_v, h2_v, 0)], 161 + off, 162 + off),
                 ([copy_task(hn_v, h2_v, 1)], 163 + off, 164 + off)] if BLN else [])
            segment("F", passes, grp, dl=BDL)
            return carry

        with scope("B"):
            jax.lax.fori_loop(0, NT - 1 if PEEL else NT, b_step, 0)
        if PEEL:
            segment("FL", FFN(NT - 1), [])
        for t in range(NT):
            cp(out_v.at[pl.ds(t * TM, TM), :], out_hbm.at[pl.ds(t * TM, TM), :], sem_out.at[t]).wait()

    @jax.jit
    def fn(A_x, A_wqkv, A_wo, B_x, B_w1, B_w3, B_w2, c, w_mod):
        x = A_x.reshape(S, D)
        V = pltpu.VMEM
        out = pl.pallas_call(
            kernel,
            in_specs=[pl.BlockSpec(memory_space=pl.ANY)] * 8,
            out_specs=pl.BlockSpec(memory_space=pl.ANY),
            out_shape=jax.ShapeDtypeStruct((S, D), BF16),
            scratch_shapes=[
                V((S, D), BF16), V((D, 3 * D), BF16), V((D // 2, 3 * D), U32), V((D, D), BF16),
                V((D, F), BF16), V((D, F), BF16), V((F, D), BF16), V((D, 6 * D), BF16),
                V((8, D), F32), V((D, 128), F32), V((2, 2 * TM, 128), F32), V((2, TM // 2, D), U32),
                V((NC, SA, 128), F32), V((NC, PAD + SA, 128), F32), V((NC, PAD + SA, 128), F32),
                V((NC, SB, 128), F32), V((NC, PAD + SB, 128), F32), V((NC, PAD + SB, 128), F32),
                V((S // 2, D), U32), V((NC, S, 128), F32), V((TM // 2, D), U32), V((S, D), BF16), V((TM // 2, D), U32), V((TM // 2, D), U32), V((32, 128), F32), V((1, D), BF16),
                pltpu.SemaphoreType.DMA((35,)), pltpu.SemaphoreType.DMA((NT,)), pltpu.SemaphoreType.REGULAR,
            ],
            compiler_params=pltpu.CompilerParams(vmem_limit_bytes=124 * 1024 * 1024, disable_bounds_checks=True,
                                                 disable_semaphore_checks=True),
        )(x, A_wqkv, A_wo, B_w1, B_w3, B_w2, c, w_mod)
        return out.reshape(1, S, D)

    return fn


_impl = make_kernel(PEEL=True, BA=(16, 158), AFP=(24, 18, 41, 43, 59, 30, 59, 0, 30), QKG=1, SKIP=3)


@jax.jit
def pallas_adaLN_cond__sliding_local_dilated__glu_gated_swiglu__prompt_kernel(A_x, A_wqkv, A_wo, B_x, B_w1, B_w3, B_w2, c, w_mod):
    return _impl(A_x, A_wqkv, A_wo, B_x, B_w1, B_w3, B_w2, c, w_mod)
```

```python
import contextlib
import functools
import math

import jax
import jax.numpy as jnp
import jax.experimental.pallas as pl
import jax.experimental.pallas.tpu as pltpu

S, D, F = 2048, 1024, 3584
DH, WIN, DIL = 32, 8, 2
NC = D // 128
PAD = 16
EPS = 1e-5
SCALE = DH ** -0.5
EXP2_C = SCALE * math.log2(math.e)
MASKED = -1e9 / SCALE
F32, BF16, U32 = jnp.float32, jnp.bfloat16, jnp.uint32
TM = 256
NT = S // TM
G = 16
NG = TM // G
HK = D // 2
SA = 2 * TM
SB = S - SA


def _xor_network(xs):
    lane = jax.lax.broadcasted_iota(jnp.int32, xs[0].shape, 1)
    for b in range(3):
        m = ((lane >> (2 + b)) & 1) == 1
        xs = [jnp.where(m, xs[i ^ (1 << b)], xs[i]) for i in range(NC)]
    return xs


def _gather_fwd(z, j):
    lane = jax.lax.broadcasted_iota(jnp.int32, z.shape, 1)
    e, g, p = lane >> 5, (lane >> 3) & 3, lane & 7
    return jnp.take_along_axis(z, g * 32 + (p ^ j) * 4 + e, axis=1)


def _gather_inv(y, j):
    lane = jax.lax.broadcasted_iota(jnp.int32, y.shape, 1)
    g, q, e = lane >> 5, (lane >> 2) & 7, lane & 3
    return jnp.take_along_axis(y, e * 32 + g * 8 + (q ^ j), axis=1)


def _pack(x):
    return pltpu.bitcast(x.astype(BF16), U32)


def _or_all(vs):
    parts = [v[r:r + 8, c:c + 128] for v in vs for r in range(0, v.shape[0], 8) for c in range(0, v.shape[1], 128)]
    while len(parts) > 1:
        parts = [parts[i] | parts[i + 1] if i + 1 < len(parts) else parts[i] for i in range(0, len(parts), 2)]
    return parts[0]


def _gate(x, g):
    if g is None:
        return x
    xb = x if x.dtype == U32 else pltpu.bitcast(x, U32)
    y = xb | jnp.tile(g, (x.shape[0] // 8, x.shape[1] // 128))
    return y if x.dtype == U32 else pltpu.bitcast(y, x.dtype)


def _rows(start, n, mult):
    if isinstance(start, int):
        return pl.ds(start, n)
    return pl.ds(pl.multiple_of(start, mult), n)


def _stats(x):
    mu = jnp.mean(x, axis=-1, keepdims=True)
    xc = x - mu
    var = jnp.mean(xc * xc, axis=-1, keepdims=True)
    return mu, xc, jax.lax.rsqrt(var + EPS)


def make_kernel(NREL=2, DL=4,
                W0=(3, 9, 1), WA=(9, 9, 7, 6, 6, 6, 6), WP=(3.5, 1.5, 0.5, 1.5, 2, 5), X2AT=6, T7L=(7, 14),
                AQ=(2, 4, 3), AA=(0, 40), AL=(2, 41), ADL=5, CPH=0.75,
                AFP=(24, 18, 41, 43, 59, 30, 59, 0, 30), AFDL=4,
                BQ=(2, 2, 4), BA=(20, 174), BL=(21, 171), BCP=(176, 178), BDL=6,
                scopes=False, only=None):

    def scope(name):
        return jax.named_scope(name) if scopes else contextlib.nullcontext()

    def kernel(x_hbm, wqkv_hbm, wo_hbm, w1_hbm, w3_hbm, w2_hbm, c_hbm, wm_hbm, out_hbm,
               x_v, wraw_v, wp_v, wo_v, w1_v, w3_v, w2_v, wmc_v, wmr_v,
               mod_v, scol_v, st_v, h1_v, qa_v, ka_v, va_v, qb_v, kb_v, vb_v, o_v, x1_v, h2_v, out_v,
               hc_v, hn_v, z_v, c_v, sems, sem_out, bar):
        cp = pltpu.make_async_copy

        dmas = {}

        def add(name, src, dst):
            dmas[name] = cp(src, dst, sems.at[len(dmas)])

        def add_x(name, t0, n):
            add(name, x_hbm.at[pl.ds(t0 * TM, n * TM), :], x_v.at[pl.ds(t0 * TM, n * TM), :])

        add("c", c_hbm, c_v)
        add_x("x0", 0, 1)
        for k in range(NC):
            for m in (1, 0):
                add(f"m{m}{k}", wm_hbm.at[:, pl.ds(m * D + k * 128, 128)], wmc_v.at[m * NC + k])
            for m in range(3):
                add(f"w{m}{k}", wqkv_hbm.at[pl.ds(k * 128, 128), pl.ds(m * D, D)], wraw_v.at[m, pl.ds(k * 128, 128), :])
            if k == 0:
                add_x("x1", 1, 1)
            if k == X2AT:
                add_x("x2", 2, 1)
        add_x("xr", 3, NT - 3)
        add("wmr", wm_hbm.at[:, pl.ds(2 * D, 4 * D)], wmr_v)
        add("wo", wo_hbm, wo_v)
        add("fw1", w1_hbm, w1_v)
        add("fw3", w3_hbm, w3_v)
        add("fw2", w2_hbm, w2_v)
        for d in dmas.values():
            d.start()
            pl.semaphore_signal(bar, 1)
            pl.semaphore_wait(bar, 1)
        for j in range(NC):
            ka_v[j, 0:PAD, :] = jnp.zeros((PAD, 128), F32)
            va_v[j, 0:PAD, :] = jnp.zeros((PAD, 128), F32)
        add("z", ka_v.at[0, pl.ds(0, 8), :], z_v.at[pl.ds(0, 8), :])
        dmas["z"].start()

        def wait(*names):
            with scope("w_" + names[0]):
                for n in names:
                    dmas[n].wait()

        def zero():
            return pltpu.bitcast(z_v[0:8, :], U32)

        def mod_task(m, j):
            src = wmc_v.at[m * NC + j] if m < 2 else wmr_v.at[:, pl.ds((m - 2) * D + j * 128, 128)]
            acc = None
            for kb in range(D // 128):
                if kb % 2 == 0:
                    rel = yield
                p = src[kb * 128:(kb + 1) * 128, :].astype(F32) * scol_v[kb * 128:(kb + 1) * 128, :]
                parts = [p[r:r + 8] for r in range(0, 128, 8)]
                a0, a1 = parts[0], parts[1]
                if kb % 2 == 0:
                    a0, a1 = _gate(a0, rel), _gate(a1, rel)
                for r in range(2, 16, 2):
                    a0, a1 = a0 + parts[r], a1 + parts[r + 1]
                a0 = a0 + a1
                acc = a0 if acc is None else acc + a0
            r = jnp.sum(acc, axis=0, keepdims=True)
            if m in (1, 4):
                r = r + 1.0
            mod_v[m:m + 1, j * 128:(j + 1) * 128] = r
            return pltpu.bitcast(jnp.broadcast_to(r, (8, 128)), U32)

        def modulate(xn, ms, dst, g, c0, c1):
            hb = _pack(xn * mod_v[ms + 1:ms + 2, c0:c1] + mod_v[ms:ms + 1, c0:c1])
            dst[g * 8:(g + 1) * 8, c0:c1] = hb
            return _or_all([hb])

        def ln1_task(t, g, dst):
            rel = yield
            xt = x_v.at[_rows(t * TM, TM, TM), :]
            _, xc, rs = _stats(_gate(xt[g * G:(g + 1) * G, :].astype(F32), rel))
            return modulate(xc * rs, 0, dst, g, 0, D)

        def stats_task(t, g):
            rel = yield
            rows = slice(t * TM + g * G, t * TM + (g + 1) * G)
            mu, _, rs = _stats(_gate(x_v[rows, :].astype(F32), rel))
            st_v[0, rows, :] = jnp.broadcast_to(mu, (G, 128))
            st_v[1, rows, :] = jnp.broadcast_to(rs, (G, 128))

        def fin_task(t, k, g0, ng):
            rel = yield
            for g in range(g0, g0 + ng):
                rows = slice(t * TM + g * G, t * TM + (g + 1) * G)
                x = _gate(x_v[rows, k * 128:(k + 1) * 128].astype(F32), rel)
                modulate((x - st_v[0, rows, :]) * st_v[1, rows, :], 0, h1_v.at[t], g, k * 128, (k + 1) * 128)

        def ln2_task(t, g, dst):
            rel = yield
            xv = x1_v.at[:, _rows(t * TM, TM, TM), :]
            x = jnp.concatenate([_gate(xv[j, g * G:(g + 1) * G, :], rel) for j in range(NC)], axis=1)
            _, xc, rs = _stats(x)
            return modulate(xc * rs, 3, dst, g, 0, D)

        def perm_select_task(m, r0, n):
            rel = yield
            xs = [_gate(pltpu.bitcast(wraw_v[m, r0:r0 + n, j * 128:(j + 1) * 128], U32), rel) for j in range(NC)]
            zs = _xor_network(xs)
            for j in range(NC):
                wp_v[r0 // 2:(r0 + n) // 2, m * D + j * 128:m * D + (j + 1) * 128] = zs[j]

        def perm_gather_task(m, j, r0, n):
            rel = yield
            sl = (slice(r0 // 2, (r0 + n) // 2), slice(m * D + j * 128, m * D + (j + 1) * 128))
            wp_v[sl] = _gather_fwd(_gate(wp_v[sl], rel), j)

        def copy_task(src, dst, hf):
            rel = yield
            dst[:, hf * HK:(hf + 1) * HK] = _gate(src[:, hf * HK:(hf + 1) * HK], rel)

        def halo_task():
            yield
            for j in range(NC):
                kb_v[j, 0:PAD, :] = ka_v[j, SA:SA + PAD, :]
                vb_v[j, 0:PAD, :] = va_v[j, SA:SA + PAD, :]

        def attn_task(first, base, span, g, pace, masked=False):
            qkg, pvg, skip = pace
            q_v, k_v, v_v = (qa_v, ka_v, va_v) if first else (qb_v, kb_v, vb_v)
            qv = q_v.at[:, _rows(base, span, 32), :]
            kv = k_v.at[:, _rows(base, span + PAD, 32), :]
            vv = v_v.at[:, _rows(base, span + PAD, 32), :]

            def shifted(ref, j, w):
                return ref[j, pl.ds(g * G + PAD - DIL * w, G), :]

            q = [qv[j, g * G:(g + 1) * G, :] for j in range(NC)]
            ls = []
            for w in range(WIN):
                if w % qkg == 0:
                    rel = yield
                acc = _gate(q[0], rel) * shifted(kv, 0, w)
                for j in range(1, NC):
                    acc = acc + q[j] * shifted(kv, j, w)
                ls.append(acc)
            ls = [l + pltpu.roll(l, 64, 1) for l in ls]
            ls = [l + pltpu.roll(l, 32, 1) for l in ls]
            if masked:
                rows = base + g * G + jax.lax.broadcasted_iota(jnp.int32, (G, 128), 0)
                ls = [ls[0]] + [jnp.where(rows >= DIL * w, ls[w], MASKED) for w in range(1, WIN)]
            mx = ls[0]
            for w in range(1, WIN):
                mx = jnp.maximum(mx, ls[w])
            ps = [jnp.exp2((l - mx) * EXP2_C) for l in ls]
            den = ps[0]
            for w in range(1, WIN):
                den = den + ps[w]
            inv = 1.0 / den
            ps = [pw * inv for pw in ps]
            for _ in range(skip):
                rel = yield
            zs = []
            for j in range(NC):
                if j % pvg == 0:
                    rel = yield
                acc = _gate(ps[0], rel) * shifted(vv, j, 0)
                for w in range(1, WIN):
                    acc = acc + ps[w] * shifted(vv, j, w)
                zs.append(_gather_inv(_pack(acc), j))
            xs = _xor_network(zs)
            half = jax.lax.shift_right_logical(base, 1) + (0 if first else SA // 2)
            ov = o_v.at[_rows(half, span // 2, 16), :]
            for j in range(NC):
                ov[g * 8:(g + 1) * 8, j * 128:(j + 1) * 128] = xs[j]
            return _or_all(xs)

        def LN1(t, dst):
            return [ln1_task(t, g, dst) for g in range(NG)]

        def LN2(t, dst):
            return [ln2_task(t, g, dst) for g in range(NG)]

        def STATS(t):
            return [stats_task(t, g) for g in range(NG)]

        def FIN(t, k):
            return [fin_task(t, k, g0, 4) for g0 in range(0, NG, 4)]

        def MOD(m, j0=0, j1=NC):
            return [mod_task(m, j) for j in range(j0, j1)]

        def PERM(m, k):
            r0 = k * 128
            return ([perm_select_task(m, r, 32) for r in range(r0, r0 + 128, 32)]
                    + [perm_gather_task(m, j, r0, 128) for j in range(NC)])

        def COPY(src, dst, lo, hi, pre):
            return [([copy_task(src, dst, 0)], lo, lo + 1, pre), ([copy_task(src, dst, 1)], hi, hi + 1, pre)]

        def run_now(tasks):
            for tk in tasks:
                try:
                    next(tk)
                    while True:
                        tk.send(None)
                except StopIteration:
                    pass

        def tie(a, tok):
            if tok is not None:
                top = a[0:8, 0:128] | (tok & zero())
                if a.shape[1] > 128:
                    top = jnp.concatenate([top, a[0:8, 128:]], axis=1)
                a = jnp.concatenate([top, a[8:]], axis=0)
            return pltpu.bitcast(a, BF16)

        def releases(res):
            return [pltpu.bitcast(res[r:r + 8, 0:128], U32) & zero() for r in range(0, TM, TM // NREL)]

        def wave_pass(k, t, nb, tok):
            m, j0 = nb // 2, (nb % 2) * 4
            dst = (qa_v, ka_v, va_v)[m]
            rows = slice(t * TM + (PAD if m else 0), (t + 1) * TM + (PAD if m else 0))
            w = pltpu.bitcast(wp_v[k * 64:(k + 1) * 64, nb * 512:(nb + 1) * 512], BF16)
            res = jnp.dot(tie(h1_v[t, :, k * 128:(k + 1) * 128], tok), w, preferred_element_type=F32)
            for jj in range(4):
                r = res[:, jj * 128:(jj + 1) * 128]
                if k > 0:
                    r = dst[j0 + jj, rows, :] + r
                dst[j0 + jj, rows, :] = r
            return releases(res)

        def qkv_pass(t, m, j, hf, st, tok):
            w = pltpu.bitcast(wp_v[hf * HK // 2:(hf + 1) * HK // 2, m * D + j * 128:m * D + (j + 1) * 128], BF16)
            res = jnp.dot(tie(hc_v[:, hf * HK:(hf + 1) * HK], tok), w, preferred_element_type=F32)
            if hf == 0:
                st["a"] = res
            else:
                res = st.pop("a") + res
                off = PAD if m else 0
                dst = (qb_v, kb_v, vb_v)[m].at[:, _rows((t - 2) * TM, TM + off, TM), :]
                dst[j, off:off + TM, :] = res
            return releases(res)

        def wo_pass(t, j, hf, st, tok):
            h = tie(o_v[_rows(t * (TM // 2), TM // 2, TM // 2), hf * HK:(hf + 1) * HK], tok)
            res = jnp.dot(h, wo_v[hf * HK:(hf + 1) * HK, j * 128:(j + 1) * 128], preferred_element_type=F32)
            if hf == 0:
                st["a"] = res
            else:
                rows, cs = _rows(t * TM, TM, TM), slice(j * 128, (j + 1) * 128)
                res = x_v[rows, cs].astype(F32) + mod_v[2:3, cs] * (st.pop("a") + res)
                x1_v[j, rows, :] = res
            return releases(res)

        def out_copy(t, j):
            rows = _rows(t * TM, TM, TM)
            return cp(out_v.at[j, rows, :], out_hbm.at[rows, pl.ds(j * 128, 128)], sem_out.at[t])

        def out_wait(t):
            rows = pl.ds(t * TM, TM)
            cp(out_hbm.at[rows, :], out_hbm.at[rows, :], sem_out.at[t]).wait()

        def WAVE(k):
            return [functools.partial(wave_pass, k, t, nb) for m in range(3) for t in range(2) for nb in (2 * m, 2 * m + 1)]

        def QKV(t):
            st = {}
            return [functools.partial(qkv_pass, t, m, j, hf, st) for m in range(3) for j in range(NC) for hf in range(2)]

        def WO(t):
            st = {}
            return [functools.partial(wo_pass, t, j, hf, st) for j in range(NC) for hf in range(2)]

        def FFN(t):
            st = {"acc": [None] * NC, "act": []}

            def gate_up_pass(which, n, hf, tok):
                w = (w1_v, w3_v)[which][hf * HK:(hf + 1) * HK, n * 128:(n + 1) * 128]
                res = jnp.dot(tie(h2_v[:, hf * HK:(hf + 1) * HK], tok), w, preferred_element_type=F32)
                if hf == 0:
                    st["a"] = res
                else:
                    res = st.pop("a") + res
                    if which == 0:
                        hg = 0.5 * res
                        st["g"] = hg + hg * jnp.tanh(hg)
                    else:
                        st["act"].append((st.pop("g") * res).astype(BF16))
                return releases(res)

            def down_pass(c, j, last, tok):
                if j == 0:
                    st["lhs"], st["act"] = jnp.concatenate(st["act"], axis=1), []
                w = w2_v[c * HK:(c + 1) * HK, j * 128:(j + 1) * 128]
                if tok is not None:
                    w = tie(pltpu.bitcast(w, U32), tok)
                res = jnp.dot(st["lhs"], w, preferred_element_type=F32)
                if st["acc"][j] is not None:
                    res = st["acc"][j] + res
                st["acc"][j] = res
                if last:
                    rows = _rows(t * TM, TM, TM)
                    out_v[j, rows, :] = (x1_v[j, rows, :] + mod_v[5:6, j * 128:(j + 1) * 128] * res).astype(BF16)
                    out_copy(t, j).start()
                return releases(res)

            out = []
            nch = F // HK
            for c in range(nch):
                for n in range(c * 4, c * 4 + 4):
                    out += [functools.partial(gate_up_pass, which, n, hf) for which in range(2) for hf in range(2)]
                out += [functools.partial(down_pass, c, j, c == nch - 1) for j in range(NC)]
            return out

        def segment(name, passes, groups=(), dl=DL, need=None):
            if only is not None and name not in only:
                return
            with scope(name):
                n = len(passes)
                active = []
                for tasks, lo, hi, *pre in groups:
                    for k, tk in enumerate(tasks):
                        active.append((int((lo + k * (hi - lo) / len(tasks)) * NREL), tk, pre[0] if pre else ()))
                        next(tk)
                deadlines = [[] for _ in range(n + dl + 1)]

                def done(tasks):
                    return all(ent[1] is not tk for tk in tasks for ent in active)

                def feed(rel, slot, i):
                    for ent in list(active):
                        if ent[0] <= slot:
                            assert done(ent[2]), (name, i)
                            try:
                                ent[1].send(rel)
                            except StopIteration as e:
                                if e.value is not None:
                                    deadlines[i + dl].append(e.value)
                                active.remove(ent)

                feed(None, 0, 0)
                slot = 1
                for i, ps in enumerate(passes):
                    assert done((need or {}).get(i, ())), (name, i)
                    for rel in ps(_or_all(deadlines[i]) if deadlines[i] else None):
                        feed(rel, slot, i)
                        slot += 1
                while active:
                    feed(None, 1 << 30, n)

        with scope("S0"):
            wait("c", "z")
            c = c_v[...].astype(F32)
            s = (c * jax.nn.sigmoid(c)).astype(BF16).astype(F32)
            eye = (jax.lax.broadcasted_iota(jnp.int32, (128, 128), 0)
                   == jax.lax.broadcasted_iota(jnp.int32, (128, 128), 1))
            ones = jnp.ones((128, 128), BF16)
            for j in range(NC):
                dg = jnp.where(eye, jnp.broadcast_to(s[:, j * 128:(j + 1) * 128], (128, 128)), 0.0).astype(BF16)
                scol_v[j * 128:(j + 1) * 128, :] = jnp.dot(dg, ones, preferred_element_type=F32)
            wait("x0")
            run_now(STATS(0))
            wait("m10", "m00")
            run_now(MOD(1, 0, 1) + MOD(0, 0, 1) + FIN(0, 0))
            wait("w00", "w10", "w20")
            run_now(PERM(0, 0))

        m0 = [functools.partial(wave_pass, 0, t, nb) for t in range(2) for nb in range(6)]
        m1 = WAVE(1)
        n0, n1, n2 = W0
        p1, p2 = PERM(1, 0), PERM(2, 0)
        segment("T0a", m0[:n0], [(p1, 0, 1), (p2, 1, n0 - 0.5)], need={2: p1})
        wait("x1")
        s1, f1, u = STATS(1), FIN(1, 0), 6 - n0
        segment("T0b", m0[n0:n1], [(s1, 0, u - 1), (f1, u - 1, u - 0.5, s1)], need={u: s1 + f1})
        wait("m11", "m01", "w01")
        mods, f0, f1, pq, u = MOD(1, 1, 2) + MOD(0, 1, 2), FIN(0, 1), FIN(1, 1), PERM(0, 1), 12 - n1
        segment("T0c", m0[n1:] + m1[:n2],
                [(mods, 0, 0.5), (f0, u - 1, u - 0.5, mods), (f1, u - 0.5, u + 0.5, mods), (pq, 0, u - 1)],
                need={u: mods + f0 + pq, u + 2: f1})
        wait("w11", "w21")
        p1, p2 = PERM(1, 1), PERM(2, 1)
        segment("T1", m1[n2:WA[1]], [(p1, 0, 3 - n2), (p2, 3 - n2, 6.5 - n2)], need={4 - n2: p1, 8 - n2: p2})
        for k in range(2, NC):
            last = k == NC - 1
            wait(f"m1{k}", f"m0{k}", f"w0{k}", f"w1{k}", f"w2{k}", *(["x2"] if last else []))
            u = 12 - WA[k - 1]
            mods = MOD(1, k, k + 1) + MOD(0, k, k + 1)
            fins = [FIN(t, k) for t in range(2)]
            perms = [PERM(m, k) for m in range(3)]
            mend = max(0.5, u - WP[0])
            groups = [(mods[:1], 0, 1), (mods[1:], mend - 0.5 if mend > 2 else 0, mend),
                      (fins[0], u - WP[1], u - WP[2], mods), (fins[1], u - WP[2], u + 1, mods),
                      (perms[0], 0, u - WP[3]), (perms[1], u - WP[3], u + WP[4]), (perms[2], u + WP[4], u + WP[5])]
            if last:
                groups.append((LN1(2, hc_v), *T7L))
            segment(f"T{k}", WAVE(k - 1)[WA[k - 1]:] + (WAVE(k) if last else WAVE(k)[:WA[k]]), groups,
                    need={u: mods + fins[0] + perms[0], u + 2: fins[1], u + 4: perms[1], u + 8: perms[2]})
        wait("xr")

        def a_step(npc, p0, t0, t, carry):
            base = jnp.minimum(p0 // 2 + (t - t0) * (npc // 2), NG - npc // 2) * (2 * G)
            att = [attn_task(True, base, npc * G, g, AQ, masked=(p0 == 0 and g == 0)) for g in range(npc)]
            l1 = LN1(jnp.minimum(t + 1, NT - 1), hn_v)
            segment("A", QKV(t), [(att, *AA), (l1, *AL)] + COPY(hn_v, hc_v, 47, 47 + CPH, l1), dl=ADL)
            return carry

        with scope("loopA1"):
            jax.lax.fori_loop(2, 4, functools.partial(a_step, 8, 0, 2), 0)
        wait("wmr", "wo")
        q4, nq = QKV(4), AFP[0]
        l1, mg, msc = LN1(5, hn_v), MOD(2), MOD(3) + MOD(4)
        segment("AF", q4[:nq] + WO(0) + q4[nq:],
                [(mg, 0, AFP[1]), (msc, AFP[1], AFP[2]), (LN2(0, h2_v), max(AFP[3], nq + 16), AFP[4], msc),
                 (MOD(5), AFP[5], AFP[6]), (l1, AFP[7], AFP[8]), ([halo_task()], 1, 2)]
                + COPY(hn_v, hc_v, 63, 63 + CPH, l1), need={nq: mg}, dl=AFDL)
        with scope("loopA2"):
            jax.lax.fori_loop(5, NT, functools.partial(a_step, 6, 16, 5), 0)
        wait("fw1", "fw3", "fw2")

        def b_step(i, carry):
            att = [attn_task(False, jnp.minimum(i, NT - 3) * TM, TM, g, BQ) for g in range(NG)]
            l2 = LN2(i + 1, hn_v)
            assert BA[0] >= 16 and BL[0] >= 16 and min(BCP) >= 176
            segment("F", WO(i + 1) + FFN(i), [(att, *BA), (l2, *BL)] + COPY(hn_v, h2_v, *BCP, l2), dl=BDL)
            return carry

        with scope("B"):
            jax.lax.fori_loop(0, NT - 1, b_step, 0)
        for t in range(NT - 2):
            out_wait(t)
        segment("FL", FFN(NT - 1))
        for t in range(NT - 2, NT):
            out_wait(t)

    @jax.jit
    def fn(A_x, A_wqkv, A_wo, B_x, B_w1, B_w3, B_w2, c, w_mod):
        V = pltpu.VMEM
        scratch = [
            V((S, D), BF16), V((3, D, D), BF16), V((D // 2, 3 * D), U32), V((D, D), BF16),
            V((D, F), BF16), V((D, F), BF16), V((F, D), BF16), V((2 * NC, D, 128), BF16), V((D, 4 * D), BF16),
            V((8, D), F32), V((D, 128), F32), V((2, SA, 128), F32), V((2, TM // 2, D), U32),
            V((NC, SA, 128), F32), V((NC, PAD + SA, 128), F32), V((NC, PAD + SA, 128), F32),
            V((NC, SB, 128), F32), V((NC, PAD + SB, 128), F32), V((NC, PAD + SB, 128), F32),
            V((S // 2, D), U32), V((NC, S, 128), F32), V((TM // 2, D), U32), V((NC, S, 128), BF16),
            V((TM // 2, D), U32), V((TM // 2, D), U32), V((32, 128), F32), V((1, D), BF16),
            pltpu.SemaphoreType.DMA((5 * NC + 11,)), pltpu.SemaphoreType.DMA((NT,)), pltpu.SemaphoreType.REGULAR,
        ]
        out = pl.pallas_call(
            kernel,
            in_specs=[pl.BlockSpec(memory_space=pl.ANY)] * 8,
            out_specs=pl.BlockSpec(memory_space=pl.ANY),
            out_shape=jax.ShapeDtypeStruct((S, D), BF16),
            scratch_shapes=scratch,
            compiler_params=pltpu.CompilerParams(vmem_limit_bytes=124 * 1024 * 1024, disable_bounds_checks=True,
                                                 disable_semaphore_checks=True),
        )(A_x.reshape(S, D), A_wqkv, A_wo, B_w1, B_w3, B_w2, c, w_mod)
        return out.reshape(1, S, D)

    return fn


_impl = make_kernel()


@jax.jit
def pallas_adaLN_cond__sliding_local_dilated__glu_gated_swiglu__prompt_kernel(A_x, A_wqkv, A_wo, B_x, B_w1, B_w3, B_w2, c, w_mod):
    return _impl(A_x, A_wqkv, A_wo, B_x, B_w1, B_w3, B_w2, c, w_mod)
```

```python
import contextlib
import functools
import math

import jax
import jax.numpy as jnp
import jax.experimental.pallas as pl
import jax.experimental.pallas.tpu as pltpu

S, D, F = 2048, 1024, 3584
DH, WIN, DIL = 32, 8, 2
NC = D // 128
PAD = 16
EPS = 1e-5
SCALE = DH ** -0.5
EXP2_C = SCALE * math.log2(math.e)
MASKED = -1e9 / SCALE
F32, BF16, U32 = jnp.float32, jnp.bfloat16, jnp.uint32
TM = 256
NT = S // TM
G = 16
NG = TM // G
HK = D // 2
SA = 2 * TM
SB = S - SA


def _xor_network(xs):
    lane = jax.lax.broadcasted_iota(jnp.int32, xs[0].shape, 1)
    for b in range(3):
        m = ((lane >> (2 + b)) & 1) == 1
        xs = [jnp.where(m, xs[i ^ (1 << b)], xs[i]) for i in range(NC)]
    return xs


def _gather_fwd(z, j):
    lane = jax.lax.broadcasted_iota(jnp.int32, z.shape, 1)
    e, g, p = lane >> 5, (lane >> 3) & 3, lane & 7
    return jnp.take_along_axis(z, g * 32 + (p ^ j) * 4 + e, axis=1)


def _gather_inv(y, j):
    lane = jax.lax.broadcasted_iota(jnp.int32, y.shape, 1)
    g, q, e = lane >> 5, (lane >> 2) & 7, lane & 3
    return jnp.take_along_axis(y, e * 32 + g * 8 + (q ^ j), axis=1)


def _pack(x):
    return pltpu.bitcast(x.astype(BF16), U32)


def _or_all(vs):
    parts = [v[r:r + 8, c:c + 128] for v in vs for r in range(0, v.shape[0], 8) for c in range(0, v.shape[1], 128)]
    while len(parts) > 1:
        parts = [parts[i] | parts[i + 1] if i + 1 < len(parts) else parts[i] for i in range(0, len(parts), 2)]
    return parts[0]


def _gate(x, g):
    if g is None:
        return x
    xb = x if x.dtype == U32 else pltpu.bitcast(x, U32)
    y = xb | jnp.tile(g, (x.shape[0] // 8, x.shape[1] // 128))
    return y if x.dtype == U32 else pltpu.bitcast(y, x.dtype)


def _rows(start, n, mult):
    if isinstance(start, int):
        return pl.ds(start, n)
    return pl.ds(pl.multiple_of(start, mult), n)


def _stats(x):
    mu = jnp.mean(x, axis=-1, keepdims=True)
    xc = x - mu
    var = jnp.mean(xc * xc, axis=-1, keepdims=True)
    return mu, xc, jax.lax.rsqrt(var + EPS)


def make_kernel(NREL=2, DL=4,
                W0=(3, 9, 1), WA=(9, 9, 6, 6, 6, 6, 6), WP=(3.5, 1.5, 0.5, 1.5, 2, 5), X2AT=6, T7L=(8, 14),
                AQ=(2, 4, 4), AA=(0, 42), AL=(1, 38), ADL=5, CPH=0.75,
                AFP=(22, 16, 38, 41, 59, 28, 59, 0, 28), AFDL=6,
                BQ=(2, 2, 5), BA=(20, 170), BL=(21, 171), BCP=(176, 178), BDL=5,
                scopes=False, only=None):

    def scope(name):
        return jax.named_scope(name) if scopes else contextlib.nullcontext()

    def kernel(x_hbm, wqkv_hbm, wo_hbm, w1_hbm, w3_hbm, w2_hbm, c_hbm, wm_hbm, out_hbm,
               x_v, wraw_v, wp_v, wo_v, w1_v, w3_v, w2_v, wmc_v, wmr_v,
               mod_v, scol_v, st_v, h1_v, qa_v, ka_v, va_v, qb_v, kb_v, vb_v, o_v, x1_v, h2_v, out_v,
               hc_v, hn_v, z_v, c_v, sems, sem_out, bar):
        cp = pltpu.make_async_copy

        dmas = {}

        def add(name, src, dst):
            dmas[name] = cp(src, dst, sems.at[len(dmas)])

        def add_x(name, t0, n):
            add(name, x_hbm.at[pl.ds(t0 * TM, n * TM), :], x_v.at[pl.ds(t0 * TM, n * TM), :])

        add("c", c_hbm, c_v)
        add_x("x0", 0, 1)
        for k in range(NC):
            for m in (1, 0):
                add(f"m{m}{k}", wm_hbm.at[:, pl.ds(m * D + k * 128, 128)], wmc_v.at[m * NC + k])
            for m in range(3):
                add(f"w{m}{k}", wqkv_hbm.at[pl.ds(k * 128, 128), pl.ds(m * D, D)], wraw_v.at[m, pl.ds(k * 128, 128), :])
            if k == 0:
                add_x("x1", 1, 1)
            if k == X2AT:
                add_x("x2", 2, 1)
        add_x("xr", 3, NT - 3)
        add("wmr", wm_hbm.at[:, pl.ds(2 * D, 4 * D)], wmr_v)
        add("wo", wo_hbm, wo_v)
        add("fw1", w1_hbm, w1_v)
        add("fw3", w3_hbm, w3_v)
        add("fw2", w2_hbm, w2_v)
        for d in dmas.values():
            d.start()
            pl.semaphore_signal(bar, 1)
            pl.semaphore_wait(bar, 1)
        for j in range(NC):
            ka_v[j, 0:PAD, :] = jnp.zeros((PAD, 128), F32)
            va_v[j, 0:PAD, :] = jnp.zeros((PAD, 128), F32)
        add("z", ka_v.at[0, pl.ds(0, 8), :], z_v.at[pl.ds(0, 8), :])
        dmas["z"].start()

        def wait(*names):
            with scope("w_" + names[0]):
                for n in names:
                    dmas[n].wait()

        def zero():
            return pltpu.bitcast(z_v[0:8, :], U32)

        def mod_task(m, j):
            src = wmc_v.at[m * NC + j] if m < 2 else wmr_v.at[:, pl.ds((m - 2) * D + j * 128, 128)]
            acc = None
            for kb in range(D // 128):
                if kb % 2 == 0:
                    rel = yield
                p = src[kb * 128:(kb + 1) * 128, :].astype(F32) * scol_v[kb * 128:(kb + 1) * 128, :]
                parts = [p[r:r + 8] for r in range(0, 128, 8)]
                a0, a1 = parts[0], parts[1]
                if kb % 2 == 0:
                    a0, a1 = _gate(a0, rel), _gate(a1, rel)
                for r in range(2, 16, 2):
                    a0, a1 = a0 + parts[r], a1 + parts[r + 1]
                a0 = a0 + a1
                acc = a0 if acc is None else acc + a0
            r = jnp.sum(acc, axis=0, keepdims=True)
            if m in (1, 4):
                r = r + 1.0
            mod_v[m:m + 1, j * 128:(j + 1) * 128] = r
            return pltpu.bitcast(jnp.broadcast_to(r, (8, 128)), U32)

        def modulate(xn, ms, dst, g, c0, c1):
            hb = _pack(xn * mod_v[ms + 1:ms + 2, c0:c1] + mod_v[ms:ms + 1, c0:c1])
            dst[g * 8:(g + 1) * 8, c0:c1] = hb
            return _or_all([hb])

        def ln1_task(t, g, dst):
            rel = yield
            xt = x_v.at[_rows(t * TM, TM, TM), :]
            _, xc, rs = _stats(_gate(xt[g * G:(g + 1) * G, :].astype(F32), rel))
            return modulate(xc * rs, 0, dst, g, 0, D)

        def stats_task(t, g):
            rel = yield
            rows = slice(t * TM + g * G, t * TM + (g + 1) * G)
            mu, _, rs = _stats(_gate(x_v[rows, :].astype(F32), rel))
            st_v[0, rows, :] = jnp.broadcast_to(mu, (G, 128))
            st_v[1, rows, :] = jnp.broadcast_to(rs, (G, 128))

        def fin_task(t, k, g0, ng):
            rel = yield
            for g in range(g0, g0 + ng):
                rows = slice(t * TM + g * G, t * TM + (g + 1) * G)
                x = _gate(x_v[rows, k * 128:(k + 1) * 128].astype(F32), rel)
                modulate((x - st_v[0, rows, :]) * st_v[1, rows, :], 0, h1_v.at[t], g, k * 128, (k + 1) * 128)

        def ln2_task(t, g, dst):
            rel = yield
            xv = x1_v.at[:, _rows(t * TM, TM, TM), :]
            x = jnp.concatenate([_gate(xv[j, g * G:(g + 1) * G, :], rel) for j in range(NC)], axis=1)
            _, xc, rs = _stats(x)
            return modulate(xc * rs, 3, dst, g, 0, D)

        def perm_select_task(m, r0, n):
            rel = yield
            xs = [_gate(pltpu.bitcast(wraw_v[m, r0:r0 + n, j * 128:(j + 1) * 128], U32), rel) for j in range(NC)]
            zs = _xor_network(xs)
            for j in range(NC):
                wp_v[r0 // 2:(r0 + n) // 2, m * D + j * 128:m * D + (j + 1) * 128] = zs[j]

        def perm_gather_task(m, j, r0, n):
            rel = yield
            sl = (slice(r0 // 2, (r0 + n) // 2), slice(m * D + j * 128, m * D + (j + 1) * 128))
            wp_v[sl] = _gather_fwd(_gate(wp_v[sl], rel), j)

        def copy_task(src, dst, hf):
            rel = yield
            dst[:, hf * HK:(hf + 1) * HK] = _gate(src[:, hf * HK:(hf + 1) * HK], rel)

        def halo_task():
            yield
            for j in range(NC):
                kb_v[j, 0:PAD, :] = ka_v[j, SA:SA + PAD, :]
                vb_v[j, 0:PAD, :] = va_v[j, SA:SA + PAD, :]

        def attn_task(first, base, span, g, pace, masked=False):
            qkg, pvg, skip = pace
            q_v, k_v, v_v = (qa_v, ka_v, va_v) if first else (qb_v, kb_v, vb_v)
            qv = q_v.at[:, _rows(base, span, 32), :]
            kv = k_v.at[:, _rows(base, span + PAD, 32), :]
            vv = v_v.at[:, _rows(base, span + PAD, 32), :]

            def shifted(ref, j, w):
                return ref[j, pl.ds(g * G + PAD - DIL * w, G), :]

            q = [qv[j, g * G:(g + 1) * G, :] for j in range(NC)]
            ls = []
            for w in range(WIN):
                if w % qkg == 0:
                    rel = yield
                acc = _gate(q[0], rel) * shifted(kv, 0, w)
                for j in range(1, NC):
                    acc = acc + q[j] * shifted(kv, j, w)
                ls.append(acc)
            ls = [l + pltpu.roll(l, 64, 1) for l in ls]
            ls = [l + pltpu.roll(l, 32, 1) for l in ls]
            if masked:
                rows = base + g * G + jax.lax.broadcasted_iota(jnp.int32, (G, 128), 0)
                ls = [ls[0]] + [jnp.where(rows >= DIL * w, ls[w], MASKED) for w in range(1, WIN)]
            mx = ls[0]
            for w in range(1, WIN):
                mx = jnp.maximum(mx, ls[w])
            ps = [jnp.exp2((l - mx) * EXP2_C) for l in ls]
            den = ps[0]
            for w in range(1, WIN):
                den = den + ps[w]
            inv = 1.0 / den
            ps = [pw * inv for pw in ps]
            for _ in range(skip):
                rel = yield
            zs = []
            for j in range(NC):
                if j % pvg == 0:
                    rel = yield
                acc = _gate(ps[0], rel) * shifted(vv, j, 0)
                for w in range(1, WIN):
                    acc = acc + ps[w] * shifted(vv, j, w)
                zs.append(_gather_inv(_pack(acc), j))
            xs = _xor_network(zs)
            half = jax.lax.shift_right_logical(base, 1) + (0 if first else SA // 2)
            ov = o_v.at[_rows(half, span // 2, 16), :]
            for j in range(NC):
                ov[g * 8:(g + 1) * 8, j * 128:(j + 1) * 128] = xs[j]
            return _or_all(xs)

        def LN1(t, dst):
            return [ln1_task(t, g, dst) for g in range(NG)]

        def LN2(t, dst):
            return [ln2_task(t, g, dst) for g in range(NG)]

        def STATS(t):
            return [stats_task(t, g) for g in range(NG)]

        def FIN(t, k):
            return [fin_task(t, k, g0, 4) for g0 in range(0, NG, 4)]

        def MOD(m, j0=0, j1=NC):
            return [mod_task(m, j) for j in range(j0, j1)]

        def PERM(m, k):
            r0 = k * 128
            return ([perm_select_task(m, r, 32) for r in range(r0, r0 + 128, 32)]
                    + [perm_gather_task(m, j, r0, 128) for j in range(NC)])

        def COPY(src, dst, lo, hi, pre):
            return [([copy_task(src, dst, 0)], lo, lo + 1, pre), ([copy_task(src, dst, 1)], hi, hi + 1, pre)]

        def run_now(tasks):
            for tk in tasks:
                try:
                    next(tk)
                    while True:
                        tk.send(None)
                except StopIteration:
                    pass

        def tie(a, tok):
            if tok is not None:
                top = a[0:8, 0:128] | (tok & zero())
                if a.shape[1] > 128:
                    top = jnp.concatenate([top, a[0:8, 128:]], axis=1)
                a = jnp.concatenate([top, a[8:]], axis=0)
            return pltpu.bitcast(a, BF16)

        def releases(res):
            return [pltpu.bitcast(res[r:r + 8, 0:128], U32) & zero() for r in range(0, TM, TM // NREL)]

        def wave_pass(k, t, nb, tok):
            m, j0 = nb // 2, (nb % 2) * 4
            dst = (qa_v, ka_v, va_v)[m]
            rows = slice(t * TM + (PAD if m else 0), (t + 1) * TM + (PAD if m else 0))
            w = pltpu.bitcast(wp_v[k * 64:(k + 1) * 64, nb * 512:(nb + 1) * 512], BF16)
            res = jnp.dot(tie(h1_v[t, :, k * 128:(k + 1) * 128], tok), w, preferred_element_type=F32)
            for jj in range(4):
                r = res[:, jj * 128:(jj + 1) * 128]
                if k > 0:
                    r = dst[j0 + jj, rows, :] + r
                dst[j0 + jj, rows, :] = r
            return releases(res)

        def qkv_pass(t, m, j, hf, st, tok):
            w = pltpu.bitcast(wp_v[hf * HK // 2:(hf + 1) * HK // 2, m * D + j * 128:m * D + (j + 1) * 128], BF16)
            res = jnp.dot(tie(hc_v[:, hf * HK:(hf + 1) * HK], tok), w, preferred_element_type=F32)
            if hf == 0:
                st["a"] = res
            else:
                res = st.pop("a") + res
                off = PAD if m else 0
                dst = (qb_v, kb_v, vb_v)[m].at[:, _rows((t - 2) * TM, TM + off, TM), :]
                dst[j, off:off + TM, :] = res
            return releases(res)

        def wo_pass(t, j, hf, st, tok):
            h = tie(o_v[_rows(t * (TM // 2), TM // 2, TM // 2), hf * HK:(hf + 1) * HK], tok)
            res = jnp.dot(h, wo_v[hf * HK:(hf + 1) * HK, j * 128:(j + 1) * 128], preferred_element_type=F32)
            if hf == 0:
                st["a"] = res
            else:
                rows, cs = _rows(t * TM, TM, TM), slice(j * 128, (j + 1) * 128)
                res = x_v[rows, cs].astype(F32) + mod_v[2:3, cs] * (st.pop("a") + res)
                x1_v[j, rows, :] = res
            return releases(res)

        def out_copy(t, j):
            rows = _rows(t * TM, TM, TM)
            return cp(out_v.at[j, rows, :], out_hbm.at[rows, pl.ds(j * 128, 128)], sem_out.at[t])

        def out_wait(t):
            rows = pl.ds(t * TM, TM)
            cp(out_hbm.at[rows, :], out_hbm.at[rows, :], sem_out.at[t]).wait()

        def WAVE(k):
            return [functools.partial(wave_pass, k, t, nb) for m in range(3) for t in range(2) for nb in (2 * m, 2 * m + 1)]

        def QKV(t):
            st = {}
            return [functools.partial(qkv_pass, t, m, j, hf, st) for m in range(3) for j in range(NC) for hf in range(2)]

        def WO(t):
            st = {}
            return [functools.partial(wo_pass, t, j, hf, st) for j in range(NC) for hf in range(2)]

        def FFN(t):
            st = {"acc": [None] * NC, "act": []}

            def gate_up_pass(which, n, hf, tok):
                w = (w1_v, w3_v)[which][hf * HK:(hf + 1) * HK, n * 128:(n + 1) * 128]
                res = jnp.dot(tie(h2_v[:, hf * HK:(hf + 1) * HK], tok), w, preferred_element_type=F32)
                if hf == 0:
                    st["a"] = res
                else:
                    res = st.pop("a") + res
                    if which == 0:
                        hg = 0.5 * res
                        st["g"] = hg + hg * jnp.tanh(hg)
                    else:
                        st["act"].append((st.pop("g") * res).astype(BF16))
                return releases(res)

            def down_pass(c, j, last, tok):
                if j == 0:
                    st["lhs"], st["act"] = jnp.concatenate(st["act"], axis=1), []
                w = w2_v[c * HK:(c + 1) * HK, j * 128:(j + 1) * 128]
                if tok is not None:
                    w = tie(pltpu.bitcast(w, U32), tok)
                res = jnp.dot(st["lhs"], w, preferred_element_type=F32)
                if st["acc"][j] is not None:
                    res = st["acc"][j] + res
                st["acc"][j] = res
                if last:
                    rows = _rows(t * TM, TM, TM)
                    out_v[j, rows, :] = (x1_v[j, rows, :] + mod_v[5:6, j * 128:(j + 1) * 128] * res).astype(BF16)
                    out_copy(t, j).start()
                return releases(res)

            out = []
            nch = F // HK
            for c in range(nch):
                for n in range(c * 4, c * 4 + 4):
                    out += [functools.partial(gate_up_pass, which, n, hf) for which in range(2) for hf in range(2)]
                out += [functools.partial(down_pass, c, j, c == nch - 1) for j in range(NC)]
            return out

        def segment(name, passes, groups=(), dl=DL, need=None):
            if only is not None and name not in only:
                return
            with scope(name):
                n = len(passes)
                active = []
                for tasks, lo, hi, *pre in groups:
                    for k, tk in enumerate(tasks):
                        active.append((int((lo + k * (hi - lo) / len(tasks)) * NREL), tk, pre[0] if pre else ()))
                        next(tk)
                deadlines = [[] for _ in range(n + dl + 1)]

                def done(tasks):
                    return all(ent[1] is not tk for tk in tasks for ent in active)

                def feed(rel, slot, i):
                    for ent in list(active):
                        if ent[0] <= slot:
                            assert done(ent[2]), (name, i)
                            try:
                                ent[1].send(rel)
                            except StopIteration as e:
                                if e.value is not None:
                                    deadlines[i + dl].append(e.value)
                                active.remove(ent)

                feed(None, 0, 0)
                slot = 1
                for i, ps in enumerate(passes):
                    assert done((need or {}).get(i, ())), (name, i)
                    for rel in ps(_or_all(deadlines[i]) if deadlines[i] else None):
                        feed(rel, slot, i)
                        slot += 1
                while active:
                    feed(None, 1 << 30, n)

        with scope("S0"):
            wait("c", "z")
            c = c_v[...].astype(F32)
            s = (c * jax.nn.sigmoid(c)).astype(BF16).astype(F32)
            eye = (jax.lax.broadcasted_iota(jnp.int32, (128, 128), 0)
                   == jax.lax.broadcasted_iota(jnp.int32, (128, 128), 1))
            ones = jnp.ones((128, 128), BF16)
            for j in range(NC):
                dg = jnp.where(eye, jnp.broadcast_to(s[:, j * 128:(j + 1) * 128], (128, 128)), 0.0).astype(BF16)
                scol_v[j * 128:(j + 1) * 128, :] = jnp.dot(dg, ones, preferred_element_type=F32)
            wait("x0")
            run_now(STATS(0))
            wait("m10", "m00")
            run_now(MOD(1, 0, 1) + MOD(0, 0, 1) + FIN(0, 0))
            wait("w00", "w10", "w20")
            run_now(PERM(0, 0))

        m0 = [functools.partial(wave_pass, 0, t, nb) for t in range(2) for nb in range(6)]
        m1 = WAVE(1)
        n0, n1, n2 = W0
        p1, p2 = PERM(1, 0), PERM(2, 0)
        segment("T0a", m0[:n0], [(p1, 0, 1), (p2, 1, n0 - 0.5)], need={2: p1})
        wait("x1")
        s1, f1, u = STATS(1), FIN(1, 0), 6 - n0
        segment("T0b", m0[n0:n1], [(s1, 0, u - 1), (f1, u - 1, u - 0.5, s1)], need={u: s1 + f1})
        wait("m11", "m01", "w01")
        mods, f0, f1, pq, u = MOD(1, 1, 2) + MOD(0, 1, 2), FIN(0, 1), FIN(1, 1), PERM(0, 1), 12 - n1
        segment("T0c", m0[n1:] + m1[:n2],
                [(mods, 0, 0.5), (f0, u - 1, u - 0.5, mods), (f1, u - 0.5, u + 0.5, mods), (pq, 0, u - 1)],
                need={u: mods + f0 + pq, u + 2: f1})
        wait("w11", "w21")
        p1, p2 = PERM(1, 1), PERM(2, 1)
        segment("T1", m1[n2:WA[1]], [(p1, 0, 3 - n2), (p2, 3 - n2, 6.5 - n2)], need={4 - n2: p1, 8 - n2: p2})
        for k in range(2, NC):
            last = k == NC - 1
            wait(f"m1{k}", f"m0{k}", f"w0{k}", f"w1{k}", f"w2{k}", *(["x2"] if last else []))
            u = 12 - WA[k - 1]
            mods = MOD(1, k, k + 1) + MOD(0, k, k + 1)
            fins = [FIN(t, k) for t in range(2)]
            perms = [PERM(m, k) for m in range(3)]
            mend = max(0.5, u - WP[0])
            groups = [(mods[:1], 0, 1), (mods[1:], mend - 0.5 if mend > 2 else 0, mend),
                      (fins[0], u - WP[1], u - WP[2], mods), (fins[1], u - WP[2], u + 1, mods),
                      (perms[0], 0, u - WP[3]), (perms[1], u - WP[3], u + WP[4]), (perms[2], u + WP[4], u + WP[5])]
            if last:
                groups.append((LN1(2, hc_v), *T7L))
            segment(f"T{k}", WAVE(k - 1)[WA[k - 1]:] + (WAVE(k) if last else WAVE(k)[:WA[k]]), groups,
                    need={u: mods + fins[0] + perms[0], u + 2: fins[1], u + 4: perms[1], u + 8: perms[2]})
        wait("xr")

        def a_step(npc, p0, t0, t, carry):
            base = jnp.minimum(p0 // 2 + (t - t0) * (npc // 2), NG - npc // 2) * (2 * G)
            att = [attn_task(True, base, npc * G, g, AQ, masked=(p0 == 0 and g == 0)) for g in range(npc)]
            l1 = LN1(jnp.minimum(t + 1, NT - 1), hn_v)
            segment("A", QKV(t), [(att, *AA), (l1, *AL)] + COPY(hn_v, hc_v, 47, 47 + CPH, l1), dl=ADL)
            return carry

        with scope("loopA1"):
            jax.lax.fori_loop(2, 4, functools.partial(a_step, 8, 0, 2), 0)
        wait("wmr", "wo")
        q4, nq = QKV(4), AFP[0]
        l1, mg, msc = LN1(5, hn_v), MOD(2), MOD(3) + MOD(4)
        segment("AF", q4[:nq] + WO(0) + q4[nq:],
                [(mg, 0, AFP[1]), (msc, AFP[1], AFP[2]), (LN2(0, h2_v), max(AFP[3], nq + 16), AFP[4], msc),
                 (MOD(5), AFP[5], AFP[6]), (l1, AFP[7], AFP[8]), ([halo_task()], 1, 2)]
                + COPY(hn_v, hc_v, 63, 63 + CPH, l1), need={nq: mg}, dl=AFDL)
        with scope("loopA2"):
            jax.lax.fori_loop(5, NT, functools.partial(a_step, 6, 16, 5), 0)
        wait("fw1", "fw3", "fw2")

        def b_step(i, carry):
            att = [attn_task(False, jnp.minimum(i, NT - 3) * TM, TM, g, BQ) for g in range(NG)]
            l2 = LN2(i + 1, hn_v)
            assert BA[0] >= 16 and BL[0] >= 16 and min(BCP) >= 176
            segment("F", WO(i + 1) + FFN(i), [(att, *BA), (l2, *BL)] + COPY(hn_v, h2_v, *BCP, l2), dl=BDL)
            return carry

        with scope("B"):
            jax.lax.fori_loop(0, NT - 1, b_step, 0)
        for t in range(NT - 2):
            out_wait(t)
        segment("FL", FFN(NT - 1))
        for t in range(NT - 2, NT):
            out_wait(t)

    @jax.jit
    def fn(A_x, A_wqkv, A_wo, B_x, B_w1, B_w3, B_w2, c, w_mod):
        V = pltpu.VMEM
        scratch = [
            V((S, D), BF16), V((3, D, D), BF16), V((D // 2, 3 * D), U32), V((D, D), BF16),
            V((D, F), BF16), V((D, F), BF16), V((F, D), BF16), V((2 * NC, D, 128), BF16), V((D, 4 * D), BF16),
            V((8, D), F32), V((D, 128), F32), V((2, SA, 128), F32), V((2, TM // 2, D), U32),
            V((NC, SA, 128), F32), V((NC, PAD + SA, 128), F32), V((NC, PAD + SA, 128), F32),
            V((NC, SB, 128), F32), V((NC, PAD + SB, 128), F32), V((NC, PAD + SB, 128), F32),
            V((S // 2, D), U32), V((NC, S, 128), F32), V((TM // 2, D), U32), V((NC, S, 128), BF16),
            V((TM // 2, D), U32), V((TM // 2, D), U32), V((32, 128), F32), V((1, D), BF16),
            pltpu.SemaphoreType.DMA((5 * NC + 11,)), pltpu.SemaphoreType.DMA((NT,)), pltpu.SemaphoreType.REGULAR,
        ]
        out = pl.pallas_call(
            kernel,
            in_specs=[pl.BlockSpec(memory_space=pl.ANY)] * 8,
            out_specs=pl.BlockSpec(memory_space=pl.ANY),
            out_shape=jax.ShapeDtypeStruct((S, D), BF16),
            scratch_shapes=scratch,
            compiler_params=pltpu.CompilerParams(vmem_limit_bytes=124 * 1024 * 1024, disable_bounds_checks=True,
                                                 disable_semaphore_checks=True),
        )(A_x.reshape(S, D), A_wqkv, A_wo, B_w1, B_w3, B_w2, c, w_mod)
        return out.reshape(1, S, D)

    return fn


_impl = make_kernel()


@jax.jit
def pallas_adaLN_cond__sliding_local_dilated__glu_gated_swiglu__prompt_kernel(A_x, A_wqkv, A_wo, B_x, B_w1, B_w3, B_w2, c, w_mod):
    return _impl(A_x, A_wqkv, A_wo, B_x, B_w1, B_w3, B_w2, c, w_mod)
```

```python
import contextlib
import functools
import math

import jax
import jax.numpy as jnp
import jax.experimental.pallas as pl
import jax.experimental.pallas.tpu as pltpu

S, D, F = 2048, 1024, 3584
DH, WIN, DIL = 32, 8, 2
NC = D // 128
PAD = 16
EPS = 1e-5
SCALE = DH ** -0.5
EXP2_C = SCALE * math.log2(math.e)
MASKED = -1e9 / SCALE
F32, BF16, U32 = jnp.float32, jnp.bfloat16, jnp.uint32
TM = 256
NT = S // TM
G = 16
NG = TM // G
HK = D // 2
SA = 2 * TM
SB = S - SA


def _xor_network(xs):
    lane = jax.lax.broadcasted_iota(jnp.int32, xs[0].shape, 1)
    for b in range(3):
        m = ((lane >> (2 + b)) & 1) == 1
        xs = [jnp.where(m, xs[i ^ (1 << b)], xs[i]) for i in range(NC)]
    return xs


def _gather_fwd(z, j):
    lane = jax.lax.broadcasted_iota(jnp.int32, z.shape, 1)
    e, g, p = lane >> 5, (lane >> 3) & 3, lane & 7
    return jnp.take_along_axis(z, g * 32 + (p ^ j) * 4 + e, axis=1)


def _gather_inv(y, j):
    lane = jax.lax.broadcasted_iota(jnp.int32, y.shape, 1)
    g, q, e = lane >> 5, (lane >> 2) & 7, lane & 3
    return jnp.take_along_axis(y, e * 32 + g * 8 + (q ^ j), axis=1)


def _pack(x):
    return pltpu.bitcast(x.astype(BF16), U32)


def _or_all(vs):
    parts = [v[r:r + 8, c:c + 128] for v in vs for r in range(0, v.shape[0], 8) for c in range(0, v.shape[1], 128)]
    while len(parts) > 1:
        parts = [parts[i] | parts[i + 1] if i + 1 < len(parts) else parts[i] for i in range(0, len(parts), 2)]
    return parts[0]


def _gate(x, g):
    if g is None:
        return x
    xb = x if x.dtype == U32 else pltpu.bitcast(x, U32)
    y = xb | jnp.tile(g, (x.shape[0] // 8, x.shape[1] // 128))
    return y if x.dtype == U32 else pltpu.bitcast(y, x.dtype)


def _rows(start, n, mult):
    if isinstance(start, int):
        return pl.ds(start, n)
    return pl.ds(pl.multiple_of(start, mult), n)


def _stats(x):
    mu = jnp.mean(x, axis=-1, keepdims=True)
    xc = x - mu
    var = jnp.mean(xc * xc, axis=-1, keepdims=True)
    return mu, xc, jax.lax.rsqrt(var + EPS)


def make_kernel(NREL=2, DL=4,
                W0=(4, 10, 3), WA=(9, 10, 7, 6, 6, 6, 6), WP=(3.5, 1.5, 0.5, 1.5, 2, 5), X2AT=6, T7L=(8, 14),
                AQ=(2, 4, 4), AA=(0, 42), AL=(1, 38), ADL=5, CPH=0.75,
                AFP=(22, 16, 38, 41, 59, 28, 59, 0, 28), AFDL=6,
                BQ=(2, 2, 5), BA=(20, 174), BL=(21, 171), BCP=(176, 178), BDL=5,
                scopes=False, only=None):

    def scope(name):
        return jax.named_scope(name) if scopes else contextlib.nullcontext()

    def kernel(x_hbm, wqkv_hbm, wo_hbm, w1_hbm, w3_hbm, w2_hbm, c_hbm, wm_hbm, out_hbm,
               x_v, wraw_v, wp_v, wo_v, w1_v, w3_v, w2_v, wmc_v, wmr_v,
               mod_v, scol_v, st_v, h1_v, qa_v, ka_v, va_v, qb_v, kb_v, vb_v, o_v, x1_v, h2_v, out_v,
               hc_v, hn_v, z_v, c_v, sems, sem_out, bar):
        cp = pltpu.make_async_copy

        dmas = {}

        def add(name, src, dst):
            dmas[name] = cp(src, dst, sems.at[len(dmas)])

        def add_x(name, t0, n):
            add(name, x_hbm.at[pl.ds(t0 * TM, n * TM), :], x_v.at[pl.ds(t0 * TM, n * TM), :])

        add("c", c_hbm, c_v)
        add_x("x0", 0, 1)
        for k in range(NC):
            for m in (1, 0):
                add(f"m{m}{k}", wm_hbm.at[:, pl.ds(m * D + k * 128, 128)], wmc_v.at[m * NC + k])
            for m in range(3):
                add(f"w{m}{k}", wqkv_hbm.at[pl.ds(k * 128, 128), pl.ds(m * D, D)], wraw_v.at[m, pl.ds(k * 128, 128), :])
            if k == 0:
                add_x("x1", 1, 1)
            if k == X2AT:
                add_x("x2", 2, 1)
        add_x("xr", 3, NT - 3)
        add("wmr", wm_hbm.at[:, pl.ds(2 * D, 4 * D)], wmr_v)
        add("wo", wo_hbm, wo_v)
        add("fw1", w1_hbm, w1_v)
        add("fw3", w3_hbm, w3_v)
        add("fw2", w2_hbm, w2_v)
        for d in dmas.values():
            d.start()
            pl.semaphore_signal(bar, 1)
            pl.semaphore_wait(bar, 1)
        for j in range(NC):
            ka_v[j, 0:PAD, :] = jnp.zeros((PAD, 128), F32)
            va_v[j, 0:PAD, :] = jnp.zeros((PAD, 128), F32)
        add("z", ka_v.at[0, pl.ds(0, 8), :], z_v.at[pl.ds(0, 8), :])
        dmas["z"].start()

        def wait(*names):
            with scope("w_" + names[0]):
                for n in names:
                    dmas[n].wait()

        def zero():
            return pltpu.bitcast(z_v[0:8, :], U32)

        def mod_task(m, j):
            src = wmc_v.at[m * NC + j] if m < 2 else wmr_v.at[:, pl.ds((m - 2) * D + j * 128, 128)]
            acc = None
            for kb in range(D // 128):
                if kb % 2 == 0:
                    rel = yield
                p = src[kb * 128:(kb + 1) * 128, :].astype(F32) * scol_v[kb * 128:(kb + 1) * 128, :]
                parts = [p[r:r + 8] for r in range(0, 128, 8)]
                a0, a1 = parts[0], parts[1]
                if kb % 2 == 0:
                    a0, a1 = _gate(a0, rel), _gate(a1, rel)
                for r in range(2, 16, 2):
                    a0, a1 = a0 + parts[r], a1 + parts[r + 1]
                a0 = a0 + a1
                acc = a0 if acc is None else acc + a0
            r = jnp.sum(acc, axis=0, keepdims=True)
            if m in (1, 4):
                r = r + 1.0
            mod_v[m:m + 1, j * 128:(j + 1) * 128] = r
            return pltpu.bitcast(jnp.broadcast_to(r, (8, 128)), U32)

        def modulate(xn, ms, dst, g, c0, c1):
            hb = _pack(xn * mod_v[ms + 1:ms + 2, c0:c1] + mod_v[ms:ms + 1, c0:c1])
            dst[g * 8:(g + 1) * 8, c0:c1] = hb
            return _or_all([hb])

        def ln1_task(t, g, dst):
            rel = yield
            xt = x_v.at[_rows(t * TM, TM, TM), :]
            _, xc, rs = _stats(_gate(xt[g * G:(g + 1) * G, :].astype(F32), rel))
            return modulate(xc * rs, 0, dst, g, 0, D)

        def stats_task(t, g):
            rel = yield
            rows = slice(t * TM + g * G, t * TM + (g + 1) * G)
            mu, _, rs = _stats(_gate(x_v[rows, :].astype(F32), rel))
            st_v[0, rows, :] = jnp.broadcast_to(mu, (G, 128))
            st_v[1, rows, :] = jnp.broadcast_to(rs, (G, 128))

        def fin_task(t, k, g0, ng):
            rel = yield
            for g in range(g0, g0 + ng):
                rows = slice(t * TM + g * G, t * TM + (g + 1) * G)
                x = _gate(x_v[rows, k * 128:(k + 1) * 128].astype(F32), rel)
                modulate((x - st_v[0, rows, :]) * st_v[1, rows, :], 0, h1_v.at[t], g, k * 128, (k + 1) * 128)

        def ln2_task(t, g, dst):
            rel = yield
            xv = x1_v.at[:, _rows(t * TM, TM, TM), :]
            x = jnp.concatenate([_gate(xv[j, g * G:(g + 1) * G, :], rel) for j in range(NC)], axis=1)
            _, xc, rs = _stats(x)
            return modulate(xc * rs, 3, dst, g, 0, D)

        def perm_select_task(m, r0, n):
            rel = yield
            xs = [_gate(pltpu.bitcast(wraw_v[m, r0:r0 + n, j * 128:(j + 1) * 128], U32), rel) for j in range(NC)]
            zs = _xor_network(xs)
            for j in range(NC):
                wp_v[r0 // 2:(r0 + n) // 2, m * D + j * 128:m * D + (j + 1) * 128] = zs[j]

        def perm_gather_task(m, j, r0, n):
            rel = yield
            sl = (slice(r0 // 2, (r0 + n) // 2), slice(m * D + j * 128, m * D + (j + 1) * 128))
            wp_v[sl] = _gather_fwd(_gate(wp_v[sl], rel), j)

        def copy_task(src, dst, hf):
            rel = yield
            dst[:, hf * HK:(hf + 1) * HK] = _gate(src[:, hf * HK:(hf + 1) * HK], rel)

        def halo_task():
            yield
            for j in range(NC):
                kb_v[j, 0:PAD, :] = ka_v[j, SA:SA + PAD, :]
                vb_v[j, 0:PAD, :] = va_v[j, SA:SA + PAD, :]

        def attn_task(first, base, span, g, pace, masked=False):
            qkg, pvg, skip = pace
            q_v, k_v, v_v = (qa_v, ka_v, va_v) if first else (qb_v, kb_v, vb_v)
            qv = q_v.at[:, _rows(base, span, 32), :]
            kv = k_v.at[:, _rows(base, span + PAD, 32), :]
            vv = v_v.at[:, _rows(base, span + PAD, 32), :]

            def shifted(ref, j, w):
                return ref[j, pl.ds(g * G + PAD - DIL * w, G), :]

            q = [qv[j, g * G:(g + 1) * G, :] for j in range(NC)]
            ls = []
            for w in range(WIN):
                if w % qkg == 0:
                    rel = yield
                acc = _gate(q[0], rel) * shifted(kv, 0, w)
                for j in range(1, NC):
                    acc = acc + q[j] * shifted(kv, j, w)
                ls.append(acc)
            ls = [l + pltpu.roll(l, 64, 1) for l in ls]
            ls = [l + pltpu.roll(l, 32, 1) for l in ls]
            if masked:
                rows = base + g * G + jax.lax.broadcasted_iota(jnp.int32, (G, 128), 0)
                ls = [ls[0]] + [jnp.where(rows >= DIL * w, ls[w], MASKED) for w in range(1, WIN)]
            mx = ls[0]
            for w in range(1, WIN):
                mx = jnp.maximum(mx, ls[w])
            ps = [jnp.exp2((l - mx) * EXP2_C) for l in ls]
            den = ps[0]
            for w in range(1, WIN):
                den = den + ps[w]
            inv = 1.0 / den
            ps = [pw * inv for pw in ps]
            for _ in range(skip):
                rel = yield
            zs = []
            for j in range(NC):
                if j % pvg == 0:
                    rel = yield
                acc = _gate(ps[0], rel) * shifted(vv, j, 0)
                for w in range(1, WIN):
                    acc = acc + ps[w] * shifted(vv, j, w)
                zs.append(_gather_inv(_pack(acc), j))
            xs = _xor_network(zs)
            half = jax.lax.shift_right_logical(base, 1) + (0 if first else SA // 2)
            ov = o_v.at[_rows(half, span // 2, 16), :]
            for j in range(NC):
                ov[g * 8:(g + 1) * 8, j * 128:(j + 1) * 128] = xs[j]
            return _or_all(xs)

        def LN1(t, dst):
            return [ln1_task(t, g, dst) for g in range(NG)]

        def LN2(t, dst):
            return [ln2_task(t, g, dst) for g in range(NG)]

        def STATS(t):
            return [stats_task(t, g) for g in range(NG)]

        def FIN(t, k):
            return [fin_task(t, k, g0, 4) for g0 in range(0, NG, 4)]

        def MOD(m, j0=0, j1=NC):
            return [mod_task(m, j) for j in range(j0, j1)]

        def PERM(m, k):
            r0 = k * 128
            return ([perm_select_task(m, r, 32) for r in range(r0, r0 + 128, 32)]
                    + [perm_gather_task(m, j, r0, 128) for j in range(NC)])

        def COPY(src, dst, lo, hi, pre):
            return [([copy_task(src, dst, 0)], lo, lo + 1, pre), ([copy_task(src, dst, 1)], hi, hi + 1, pre)]

        def run_now(tasks):
            for tk in tasks:
                try:
                    next(tk)
                    while True:
                        tk.send(None)
                except StopIteration:
                    pass

        def tie(a, tok):
            if tok is not None:
                top = a[0:8, 0:128] | (tok & zero())
                if a.shape[1] > 128:
                    top = jnp.concatenate([top, a[0:8, 128:]], axis=1)
                a = jnp.concatenate([top, a[8:]], axis=0)
            return pltpu.bitcast(a, BF16)

        def releases(res):
            return [pltpu.bitcast(res[r:r + 8, 0:128], U32) & zero() for r in range(0, TM, TM // NREL)]

        def wave_pass(k, t, nb, tok):
            m, j0 = nb // 2, (nb % 2) * 4
            dst = (qa_v, ka_v, va_v)[m]
            rows = slice(t * TM + (PAD if m else 0), (t + 1) * TM + (PAD if m else 0))
            w = pltpu.bitcast(wp_v[k * 64:(k + 1) * 64, nb * 512:(nb + 1) * 512], BF16)
            res = jnp.dot(tie(h1_v[t, :, k * 128:(k + 1) * 128], tok), w, preferred_element_type=F32)
            for jj in range(4):
                r = res[:, jj * 128:(jj + 1) * 128]
                if k > 0:
                    r = dst[j0 + jj, rows, :] + r
                dst[j0 + jj, rows, :] = r
            return releases(res)

        def qkv_pass(t, m, j, hf, st, tok):
            w = pltpu.bitcast(wp_v[hf * HK // 2:(hf + 1) * HK // 2, m * D + j * 128:m * D + (j + 1) * 128], BF16)
            res = jnp.dot(tie(hc_v[:, hf * HK:(hf + 1) * HK], tok), w, preferred_element_type=F32)
            if hf == 0:
                st["a"] = res
            else:
                res = st.pop("a") + res
                off = PAD if m else 0
                dst = (qb_v, kb_v, vb_v)[m].at[:, _rows((t - 2) * TM, TM + off, TM), :]
                dst[j, off:off + TM, :] = res
            return releases(res)

        def wo_pass(t, j, hf, st, tok):
            h = tie(o_v[_rows(t * (TM // 2), TM // 2, TM // 2), hf * HK:(hf + 1) * HK], tok)
            res = jnp.dot(h, wo_v[hf * HK:(hf + 1) * HK, j * 128:(j + 1) * 128], preferred_element_type=F32)
            if hf == 0:
                st["a"] = res
            else:
                rows, cs = _rows(t * TM, TM, TM), slice(j * 128, (j + 1) * 128)
                res = x_v[rows, cs].astype(F32) + mod_v[2:3, cs] * (st.pop("a") + res)
                x1_v[j, rows, :] = res
            return releases(res)

        def out_copy(t, j):
            rows = _rows(t * TM, TM, TM)
            return cp(out_v.at[j, rows, :], out_hbm.at[rows, pl.ds(j * 128, 128)], sem_out.at[t])

        def out_wait(t):
            rows = pl.ds(t * TM, TM)
            cp(out_hbm.at[rows, :], out_hbm.at[rows, :], sem_out.at[t]).wait()

        def WAVE(k):
            return [functools.partial(wave_pass, k, t, nb) for m in range(3) for t in range(2) for nb in (2 * m, 2 * m + 1)]

        def QKV(t):
            st = {}
            return [functools.partial(qkv_pass, t, m, j, hf, st) for m in range(3) for j in range(NC) for hf in range(2)]

        def WO(t):
            st = {}
            return [functools.partial(wo_pass, t, j, hf, st) for j in range(NC) for hf in range(2)]

        def FFN(t):
            st = {"acc": [None] * NC, "act": []}

            def gate_up_pass(which, n, hf, tok):
                w = (w1_v, w3_v)[which][hf * HK:(hf + 1) * HK, n * 128:(n + 1) * 128]
                res = jnp.dot(tie(h2_v[:, hf * HK:(hf + 1) * HK], tok), w, preferred_element_type=F32)
                if hf == 0:
                    st["a"] = res
                else:
                    res = st.pop("a") + res
                    if which == 0:
                        hg = 0.5 * res
                        st["g"] = hg + hg * jnp.tanh(hg)
                    else:
                        st["act"].append((st.pop("g") * res).astype(BF16))
                return releases(res)

            def down_pass(c, j, last, tok):
                if j == 0:
                    st["lhs"], st["act"] = jnp.concatenate(st["act"], axis=1), []
                w = w2_v[c * HK:(c + 1) * HK, j * 128:(j + 1) * 128]
                if tok is not None:
                    w = tie(pltpu.bitcast(w, U32), tok)
                res = jnp.dot(st["lhs"], w, preferred_element_type=F32)
                if st["acc"][j] is not None:
                    res = st["acc"][j] + res
                st["acc"][j] = res
                if last:
                    rows = _rows(t * TM, TM, TM)
                    out_v[j, rows, :] = (x1_v[j, rows, :] + mod_v[5:6, j * 128:(j + 1) * 128] * res).astype(BF16)
                    out_copy(t, j).start()
                return releases(res)

            out = []
            nch = F // HK
            for c in range(nch):
                for n in range(c * 4, c * 4 + 4):
                    out += [functools.partial(gate_up_pass, which, n, hf) for which in range(2) for hf in range(2)]
                out += [functools.partial(down_pass, c, j, c == nch - 1) for j in range(NC)]
            return out

        def segment(name, passes, groups=(), dl=DL, need=None):
            if only is not None and name not in only:
                return
            with scope(name):
                n = len(passes)
                active = []
                for tasks, lo, hi, *pre in groups:
                    for k, tk in enumerate(tasks):
                        active.append((int((lo + k * (hi - lo) / len(tasks)) * NREL), tk, pre[0] if pre else ()))
                        next(tk)
                deadlines = [[] for _ in range(n + dl + 1)]

                def done(tasks):
                    return all(ent[1] is not tk for tk in tasks for ent in active)

                def feed(rel, slot, i):
                    for ent in list(active):
                        if ent[0] <= slot:
                            assert done(ent[2]), (name, i)
                            try:
                                ent[1].send(rel)
                            except StopIteration as e:
                                if e.value is not None:
                                    deadlines[i + dl].append(e.value)
                                active.remove(ent)

                feed(None, 0, 0)
                slot = 1
                for i, ps in enumerate(passes):
                    assert done((need or {}).get(i, ())), (name, i)
                    for rel in ps(_or_all(deadlines[i]) if deadlines[i] else None):
                        feed(rel, slot, i)
                        slot += 1
                while active:
                    feed(None, 1 << 30, n)

        with scope("S0"):
            wait("c", "z")
            c = c_v[...].astype(F32)
            s = (c * jax.nn.sigmoid(c)).astype(BF16).astype(F32)
            eye = (jax.lax.broadcasted_iota(jnp.int32, (128, 128), 0)
                   == jax.lax.broadcasted_iota(jnp.int32, (128, 128), 1))
            ones = jnp.ones((128, 128), BF16)
            for j in range(NC):
                dg = jnp.where(eye, jnp.broadcast_to(s[:, j * 128:(j + 1) * 128], (128, 128)), 0.0).astype(BF16)
                scol_v[j * 128:(j + 1) * 128, :] = jnp.dot(dg, ones, preferred_element_type=F32)
            wait("x0")
            run_now(STATS(0))
            wait("m10", "m00")
            run_now(MOD(1, 0, 1) + MOD(0, 0, 1) + FIN(0, 0))
            wait("w00")
            run_now(PERM(0, 0))
            wait("w10", "w20")

        m0 = [functools.partial(wave_pass, 0, t, nb) for t in range(2) for nb in range(6)]
        m1 = WAVE(1)
        n0, n1, n2 = W0
        p1, p2 = PERM(1, 0), PERM(2, 0)
        segment("T0a", m0[:n0], [(p1, 0, 1), (p2, 1, n0 - 0.5)], need={2: p1})
        wait("x1")
        s1, f1, u = STATS(1), FIN(1, 0), 6 - n0
        segment("T0b", m0[n0:n1], [(s1, 0, max(0.4, u - 1)), (f1, u - 0.5 if u < 3 else u - 1, u - 0.4, s1)], need={u: s1 + f1})
        wait("m11", "m01", "w01")
        mods, f0, f1, pq, u = MOD(1, 1, 2) + MOD(0, 1, 2), FIN(0, 1), FIN(1, 1), PERM(0, 1), 12 - n1
        segment("T0c", m0[n1:] + m1[:n2],
                [(mods, 0, 0.4), (f0, max(1.5, u - 1), max(1.5, u - 1) + 0.4, mods), (f1, u - 0.5, u + 0.5, mods), (pq, 0, u - 1)],
                need={u: mods + f0 + pq, u + 2: f1})
        wait("w11", "w21")
        p1, p2 = PERM(1, 1), PERM(2, 1)
        segment("T1", m1[n2:WA[1]], [(p1, 0, 3 - n2), (p2, 3 - n2, 6.5 - n2)], need={4 - n2: p1, 8 - n2: p2})
        for k in range(2, NC):
            last = k == NC - 1
            wait(f"m1{k}", f"m0{k}", f"w0{k}", f"w1{k}", f"w2{k}", *(["x2"] if last else []))
            u = 12 - WA[k - 1]
            mods = MOD(1, k, k + 1) + MOD(0, k, k + 1)
            fins = [FIN(t, k) for t in range(2)]
            perms = [PERM(m, k) for m in range(3)]
            mend = max(0.5, u - WP[0])
            groups = [(mods[:1], 0, 1), (mods[1:], mend - 0.5 if mend > 2 else 0, mend),
                      (fins[0], max(1.5, u - WP[1]), max(1.9, u - WP[2]), mods), (fins[1], max(1.9, u - WP[2]), u + 1, mods),
                      (perms[0], 0, max(0.9, u - WP[3])), (perms[1], max(0.9, u - WP[3]), u + WP[4]), (perms[2], u + WP[4], u + WP[5])]
            if last:
                groups.append((LN1(2, hc_v), *T7L))
            segment(f"T{k}", WAVE(k - 1)[WA[k - 1]:] + (WAVE(k) if last else WAVE(k)[:WA[k]]), groups,
                    need={u: mods + fins[0] + perms[0], u + 2: fins[1], u + 4: perms[1], u + 8: perms[2]})
        wait("xr")

        def a_step(npc, p0, t0, t, carry):
            base = jnp.minimum(p0 // 2 + (t - t0) * (npc // 2), NG - npc // 2) * (2 * G)
            att = [attn_task(True, base, npc * G, g, AQ, masked=(p0 == 0 and g == 0)) for g in range(npc)]
            l1 = LN1(jnp.minimum(t + 1, NT - 1), hn_v)
            segment("A", QKV(t), [(att, *AA), (l1, *AL)] + COPY(hn_v, hc_v, 47, 47 + CPH, l1), dl=ADL)
            return carry

        with scope("loopA1"):
            jax.lax.fori_loop(2, 4, functools.partial(a_step, 8, 0, 2), 0)
        wait("wmr", "wo")
        q4, nq = QKV(4), AFP[0]
        l1, mg, msc = LN1(5, hn_v), MOD(2), MOD(3) + MOD(4)
        segment("AF", q4[:nq] + WO(0) + q4[nq:],
                [(mg, 0, AFP[1]), (msc, AFP[1], AFP[2]), (LN2(0, h2_v), max(AFP[3], nq + 16), AFP[4], msc),
                 (MOD(5), AFP[5], AFP[6]), (l1, AFP[7], AFP[8]), ([halo_task()], 1, 2)]
                + COPY(hn_v, hc_v, 63, 63 + CPH, l1), need={nq: mg}, dl=AFDL)
        with scope("loopA2"):
            jax.lax.fori_loop(5, NT, functools.partial(a_step, 6, 16, 5), 0)
        wait("fw1", "fw3", "fw2")

        def b_step(i, carry):
            att = [attn_task(False, jnp.minimum(i, NT - 3) * TM, TM, g, BQ) for g in range(NG)]
            l2 = LN2(i + 1, hn_v)
            assert BA[0] >= 16 and BL[0] >= 16 and min(BCP) >= 176
            segment("F", WO(i + 1) + FFN(i), [(att, *BA), (l2, *BL)] + COPY(hn_v, h2_v, *BCP, l2), dl=BDL)
            return carry

        with scope("B"):
            jax.lax.fori_loop(0, NT - 1, b_step, 0)
        for t in range(NT - 2):
            out_wait(t)
        segment("FL", FFN(NT - 1))
        for t in range(NT - 2, NT):
            out_wait(t)

    @jax.jit
    def fn(A_x, A_wqkv, A_wo, B_x, B_w1, B_w3, B_w2, c, w_mod):
        V = pltpu.VMEM
        scratch = [
            V((S, D), BF16), V((3, D, D), BF16), V((D // 2, 3 * D), U32), V((D, D), BF16),
            V((D, F), BF16), V((D, F), BF16), V((F, D), BF16), V((2 * NC, D, 128), BF16), V((D, 4 * D), BF16),
            V((8, D), F32), V((D, 128), F32), V((2, SA, 128), F32), V((2, TM // 2, D), U32),
            V((NC, SA, 128), F32), V((NC, PAD + SA, 128), F32), V((NC, PAD + SA, 128), F32),
            V((NC, SB, 128), F32), V((NC, PAD + SB, 128), F32), V((NC, PAD + SB, 128), F32),
            V((S // 2, D), U32), V((NC, S, 128), F32), V((TM // 2, D), U32), V((NC, S, 128), BF16),
            V((TM // 2, D), U32), V((TM // 2, D), U32), V((32, 128), F32), V((1, D), BF16),
            pltpu.SemaphoreType.DMA((5 * NC + 11,)), pltpu.SemaphoreType.DMA((NT,)), pltpu.SemaphoreType.REGULAR,
        ]
        out = pl.pallas_call(
            kernel,
            in_specs=[pl.BlockSpec(memory_space=pl.ANY)] * 8,
            out_specs=pl.BlockSpec(memory_space=pl.ANY),
            out_shape=jax.ShapeDtypeStruct((S, D), BF16),
            scratch_shapes=scratch,
            compiler_params=pltpu.CompilerParams(vmem_limit_bytes=124 * 1024 * 1024, disable_bounds_checks=True,
                                                 disable_semaphore_checks=True),
        )(A_x.reshape(S, D), A_wqkv, A_wo, B_w1, B_w3, B_w2, c, w_mod)
        return out.reshape(1, S, D)

    return fn


_impl = make_kernel()


@jax.jit
def pallas_adaLN_cond__sliding_local_dilated__glu_gated_swiglu__prompt_kernel(A_x, A_wqkv, A_wo, B_x, B_w1, B_w3, B_w2, c, w_mod):
    return _impl(A_x, A_wqkv, A_wo, B_x, B_w1, B_w3, B_w2, c, w_mod)
```

```python
import contextlib
import functools
import math

import jax
import jax.numpy as jnp
import jax.experimental.pallas as pl
import jax.experimental.pallas.tpu as pltpu

S, D, F = 2048, 1024, 3584
DH, WIN, DIL = 32, 8, 2
NC = D // 128
PAD = 16
EPS = 1e-5
SCALE = DH ** -0.5
EXP2_C = SCALE * math.log2(math.e)
MASKED = -1e9 / SCALE
F32, BF16, U32 = jnp.float32, jnp.bfloat16, jnp.uint32
TM = 256
NT = S // TM
G = 16
NG = TM // G
HK = D // 2
SA = 2 * TM
SB = S - SA


def _xor_network(xs):
    lane = jax.lax.broadcasted_iota(jnp.int32, xs[0].shape, 1)
    for b in range(3):
        m = ((lane >> (2 + b)) & 1) == 1
        xs = [jnp.where(m, xs[i ^ (1 << b)], xs[i]) for i in range(NC)]
    return xs


def _gather_fwd(z, j):
    lane = jax.lax.broadcasted_iota(jnp.int32, z.shape, 1)
    e, g, p = lane >> 5, (lane >> 3) & 3, lane & 7
    return jnp.take_along_axis(z, g * 32 + (p ^ j) * 4 + e, axis=1)


def _gather_inv(y, j):
    lane = jax.lax.broadcasted_iota(jnp.int32, y.shape, 1)
    g, q, e = lane >> 5, (lane >> 2) & 7, lane & 3
    return jnp.take_along_axis(y, e * 32 + g * 8 + (q ^ j), axis=1)


def _pack(x):
    return pltpu.bitcast(x.astype(BF16), U32)


def _or_all(vs):
    parts = [v[r:r + 8, c:c + 128] for v in vs for r in range(0, v.shape[0], 8) for c in range(0, v.shape[1], 128)]
    while len(parts) > 1:
        parts = [parts[i] | parts[i + 1] if i + 1 < len(parts) else parts[i] for i in range(0, len(parts), 2)]
    return parts[0]


def _gate(x, g):
    if g is None:
        return x
    xb = x if x.dtype == U32 else pltpu.bitcast(x, U32)
    y = xb | jnp.tile(g, (x.shape[0] // 8, x.shape[1] // 128))
    return y if x.dtype == U32 else pltpu.bitcast(y, x.dtype)


def _rows(start, n, mult):
    if isinstance(start, int):
        return pl.ds(start, n)
    return pl.ds(pl.multiple_of(start, mult), n)


def _stats(x):
    mu = jnp.mean(x, axis=-1, keepdims=True)
    xc = x - mu
    var = jnp.mean(xc * xc, axis=-1, keepdims=True)
    return mu, xc, jax.lax.rsqrt(var + EPS)


def make_kernel(NREL=2, DL=4,
                W0=(4, 10, 3), WA=(9, 10, 7, 6, 6, 6, 6), WP=(2.5, 1, 0.25, 1, 2, 6), X2AT=6, T7L=(7, 14),
                AQ=(2, 4, 4), AA=(0, 42), AL=(1, 38), ADL=5, CPH=0.75,
                AFP=(18, 13, 34, 36, 58, 34, 60, 0, 34), AFDL=5,
                BW=2, BQ=(2, 2, 5), BA=(20, 170), BL=(21, 171), BCP=(176, 178), BDL=5,
                MG=1, AFN=4, AFL=(2, 3), AN=2, ALS=(0, 0), BN=2, BLS=(0, 0), TMG=2, TN=4, TLS=(1, 3), scopes=False, only=None):

    def scope(name):
        return jax.named_scope(name) if scopes else contextlib.nullcontext()

    def kernel(x_hbm, wqkv_hbm, wo_hbm, w1_hbm, w3_hbm, w2_hbm, c_hbm, wm_hbm, out_hbm,
               x_v, wraw_v, wp_v, wo_v, w1_v, w3_v, w2_v, wmc_v, wmr_v,
               mod_v, scol_v, st_v, h1_v, qa_v, ka_v, va_v, qb_v, kb_v, vb_v, o_v, x1_v, h2_v, out_v,
               hc_v, hn_v, z_v, c_v, sems, sem_out, bar):
        cp = pltpu.make_async_copy

        dmas = {}

        def add(name, src, dst):
            dmas[name] = cp(src, dst, sems.at[len(dmas)])

        def add_x(name, t0, n):
            add(name, x_hbm.at[pl.ds(t0 * TM, n * TM), :], x_v.at[pl.ds(t0 * TM, n * TM), :])

        add("c", c_hbm, c_v)
        add_x("x0", 0, 1)
        for k in range(NC):
            for m in (1, 0):
                add(f"m{m}{k}", wm_hbm.at[:, pl.ds(m * D + k * 128, 128)], wmc_v.at[m * NC + k])
            for m in range(3):
                add(f"w{m}{k}", wqkv_hbm.at[pl.ds(k * 128, 128), pl.ds(m * D, D)], wraw_v.at[m, pl.ds(k * 128, 128), :])
            if k == 0:
                add_x("x1", 1, 1)
            if k == X2AT:
                add_x("x2", 2, 1)
        add_x("xr", 3, NT - 3)
        add("wmr", wm_hbm.at[:, pl.ds(2 * D, 4 * D)], wmr_v)
        add("wo", wo_hbm, wo_v)
        add("fw1", w1_hbm, w1_v)
        add("fw3", w3_hbm, w3_v)
        add("fw2", w2_hbm, w2_v)
        for d in dmas.values():
            d.start()
            pl.semaphore_signal(bar, 1)
            pl.semaphore_wait(bar, 1)
        for j in range(NC):
            ka_v[j, 0:PAD, :] = jnp.zeros((PAD, 128), F32)
            va_v[j, 0:PAD, :] = jnp.zeros((PAD, 128), F32)
        add("z", ka_v.at[0, pl.ds(0, 8), :], z_v.at[pl.ds(0, 8), :])
        dmas["z"].start()

        def wait(*names):
            with scope("w_" + names[0]):
                for n in names:
                    dmas[n].wait()

        def zero():
            return pltpu.bitcast(z_v[0:8, :], U32)

        cur = {"nrel": NREL, "lns": (0, 0)}

        def mod_task(m, j, mg=2):
            src = wmc_v.at[m * NC + j] if m < 2 else wmr_v.at[:, pl.ds((m - 2) * D + j * 128, 128)]
            acc = None
            for kb in range(D // 128):
                if kb % mg == 0:
                    rel = yield
                p = src[kb * 128:(kb + 1) * 128, :].astype(F32) * scol_v[kb * 128:(kb + 1) * 128, :]
                parts = [p[r:r + 8] for r in range(0, 128, 8)]
                a0, a1 = parts[0], parts[1]
                if kb % mg == 0:
                    a0, a1 = _gate(a0, rel), _gate(a1, rel)
                for r in range(2, 16, 2):
                    a0, a1 = a0 + parts[r], a1 + parts[r + 1]
                a0 = a0 + a1
                acc = a0 if acc is None else acc + a0
            r = jnp.sum(acc, axis=0, keepdims=True)
            if m in (1, 4):
                r = r + 1.0
            mod_v[m:m + 1, j * 128:(j + 1) * 128] = r
            return pltpu.bitcast(jnp.broadcast_to(r, (8, 128)), U32)

        def modulate(xn, ms, dst, g, c0, c1):
            hb = _pack(xn * mod_v[ms + 1:ms + 2, c0:c1] + mod_v[ms:ms + 1, c0:c1])
            dst[g * 8:(g + 1) * 8, c0:c1] = hb
            return _or_all([hb])

        def ln_tail(xc, rs, ms, dst, g):
            ns, skip = cur["lns"]
            if ns == 0:
                return modulate(xc * rs, ms, dst, g, 0, D)
            for _ in range(skip):
                yield
            rs = jnp.broadcast_to(rs, (G, 128))
            toks = []
            cw = D // ns
            for p in range(ns):
                rel = yield
                r = jnp.tile(_gate(rs, rel), (1, cw // 128))
                toks.append(modulate(xc[:, p * cw:(p + 1) * cw] * r, ms, dst, g, p * cw, (p + 1) * cw))
            return _or_all(toks)

        def ln1_task(t, g, dst):
            rel = yield
            xt = x_v.at[_rows(t * TM, TM, TM), :]
            _, xc, rs = _stats(_gate(xt[g * G:(g + 1) * G, :].astype(F32), rel))
            return (yield from ln_tail(xc, rs, 0, dst, g))

        def stats_task(t, g):
            rel = yield
            rows = slice(t * TM + g * G, t * TM + (g + 1) * G)
            mu, _, rs = _stats(_gate(x_v[rows, :].astype(F32), rel))
            st_v[0, rows, :] = jnp.broadcast_to(mu, (G, 128))
            st_v[1, rows, :] = jnp.broadcast_to(rs, (G, 128))

        def fin_task(t, k, g0, ng):
            rel = yield
            for g in range(g0, g0 + ng):
                rows = slice(t * TM + g * G, t * TM + (g + 1) * G)
                x = _gate(x_v[rows, k * 128:(k + 1) * 128].astype(F32), rel)
                modulate((x - st_v[0, rows, :]) * st_v[1, rows, :], 0, h1_v.at[t], g, k * 128, (k + 1) * 128)

        def ln2_task(t, g, dst):
            rel = yield
            xv = x1_v.at[:, _rows(t * TM, TM, TM), :]
            x = jnp.concatenate([_gate(xv[j, g * G:(g + 1) * G, :], rel) for j in range(NC)], axis=1)
            _, xc, rs = _stats(x)
            return (yield from ln_tail(xc, rs, 3, dst, g))

        def perm_select_task(m, r0, n):
            rel = yield
            xs = [_gate(pltpu.bitcast(wraw_v[m, r0:r0 + n, j * 128:(j + 1) * 128], U32), rel) for j in range(NC)]
            zs = _xor_network(xs)
            for j in range(NC):
                wp_v[r0 // 2:(r0 + n) // 2, m * D + j * 128:m * D + (j + 1) * 128] = zs[j]

        def perm_gather_task(m, j, r0, n):
            rel = yield
            sl = (slice(r0 // 2, (r0 + n) // 2), slice(m * D + j * 128, m * D + (j + 1) * 128))
            wp_v[sl] = _gather_fwd(_gate(wp_v[sl], rel), j)

        def copy_task(src, dst, hf):
            rel = yield
            dst[:, hf * HK:(hf + 1) * HK] = _gate(src[:, hf * HK:(hf + 1) * HK], rel)

        def halo_task():
            yield
            for j in range(NC):
                kb_v[j, 0:PAD, :] = ka_v[j, SA:SA + PAD, :]
                vb_v[j, 0:PAD, :] = va_v[j, SA:SA + PAD, :]

        def attn_task(first, base, span, g, pace, masked=False):
            qkg, pvg, skip = pace
            q_v, k_v, v_v = (qa_v, ka_v, va_v) if first else (qb_v, kb_v, vb_v)
            qv = q_v.at[:, _rows(base, span, 32), :]
            kv = k_v.at[:, _rows(base, span + PAD, 32), :]
            vv = v_v.at[:, _rows(base, span + PAD, 32), :]

            def shifted(ref, j, w):
                return ref[j, pl.ds(g * G + PAD - DIL * w, G), :]

            q = [qv[j, g * G:(g + 1) * G, :] for j in range(NC)]
            ls = []
            for w in range(WIN):
                if w % qkg == 0:
                    rel = yield
                acc = _gate(q[0], rel) * shifted(kv, 0, w)
                for j in range(1, NC):
                    acc = acc + q[j] * shifted(kv, j, w)
                ls.append(acc)
            ls = [l + pltpu.roll(l, 64, 1) for l in ls]
            ls = [l + pltpu.roll(l, 32, 1) for l in ls]
            if masked:
                rows = base + g * G + jax.lax.broadcasted_iota(jnp.int32, (G, 128), 0)
                ls = [ls[0]] + [jnp.where(rows >= DIL * w, ls[w], MASKED) for w in range(1, WIN)]
            mx = ls[0]
            for w in range(1, WIN):
                mx = jnp.maximum(mx, ls[w])
            ps = [jnp.exp2((l - mx) * EXP2_C) for l in ls]
            den = ps[0]
            for w in range(1, WIN):
                den = den + ps[w]
            inv = 1.0 / den
            ps = [pw * inv for pw in ps]
            for _ in range(skip):
                rel = yield
            zs = []
            for j in range(NC):
                if j % pvg == 0:
                    rel = yield
                acc = _gate(ps[0], rel) * shifted(vv, j, 0)
                for w in range(1, WIN):
                    acc = acc + ps[w] * shifted(vv, j, w)
                zs.append(_gather_inv(_pack(acc), j))
            xs = _xor_network(zs)
            half = jax.lax.shift_right_logical(base, 1) + (0 if first else SA // 2)
            ov = o_v.at[_rows(half, span // 2, 16), :]
            for j in range(NC):
                ov[g * 8:(g + 1) * 8, j * 128:(j + 1) * 128] = xs[j]
            return _or_all(xs)

        def LN1(t, dst):
            return [ln1_task(t, g, dst) for g in range(NG)]

        def LN2(t, dst):
            return [ln2_task(t, g, dst) for g in range(NG)]

        def STATS(t):
            return [stats_task(t, g) for g in range(NG)]

        def FIN(t, k):
            return [fin_task(t, k, g0, 4) for g0 in range(0, NG, 4)]

        def MOD(m, j0=0, j1=NC, mg=2):
            return [mod_task(m, j, mg) for j in range(j0, j1)]

        def PERM(m, k):
            r0 = k * 128
            return ([perm_select_task(m, r, 32) for r in range(r0, r0 + 128, 32)]
                    + [perm_gather_task(m, j, r0, 128) for j in range(NC)])

        def COPY(src, dst, lo, hi, pre):
            return [([copy_task(src, dst, 0)], lo, lo + 1, pre), ([copy_task(src, dst, 1)], hi, hi + 1, pre)]

        def run_now(tasks):
            for tk in tasks:
                try:
                    next(tk)
                    while True:
                        tk.send(None)
                except StopIteration:
                    pass

        def tie(a, tok):
            if tok is not None:
                top = a[0:8, 0:128] | (tok & zero())
                if a.shape[1] > 128:
                    top = jnp.concatenate([top, a[0:8, 128:]], axis=1)
                a = jnp.concatenate([top, a[8:]], axis=0)
            return pltpu.bitcast(a, BF16)


        def releases(res):
            return [pltpu.bitcast(res[r:r + 8, 0:128], U32) & zero() for r in range(0, TM, TM // cur["nrel"])]

        def wave_pass(k, t, nb, tok):
            m, j0 = nb // 2, (nb % 2) * 4
            dst = (qa_v, ka_v, va_v)[m]
            rows = slice(t * TM + (PAD if m else 0), (t + 1) * TM + (PAD if m else 0))
            w = pltpu.bitcast(wp_v[k * 64:(k + 1) * 64, nb * 512:(nb + 1) * 512], BF16)
            res = jnp.dot(tie(h1_v[t, :, k * 128:(k + 1) * 128], tok), w, preferred_element_type=F32)
            for jj in range(4):
                r = res[:, jj * 128:(jj + 1) * 128]
                if k > 0:
                    r = dst[j0 + jj, rows, :] + r
                dst[j0 + jj, rows, :] = r
            return releases(res)

        def qkv_pass(t, m, j, hf, st, tok):
            w = pltpu.bitcast(wp_v[hf * HK // 2:(hf + 1) * HK // 2, m * D + j * 128:m * D + (j + 1) * 128], BF16)
            res = jnp.dot(tie(hc_v[:, hf * HK:(hf + 1) * HK], tok), w, preferred_element_type=F32)
            if hf == 0:
                st["a"] = res
            else:
                res = st.pop("a") + res
                off = PAD if m else 0
                dst = (qb_v, kb_v, vb_v)[m].at[:, _rows((t - 2) * TM, TM + off, TM), :]
                dst[j, off:off + TM, :] = res
            return releases(res)

        def wo_pass(t, j, hf, st, tok):
            h = tie(o_v[_rows(t * (TM // 2), TM // 2, TM // 2), hf * HK:(hf + 1) * HK], tok)
            res = jnp.dot(h, wo_v[hf * HK:(hf + 1) * HK, j * 128:(j + 1) * 128], preferred_element_type=F32)
            if hf == 0:
                st["a"] = res
            else:
                rows, cs = _rows(t * TM, TM, TM), slice(j * 128, (j + 1) * 128)
                res = x_v[rows, cs].astype(F32) + mod_v[2:3, cs] * (st.pop("a") + res)
                x1_v[j, rows, :] = res
            return releases(res)

        def out_copy(t, j):
            rows = _rows(t * TM, TM, TM)
            return cp(out_v.at[j, rows, :], out_hbm.at[rows, pl.ds(j * 128, 128)], sem_out.at[t])

        def out_wait(t):
            rows = pl.ds(t * TM, TM)
            cp(out_hbm.at[rows, :], out_hbm.at[rows, :], sem_out.at[t]).wait()

        def WAVE(k):
            return [functools.partial(wave_pass, k, t, nb) for m in range(3) for t in range(2) for nb in (2 * m, 2 * m + 1)]

        def QKV(t):
            st = {}
            return [functools.partial(qkv_pass, t, m, j, hf, st) for m in range(3) for j in range(NC) for hf in range(2)]

        def WO(t):
            st = {}
            return [functools.partial(wo_pass, t, j, hf, st) for j in range(NC) for hf in range(2)]

        def FFN(t):
            st = {"acc": [None] * NC, "act": []}

            def gate_up_pass(which, n, hf, tok):
                w = (w1_v, w3_v)[which][hf * HK:(hf + 1) * HK, n * 128:(n + 1) * 128]
                res = jnp.dot(tie(h2_v[:, hf * HK:(hf + 1) * HK], tok), w, preferred_element_type=F32)
                if hf == 0:
                    st["a"] = res
                else:
                    res = st.pop("a") + res
                    if which == 0:
                        hg = 0.5 * res
                        st["g"] = hg + hg * jnp.tanh(hg)
                    else:
                        st["act"].append((st.pop("g") * res).astype(BF16))
                return releases(res)

            def down_pass(c, j, last, tok):
                if j == 0:
                    st["lhs"], st["act"] = jnp.concatenate(st["act"], axis=1), []
                w = w2_v[c * HK:(c + 1) * HK, j * 128:(j + 1) * 128]
                if tok is not None:
                    w = tie(pltpu.bitcast(w, U32), tok)
                res = jnp.dot(st["lhs"], w, preferred_element_type=F32)
                if st["acc"][j] is not None:
                    res = st["acc"][j] + res
                st["acc"][j] = res
                if last:
                    rows = _rows(t * TM, TM, TM)
                    out_v[j, rows, :] = (x1_v[j, rows, :] + mod_v[5:6, j * 128:(j + 1) * 128] * res).astype(BF16)
                    out_copy(t, j).start()
                return releases(res)

            out = []
            nch = F // HK
            for c in range(nch):
                for n in range(c * 4, c * 4 + 4):
                    out += [functools.partial(gate_up_pass, which, n, hf) for which in range(2) for hf in range(2)]
                out += [functools.partial(down_pass, c, j, c == nch - 1) for j in range(NC)]
            return out

        def segment(name, passes, groups=(), dl=DL, need=None, nrel=NREL, lns=(0, 0)):
            if only is not None and name not in only:
                return
            with scope(name):
                n = len(passes)
                cur["nrel"], cur["lns"] = nrel, lns
                active = []
                for tasks, lo, hi, *pre in groups:
                    for k, tk in enumerate(tasks):
                        active.append((int((lo + k * (hi - lo) / len(tasks)) * nrel), tk, pre[0] if pre else ()))
                        next(tk)
                deadlines = [[] for _ in range(n + dl + 1)]

                def done(tasks):
                    return all(ent[1] is not tk for tk in tasks for ent in active)

                def feed(rel, slot, i):
                    for ent in list(active):
                        if ent[0] <= slot:
                            assert done(ent[2]), (name, i)
                            try:
                                ent[1].send(rel)
                            except StopIteration as e:
                                if e.value is not None:
                                    deadlines[i + dl].append(e.value)
                                active.remove(ent)

                feed(None, 0, 0)
                slot = 1
                for i, ps in enumerate(passes):
                    assert done((need or {}).get(i, ())), (name, i)
                    for rel in ps(_or_all(deadlines[i]) if deadlines[i] else None):
                        feed(rel, slot, i)
                        slot += 1
                while active:
                    feed(None, 1 << 30, n)

        with scope("S0"):
            wait("c", "z")
            c = c_v[...].astype(F32)
            s = (c * jax.nn.sigmoid(c)).astype(BF16).astype(F32)
            eye = (jax.lax.broadcasted_iota(jnp.int32, (128, 128), 0)
                   == jax.lax.broadcasted_iota(jnp.int32, (128, 128), 1))
            ones = jnp.ones((128, 128), BF16)
            for j in range(NC):
                dg = jnp.where(eye, jnp.broadcast_to(s[:, j * 128:(j + 1) * 128], (128, 128)), 0.0).astype(BF16)
                scol_v[j * 128:(j + 1) * 128, :] = jnp.dot(dg, ones, preferred_element_type=F32)
            wait("x0")
            run_now(STATS(0))
            wait("m10", "m00")
            run_now(MOD(1, 0, 1) + MOD(0, 0, 1) + FIN(0, 0))
            wait("w00")
            run_now(PERM(0, 0))
            wait("w10", "w20")

        m0 = [functools.partial(wave_pass, 0, t, nb) for t in range(2) for nb in range(6)]
        m1 = WAVE(1)
        n0, n1, n2 = W0
        p1, p2 = PERM(1, 0), PERM(2, 0)
        segment("T0a", m0[:n0], [(p1, 0, 1), (p2, 1, n0 - 0.5)], need={2: p1})
        wait("x1")
        s1, f1, u = STATS(1), FIN(1, 0), 6 - n0
        segment("T0b", m0[n0:n1], [(s1, 0, max(0.4, u - 1)), (f1, u - 0.5 if u < 3 else u - 1, u - 0.4, s1)], need={u: s1 + f1})
        wait("m11", "m01", "w01")
        mods, f0, f1, pq, u = MOD(1, 1, 2) + MOD(0, 1, 2), FIN(0, 1), FIN(1, 1), PERM(0, 1), 12 - n1
        segment("T0c", m0[n1:] + m1[:n2],
                [(mods, 0, 0.4), (f0, max(1.5, u - 1), max(1.5, u - 1) + 0.4, mods), (f1, u - 0.5, u + 0.5, mods), (pq, 0, u - 1)],
                need={u: mods + f0 + pq, u + 2: f1})
        wait("w11", "w21")
        p1, p2 = PERM(1, 1), PERM(2, 1)
        segment("T1", m1[n2:WA[1]], [(p1, 0, 3 - n2), (p2, 3 - n2, 6.5 - n2)], need={4 - n2: p1, 8 - n2: p2})
        for k in range(2, NC):
            last = k == NC - 1
            wait(f"m1{k}", f"m0{k}", f"w0{k}", f"w1{k}", f"w2{k}", *(["x2"] if last else []))
            u = 12 - WA[k - 1]
            mods = MOD(1, k, k + 1, TMG) + MOD(0, k, k + 1, TMG)
            fins = [FIN(t, k) for t in range(2)]
            perms = [PERM(m, k) for m in range(3)]
            mend = max(0.5, u - WP[0])
            fmin = (8 // TMG - 1) / TN + (mend - 0.5 if mend > 2 else 0)
            groups = [(mods[:1], 0, 1), (mods[1:], mend - 0.5 if mend > 2 else 0, mend),
                      (fins[0], max(fmin, u - WP[1]), max(fmin + 0.2, u - WP[2]), mods), (fins[1], max(fmin + 0.2, u - WP[2]), u + 1, mods),
                      (perms[0], 0, max(0.9, u - WP[3])), (perms[1], max(0.9, u - WP[3]), u + WP[4]), (perms[2], u + WP[4], u + WP[5])]
            if last:
                groups.append((LN1(2, hc_v), *T7L))
            segment(f"T{k}", WAVE(k - 1)[WA[k - 1]:] + (WAVE(k) if last else WAVE(k)[:WA[k]]), groups,
                    need={u: mods + fins[0] + perms[0], u + 2: fins[1], u + 4: perms[1], u + 8: perms[2]}, nrel=TN, lns=TLS)
        wait("xr")

        def a_step(npc, p0, t0, t, carry):
            base = jnp.minimum(p0 // 2 + (t - t0) * (npc // 2), NG - npc // 2) * (2 * G)
            att = [attn_task(True, base, npc * G, g, AQ, masked=(p0 == 0 and g == 0)) for g in range(npc)]
            l1 = LN1(jnp.minimum(t + 1, NT - 1), hn_v)
            segment("A", QKV(t), [(att, *AA), (l1, *AL)] + COPY(hn_v, hc_v, 47, 47 + CPH, l1), dl=ADL, nrel=AN, lns=ALS)
            return carry

        with scope("loopA1"):
            jax.lax.fori_loop(2, 4, functools.partial(a_step, 8, 0, 2), 0)
        wait("wmr", "wo")
        q4, nq = QKV(4), AFP[0]
        l1, mg, msc = LN1(5, hn_v), MOD(2, mg=MG), MOD(3, mg=MG) + MOD(4, mg=MG)
        segment("AF", q4[:nq] + WO(0) + q4[nq:],
                [(mg, 0, AFP[1]), (msc, AFP[1], AFP[2]), (LN2(0, h2_v), max(AFP[3], nq + 16), AFP[4], msc),
                 (MOD(5, mg=MG), AFP[5], AFP[6]), (l1, AFP[7], AFP[8]), ([halo_task()], 1, 2)]
                + COPY(hn_v, hc_v, 63, 63 + CPH, l1), need={nq: mg}, dl=AFDL, nrel=AFN, lns=AFL)
        with scope("loopA2"):
            jax.lax.fori_loop(5, NT, functools.partial(a_step, 6, 16, 5), 0)
        wait("fw1", "fw3", "fw2")

        def b_step(i, carry):
            att = [attn_task(False, jnp.minimum(i, NT - 3) * TM, TM, g, BQ) for g in range(NG)]
            l2 = LN2(i + 1, hn_v)
            assert BA[0] >= 16 + BW and BL[0] >= 16 + BW and min(BCP) >= 176
            ffn = FFN(i)
            segment("F", ffn[:BW] + WO(i + 1) + ffn[BW:], [(att, *BA), (l2, *BL)] + COPY(hn_v, h2_v, *BCP, l2), dl=BDL, nrel=BN, lns=BLS)
            return carry

        with scope("B"):
            jax.lax.fori_loop(0, NT - 1, b_step, 0)
        for t in range(NT - 2):
            out_wait(t)
        segment("FL", FFN(NT - 1))
        with scope("fin"):
            for t in range(NT - 2, NT):
                out_wait(t)

    @jax.jit
    def fn(A_x, A_wqkv, A_wo, B_x, B_w1, B_w3, B_w2, c, w_mod):
        V = pltpu.VMEM
        scratch = [
            V((S, D), BF16), V((3, D, D), BF16), V((D // 2, 3 * D), U32), V((D, D), BF16),
            V((D, F), BF16), V((D, F), BF16), V((F, D), BF16), V((2 * NC, D, 128), BF16), V((D, 4 * D), BF16),
            V((8, D), F32), V((D, 128), F32), V((2, SA, 128), F32), V((2, TM // 2, D), U32),
            V((NC, SA, 128), F32), V((NC, PAD + SA, 128), F32), V((NC, PAD + SA, 128), F32),
            V((NC, SB, 128), F32), V((NC, PAD + SB, 128), F32), V((NC, PAD + SB, 128), F32),
            V((S // 2, D), U32), V((NC, S, 128), F32), V((TM // 2, D), U32), V((NC, S, 128), BF16),
            V((TM // 2, D), U32), V((TM // 2, D), U32), V((32, 128), F32), V((1, D), BF16),
            pltpu.SemaphoreType.DMA((5 * NC + 11,)), pltpu.SemaphoreType.DMA((NT,)), pltpu.SemaphoreType.REGULAR,
        ]
        out = pl.pallas_call(
            kernel,
            in_specs=[pl.BlockSpec(memory_space=pl.ANY)] * 8,
            out_specs=pl.BlockSpec(memory_space=pl.ANY),
            out_shape=jax.ShapeDtypeStruct((S, D), BF16),
            scratch_shapes=scratch,
            compiler_params=pltpu.CompilerParams(vmem_limit_bytes=124 * 1024 * 1024, disable_bounds_checks=True,
                                                 disable_semaphore_checks=True),
        )(A_x.reshape(S, D), A_wqkv, A_wo, B_w1, B_w3, B_w2, c, w_mod)
        return out.reshape(1, S, D)

    return fn


_impl = make_kernel()


@jax.jit
def pallas_adaLN_cond__sliding_local_dilated__glu_gated_swiglu__prompt_kernel(A_x, A_wqkv, A_wo, B_x, B_w1, B_w3, B_w2, c, w_mod):
    return _impl(A_x, A_wqkv, A_wo, B_x, B_w1, B_w3, B_w2, c, w_mod)
```

```python
import contextlib
import functools
import math

import jax
import jax.numpy as jnp
import jax.experimental.pallas as pl
import jax.experimental.pallas.tpu as pltpu

S, D, F = 2048, 1024, 3584
DH, WIN, DIL = 32, 8, 2
NC = D // 128
PAD = 16
EPS = 1e-5
SCALE = DH ** -0.5
EXP2_C = SCALE * math.log2(math.e)
MASKED = -1e9 / SCALE
F32, BF16, U32 = jnp.float32, jnp.bfloat16, jnp.uint32
TM = 256
NT = S // TM
G = 16
NG = TM // G
HK = D // 2
SA = 2 * TM
SB = S - SA


def _xor_network(xs):
    lane = jax.lax.broadcasted_iota(jnp.int32, xs[0].shape, 1)
    for b in range(3):
        m = ((lane >> (2 + b)) & 1) == 1
        xs = [jnp.where(m, xs[i ^ (1 << b)], xs[i]) for i in range(NC)]
    return xs


def _gather_fwd(z, j):
    lane = jax.lax.broadcasted_iota(jnp.int32, z.shape, 1)
    e, g, p = lane >> 5, (lane >> 3) & 3, lane & 7
    return jnp.take_along_axis(z, g * 32 + (p ^ j) * 4 + e, axis=1)


def _gather_inv(y, j):
    lane = jax.lax.broadcasted_iota(jnp.int32, y.shape, 1)
    g, q, e = lane >> 5, (lane >> 2) & 7, lane & 3
    return jnp.take_along_axis(y, e * 32 + g * 8 + (q ^ j), axis=1)


def _pack(x):
    return pltpu.bitcast(x.astype(BF16), U32)


def _or_all(vs):
    parts = [v[r:r + 8, c:c + 128] for v in vs for r in range(0, v.shape[0], 8) for c in range(0, v.shape[1], 128)]
    while len(parts) > 1:
        parts = [parts[i] | parts[i + 1] if i + 1 < len(parts) else parts[i] for i in range(0, len(parts), 2)]
    return parts[0]


def _gate(x, g):
    if g is None:
        return x
    xb = x if x.dtype == U32 else pltpu.bitcast(x, U32)
    y = xb | jnp.tile(g, (x.shape[0] // 8, x.shape[1] // 128))
    return y if x.dtype == U32 else pltpu.bitcast(y, x.dtype)


def _rows(start, n, mult):
    if isinstance(start, int):
        return pl.ds(start, n)
    return pl.ds(pl.multiple_of(start, mult), n)


def _stats(x):
    mu = jnp.mean(x, axis=-1, keepdims=True)
    xc = x - mu
    var = jnp.mean(xc * xc, axis=-1, keepdims=True)
    return mu, xc, jax.lax.rsqrt(var + EPS)


def make_kernel(NREL=2, DL=4,
                W0=(4, 10, 3), WA=(9, 10, 7, 6, 6, 6, 6), WP=(2.5, 1, 0.25, 1, 2, 6), X2AT=6, T7L=(5, 13),
                AQ=(2, 1, 9, 3), AA=(1, 40), AL=(2, 38), ADL=4,
                NOV=0, DSH=1, QKJ=True, PVW=2, C0=1, NPC=6, AFQ=(1, 1, 12, 3), AFP=(20, 15, 36, 38, 58, 60, 84, 0, 16), AFDL=5,
                BW=2, BQ=(1, 1, 20, 5), BA=(18, 170), BL=(20, 149), BCP=(8, 28), AFC=(66, 86), QT=4, ACN=(8, 4), BDL=6,
                MG=1, AFN=4, AFL=(0, 0), AN=4, ALS=(2, 4), BN=4, BLS=(2, 4), TMG=2, TN=4, TLS=(1, 3), scopes=False, only=None):

    def scope(name):
        return jax.named_scope(name) if scopes else contextlib.nullcontext()

    def kernel(x_hbm, wqkv_hbm, wo_hbm, w1_hbm, w3_hbm, w2_hbm, c_hbm, wm_hbm, out_hbm,
               x_v, wraw_v, wp_v, wo_v, w1_v, w3_v, w2_v, wmc_v, wmr_v,
               mod_v, scol_v, st_v, h1_v, qa_v, ka_v, va_v, qb_v, kb_v, vb_v, o_v, x1_v, h2_v, out_v,
               hc_v, hn_v, acc_v, z_v, c_v, sems, sem_out, bar):
        cp = pltpu.make_async_copy

        dmas = {}

        def add(name, src, dst):
            dmas[name] = cp(src, dst, sems.at[len(dmas)])

        def add_x(name, t0, n):
            add(name, x_hbm.at[pl.ds(t0 * TM, n * TM), :], x_v.at[pl.ds(t0 * TM, n * TM), :])

        add("c", c_hbm, c_v)
        add_x("x0", 0, 1)
        for k in range(NC):
            for m in (1, 0):
                add(f"m{m}{k}", wm_hbm.at[:, pl.ds(m * D + k * 128, 128)], wmc_v.at[m * NC + k])
            for m in range(3):
                add(f"w{m}{k}", wqkv_hbm.at[pl.ds(k * 128, 128), pl.ds(m * D, D)], wraw_v.at[m, pl.ds(k * 128, 128), :])
            if k == 0:
                add_x("x1", 1, 1)
            if k == X2AT:
                add_x("x2", 2, 1)
        add_x("xr", 3, NT - 3)
        add("wmr", wm_hbm.at[:, pl.ds(2 * D, 4 * D)], wmr_v)
        add("wo", wo_hbm, wo_v)
        add("fw1", w1_hbm, w1_v)
        add("fw3", w3_hbm, w3_v)
        add("fw2a", w2_hbm.at[pl.ds(0, C0 * HK), :], w2_v.at[pl.ds(0, C0 * HK), :])
        add("fw2b", w2_hbm.at[pl.ds(C0 * HK, F - C0 * HK), :], w2_v.at[pl.ds(C0 * HK, F - C0 * HK), :])
        for d in dmas.values():
            d.start()
            pl.semaphore_signal(bar, 1)
            pl.semaphore_wait(bar, 1)
        for j in range(NC):
            ka_v[j, 0:PAD, :] = jnp.zeros((PAD, 128), F32)
            va_v[j, 0:PAD, :] = jnp.zeros((PAD, 128), F32)
        add("z", ka_v.at[0, pl.ds(0, 8), :], z_v.at[pl.ds(0, 8), :])
        dmas["z"].start()

        def wait(*names):
            with scope("w_" + names[0]):
                for n in names:
                    dmas[n].wait()

        def zero():
            return pltpu.bitcast(z_v[0:8, :], U32)

        cur = {"nrel": NREL, "lns": (0, 0)}

        def mod_task(m, j, mg=2):
            src = wmc_v.at[m * NC + j] if m < 2 else wmr_v.at[:, pl.ds((m - 2) * D + j * 128, 128)]
            acc = None
            for kb in range(D // 128):
                if kb % mg == 0:
                    rel = yield
                p = src[kb * 128:(kb + 1) * 128, :].astype(F32) * scol_v[kb * 128:(kb + 1) * 128, :]
                parts = [p[r:r + 8] for r in range(0, 128, 8)]
                a0, a1 = parts[0], parts[1]
                if kb % mg == 0:
                    a0, a1 = _gate(a0, rel), _gate(a1, rel)
                for r in range(2, 16, 2):
                    a0, a1 = a0 + parts[r], a1 + parts[r + 1]
                a0 = a0 + a1
                acc = a0 if acc is None else acc + a0
            r = jnp.sum(acc, axis=0, keepdims=True)
            if m in (1, 4):
                r = r + 1.0
            mod_v[m:m + 1, j * 128:(j + 1) * 128] = r
            return pltpu.bitcast(jnp.broadcast_to(r, (8, 128)), U32)

        def modulate(xn, ms, dst, g, c0, c1):
            hb = _pack(xn * mod_v[ms + 1:ms + 2, c0:c1] + mod_v[ms:ms + 1, c0:c1])
            dst[g * 8:(g + 1) * 8, c0:c1] = hb
            return _or_all([hb])

        def ln_tail(xc, rs, ms, dst, g):
            ns, skip = cur["lns"]
            if ns == 0:
                return modulate(xc * rs, ms, dst, g, 0, D)
            for _ in range(skip):
                yield
            rs = jnp.broadcast_to(rs, (G, 128))
            toks = []
            cw = D // ns
            for p in range(ns):
                rel = yield
                r = jnp.tile(_gate(rs, rel), (1, cw // 128))
                toks.append(modulate(xc[:, p * cw:(p + 1) * cw] * r, ms, dst, g, p * cw, (p + 1) * cw))
            return _or_all(toks)

        def ln1_task(t, g, dst):
            rel = yield
            xt = x_v.at[_rows(t * TM, TM, TM), :]
            _, xc, rs = _stats(_gate(xt[g * G:(g + 1) * G, :].astype(F32), rel))
            return (yield from ln_tail(xc, rs, 0, dst, g))

        def stats_task(t, g):
            rel = yield
            rows = slice(t * TM + g * G, t * TM + (g + 1) * G)
            mu, _, rs = _stats(_gate(x_v[rows, :].astype(F32), rel))
            st_v[0, rows, :] = jnp.broadcast_to(mu, (G, 128))
            st_v[1, rows, :] = jnp.broadcast_to(rs, (G, 128))

        def fin_task(t, k, g0, ng):
            rel = yield
            for g in range(g0, g0 + ng):
                rows = slice(t * TM + g * G, t * TM + (g + 1) * G)
                x = _gate(x_v[rows, k * 128:(k + 1) * 128].astype(F32), rel)
                modulate((x - st_v[0, rows, :]) * st_v[1, rows, :], 0, h1_v.at[t], g, k * 128, (k + 1) * 128)

        def ln2_task(t, g, dst):
            rel = yield
            xv = x1_v.at[:, _rows(t * TM, TM, TM), :]
            x = jnp.concatenate([_gate(xv[j, g * G:(g + 1) * G, :], rel) for j in range(NC)], axis=1)
            _, xc, rs = _stats(x)
            return (yield from ln_tail(xc, rs, 3, dst, g))

        def perm_select_task(m, r0, n):
            rel = yield
            xs = [_gate(pltpu.bitcast(wraw_v[m, r0:r0 + n, j * 128:(j + 1) * 128], U32), rel) for j in range(NC)]
            zs = _xor_network(xs)
            for j in range(NC):
                wp_v[r0 // 2:(r0 + n) // 2, m * D + j * 128:m * D + (j + 1) * 128] = zs[j]

        def perm_gather_task(m, j, r0, n):
            rel = yield
            sl = (slice(r0 // 2, (r0 + n) // 2), slice(m * D + j * 128, m * D + (j + 1) * 128))
            wp_v[sl] = _gather_fwd(_gate(wp_v[sl], rel), j)

        def copy_task(src, dst, r0, nr, c0, c1):
            rel = yield
            dst[r0:r0 + nr, c0:c1] = _gate(src[r0:r0 + nr, c0:c1], rel)

        def halo_task():
            yield
            for j in range(NC):
                kb_v[j, 0:PAD, :] = ka_v[j, SA:SA + PAD, :]
                vb_v[j, 0:PAD, :] = va_v[j, SA:SA + PAD, :]

        def attn_task(first, base, span, g, pace, masked=False):
            qkg, pvg, skip, smd = pace
            q_v, k_v, v_v = (qa_v, ka_v, va_v) if first else (qb_v, kb_v, vb_v)
            qv = q_v.at[:, _rows(base, span, 32), :]
            kv = k_v.at[:, _rows(base, span + PAD, 32), :]
            vv = v_v.at[:, _rows(base, span + PAD, 32), :]

            def shifted(ref, j, w):
                return ref[j, pl.ds(g * G + PAD - DIL * w, G), :]

            if QKJ:
                ls = [None] * WIN
                for j in range(NC):
                    if j % qkg == 0:
                        rel = yield
                    q = _gate(qv[j, g * G:(g + 1) * G, :], rel)
                    for w in range(WIN):
                        p = q * shifted(kv, j, w)
                        ls[w] = p if j == 0 else ls[w] + p
            else:
                q = [qv[j, g * G:(g + 1) * G, :] for j in range(NC)]
                ls = []
                for w in range(WIN):
                    if w % qkg == 0:
                        rel = yield
                    acc = _gate(q[0], rel) * shifted(kv, 0, w)
                    for j in range(1, NC):
                        acc = acc + q[j] * shifted(kv, j, w)
                    ls.append(acc)
            ls = [l + pltpu.roll(l, 64, 1) for l in ls]
            ls = [l + pltpu.roll(l, 32, 1) for l in ls]
            if masked:
                rows = base + g * G + jax.lax.broadcasted_iota(jnp.int32, (G, 128), 0)
                ls = [ls[0]] + [jnp.where(rows >= DIL * w, ls[w], MASKED) for w in range(1, WIN)]
            mx = ls[0]
            for w in range(1, WIN):
                mx = jnp.maximum(mx, ls[w])
            ps = [jnp.exp2((l - mx) * EXP2_C) for l in ls]
            den = ps[0]
            for w in range(1, WIN):
                den = den + ps[w]
            inv = 1.0 / den
            ps = [pw * inv for pw in ps]
            if smd:
                yield _or_all([pltpu.bitcast(ps[0], U32)]), smd
            for _ in range(skip - (1 if smd else 0)):
                yield
            zs = []
            if PVW == 1:
                os_ = [None] * NC
                for w in range(WIN):
                    if w % pvg == 0:
                        rel = yield
                    p = _gate(ps[w], rel)
                    for j in range(NC):
                        pv = p * shifted(vv, j, w)
                        os_[j] = pv if w == 0 else os_[j] + pv
                for j in range(NC):
                    if j % 4 == 0:
                        rel = yield
                    zs.append(_gather_inv(_pack(_gate(os_[j], rel)), j))
            else:
                for j in range(NC):
                    if j % pvg == 0:
                        rel = yield
                        pg = [_gate(p, rel) for p in ps] if PVW == 2 else [_gate(ps[0], rel)] + ps[1:]
                    acc = pg[0] * shifted(vv, j, 0)
                    for w in range(1, WIN):
                        acc = acc + pg[w] * shifted(vv, j, w)
                    zs.append(_gather_inv(_pack(acc), j))
            xs = _xor_network(zs)
            half = (base // 2 if isinstance(base, int) else jax.lax.shift_right_logical(base, 1)) + (0 if first else SA // 2)
            ov = o_v.at[_rows(half, span // 2, 16), :]
            for j in range(NC):
                ov[g * 8:(g + 1) * 8, j * 128:(j + 1) * 128] = xs[j]
            return _or_all(xs)

        def LN1(t, dst):
            return [ln1_task(t, g, dst) for g in range(NG)]

        def LN2(t, dst):
            return [ln2_task(t, g, dst) for g in range(NG)]

        def STATS(t):
            return [stats_task(t, g) for g in range(NG)]

        def FIN(t, k):
            return [fin_task(t, k, g0, 4) for g0 in range(0, NG, 4)]

        def MOD(m, j0=0, j1=NC, mg=2):
            return [mod_task(m, j, mg) for j in range(j0, j1)]

        def PERM(m, k):
            r0 = k * 128
            return ([perm_select_task(m, r, 32) for r in range(r0, r0 + 128, 32)]
                    + [perm_gather_task(m, j, r0, 128) for j in range(NC)])

        def COPY(src, dst, n, lo, hi, pre, c0=0, c1=D):
            nr = TM // 2 // n
            return ([copy_task(src, dst, r, nr, c0, c1) for r in range(0, TM // 2, nr)], lo, hi, pre)

        def run_now(tasks):
            for tk in tasks:
                try:
                    next(tk)
                    while True:
                        tk.send(None)
                except StopIteration:
                    pass

        def tie(a, tok):
            if tok is not None:
                top = a[0:8, 0:128] | (tok & zero())
                if a.shape[1] > 128:
                    top = jnp.concatenate([top, a[0:8, 128:]], axis=1)
                a = jnp.concatenate([top, a[8:]], axis=0)
            return pltpu.bitcast(a, BF16)


        def releases(res):
            return [pltpu.bitcast(res[r:r + 8, 0:128], U32) & zero() for r in range(0, TM, TM // cur["nrel"])]

        def wave_pass(k, t, nb, tok):
            m, j0 = nb // 2, (nb % 2) * 4
            dst = (qa_v, ka_v, va_v)[m]
            rows = slice(t * TM + (PAD if m else 0), (t + 1) * TM + (PAD if m else 0))
            w = pltpu.bitcast(wp_v[k * 64:(k + 1) * 64, nb * 512:(nb + 1) * 512], BF16)
            res = jnp.dot(tie(h1_v[t, :, k * 128:(k + 1) * 128], tok), w, preferred_element_type=F32)
            for jj in range(4):
                r = res[:, jj * 128:(jj + 1) * 128]
                if k > 0:
                    r = dst[j0 + jj, rows, :] + r
                dst[j0 + jj, rows, :] = r
            return releases(res)

        def qkv_pass(t, m, j, hf, st, tok):
            w = pltpu.bitcast(wp_v[hf * HK // 2:(hf + 1) * HK // 2, m * D + j * 128:m * D + (j + 1) * 128], BF16)
            res = jnp.dot(tie(hc_v[:, hf * HK:(hf + 1) * HK], tok), w, preferred_element_type=F32)
            if hf == 0:
                st[m, j] = res
            else:
                res = st.pop((m, j)) + res
                off = PAD if m else 0
                dst = (qb_v, kb_v, vb_v)[m].at[:, _rows((t - 2) * TM, TM + off, TM), :]
                dst[j, off:off + TM, :] = res
            return releases(res)

        def wo_pass(t, j, hf, st, tok):
            h = tie(o_v[_rows(t * (TM // 2), TM // 2, TM // 2), hf * HK:(hf + 1) * HK], tok)
            res = jnp.dot(h, wo_v[hf * HK:(hf + 1) * HK, j * 128:(j + 1) * 128], preferred_element_type=F32)
            if hf == 0:
                st["a"] = res
            else:
                rows, cs = _rows(t * TM, TM, TM), slice(j * 128, (j + 1) * 128)
                res = x_v[rows, cs].astype(F32) + mod_v[2:3, cs] * (st.pop("a") + res)
                x1_v[j, rows, :] = res
            return releases(res)

        def out_copy(t, j):
            rows = _rows(t * TM, TM, TM)
            return cp(out_v.at[j, rows, :], out_hbm.at[rows, pl.ds(j * 128, 128)], sem_out.at[t])

        def out_wait(t):
            rows = pl.ds(t * TM, TM)
            cp(out_hbm.at[rows, :], out_hbm.at[rows, :], sem_out.at[t]).wait()

        def WAVE(k):
            return [functools.partial(wave_pass, k, t, nb) for m in range(3) for t in range(2) for nb in (2 * m, 2 * m + 1)]

        def QKV(t):
            order = [(m, j, hf) for m in range(3) for j in range(NC) for hf in range(2)]
            order = order[:-2 * QT] + order[-2 * QT::2] + order[-2 * QT + 1::2]
            st = {}
            return [functools.partial(qkv_pass, t, m, j, hf, st) for m, j, hf in order]

        def WO(t):
            st = {}
            return [functools.partial(wo_pass, t, j, hf, st) for j in range(NC) for hf in range(2)]

        def FFN(t, c0, c1):
            st = {"acc": [None] * NC, "act": []}
            h_v = hn_v if c0 == 0 else h2_v

            def gate_up_pass(which, n, hf, tok):
                w = (w1_v, w3_v)[which][hf * HK:(hf + 1) * HK, n * 128:(n + 1) * 128]
                res = jnp.dot(tie(h_v[:, hf * HK:(hf + 1) * HK], tok), w, preferred_element_type=F32)
                if hf == 0:
                    st["a"] = res
                else:
                    res = st.pop("a") + res
                    if which == 0:
                        hg = 0.5 * res
                        st["g"] = hg + hg * jnp.tanh(hg)
                    else:
                        st["act"].append((st.pop("g") * res).astype(BF16))
                return releases(res)

            def down_pass(c, j, last, tok):
                if j == 0:
                    st["lhs"], st["act"] = jnp.concatenate(st["act"], axis=1), []
                w = w2_v[c * HK:(c + 1) * HK, j * 128:(j + 1) * 128]
                if tok is not None:
                    w = tie(pltpu.bitcast(w, U32), tok)
                res = jnp.dot(st["lhs"], w, preferred_element_type=F32)
                if c > 0:
                    res = (acc_v[j] if c == c0 else st["acc"][j]) + res
                st["acc"][j] = res
                if c == c1 - 1 and not last:
                    acc_v[j] = res
                if last:
                    rows = _rows(t * TM, TM, TM)
                    out_v[j, rows, :] = (x1_v[j, rows, :] + mod_v[5:6, j * 128:(j + 1) * 128] * res).astype(BF16)
                    out_copy(t, j).start()
                return releases(res)

            out = []
            nch = F // HK
            for c in range(c0, c1):
                for n in range(c * 4, c * 4 + 4):
                    out += [functools.partial(gate_up_pass, which, n, hf) for which in range(2) for hf in range(2)]
                out += [functools.partial(down_pass, c, j, c == nch - 1) for j in range(NC)]
            return out

        def segment(name, passes, groups=(), dl=DL, need=None, nrel=NREL, lns=(0, 0)):
            if only is not None and name not in only:
                return
            with scope(name):
                n = len(passes)
                cur["nrel"], cur["lns"] = nrel, lns
                active = []
                for tasks, lo, hi, *pre in groups:
                    for k, tk in enumerate(tasks):
                        active.append((int((lo + k * (hi - lo) / len(tasks)) * nrel), tk, pre[0] if pre else ()))
                        next(tk)
                deadlines = [[] for _ in range(n + dl + 8)]

                def due(p):
                    return p + DSH if p < n and passes[p].func.__name__ == "down_pass" else p

                def done(tasks):
                    return all(ent[1] is not tk for tk in tasks for ent in active)

                def feed(rel, slot, i):
                    for ent in list(active):
                        if ent[0] <= slot:
                            assert done(ent[2]), (name, i)
                            try:
                                mid = ent[1].send(rel)
                                if mid is not None:
                                    deadlines[due(i + mid[1])].append(mid[0])
                            except StopIteration as e:
                                if e.value is not None:
                                    deadlines[due(i + dl)].append(e.value)
                                active.remove(ent)

                feed(None, 0, 0)
                slot = 1
                for i, ps in enumerate(passes):
                    assert done((need or {}).get(i, ())), (name, i)
                    for rel in ps(_or_all(deadlines[i]) if deadlines[i] else None):
                        feed(rel, slot, i)
                        slot += 1
                while active:
                    feed(None, 1 << 30, n)

        with scope("S0"):
            wait("c", "z")
            c = c_v[...].astype(F32)
            s = (c * jax.nn.sigmoid(c)).astype(BF16).astype(F32)
            eye = (jax.lax.broadcasted_iota(jnp.int32, (128, 128), 0)
                   == jax.lax.broadcasted_iota(jnp.int32, (128, 128), 1))
            ones = jnp.ones((128, 128), BF16)
            for j in range(NC):
                dg = jnp.where(eye, jnp.broadcast_to(s[:, j * 128:(j + 1) * 128], (128, 128)), 0.0).astype(BF16)
                scol_v[j * 128:(j + 1) * 128, :] = jnp.dot(dg, ones, preferred_element_type=F32)
            wait("x0")
            run_now(STATS(0))
            wait("m10", "m00")
            run_now(MOD(1, 0, 1) + MOD(0, 0, 1) + FIN(0, 0))
            wait("w00")
            run_now(PERM(0, 0))
            wait("w10", "w20")

        m0 = [functools.partial(wave_pass, 0, t, nb) for t in range(2) for nb in range(6)]
        m1 = WAVE(1)
        n0, n1, n2 = W0
        p1, p2 = PERM(1, 0), PERM(2, 0)
        segment("T0a", m0[:n0], [(p1, 0, 1), (p2, 1, n0 - 0.5)], need={2: p1})
        wait("x1")
        s1, f1, u = STATS(1), FIN(1, 0), 6 - n0
        segment("T0b", m0[n0:n1], [(s1, 0, max(0.4, u - 1)), (f1, u - 0.5 if u < 3 else u - 1, u - 0.4, s1)], need={u: s1 + f1})
        wait("m11", "m01", "w01")
        mods, f0, f1, pq, u = MOD(1, 1, 2) + MOD(0, 1, 2), FIN(0, 1), FIN(1, 1), PERM(0, 1), 12 - n1
        segment("T0c", m0[n1:] + m1[:n2],
                [(mods, 0, 0.4), (f0, max(1.5, u - 1), max(1.5, u - 1) + 0.4, mods), (f1, u - 0.5, u + 0.5, mods), (pq, 0, u - 1)],
                need={u: mods + f0 + pq, u + 2: f1})
        wait("w11", "w21")
        p1, p2 = PERM(1, 1), PERM(2, 1)
        segment("T1", m1[n2:WA[1]], [(p1, 0, 3 - n2), (p2, 3 - n2, 6.5 - n2)], need={4 - n2: p1, 8 - n2: p2})
        for k in range(2, NC):
            last = k == NC - 1
            wait(f"m1{k}", f"m0{k}", f"w0{k}", f"w1{k}", f"w2{k}", *(["x2"] if last else []))
            u = 12 - WA[k - 1]
            mods = MOD(1, k, k + 1, TMG) + MOD(0, k, k + 1, TMG)
            fins = [FIN(t, k) for t in range(2)]
            perms = [PERM(m, k) for m in range(3)]
            mend = max(0.5, u - WP[0])
            fmin = (8 // TMG - 1) / TN + (mend - 0.5 if mend > 2 else 0)
            groups = [(mods[:1], 0, 1), (mods[1:], mend - 0.5 if mend > 2 else 0, mend),
                      (fins[0], max(fmin, u - WP[1]), max(fmin + 0.2, u - WP[2]), mods), (fins[1], max(fmin + 0.2, u - WP[2]), u + 1, mods),
                      (perms[0], 0, max(0.9, u - WP[3])), (perms[1], max(0.9, u - WP[3]), u + WP[4]), (perms[2], u + WP[4], u + WP[5])]
            if last:
                groups.append((LN1(2, hc_v), *T7L))
            segment(f"T{k}", WAVE(k - 1)[WA[k - 1]:] + (WAVE(k) if last else WAVE(k)[:WA[k]]), groups,
                    need={u: mods + fins[0] + perms[0], u + 2: fins[1], u + 4: perms[1], u + 8: perms[2]}, nrel=TN, lns=TLS)
        wait("xr")

        def a_step(t, carry):
            base = (t - 2) * (NPC * G)
            att = [attn_task(True, base, NPC * G, g, AQ, masked=(g == 0)) for g in range(NPC)]
            l1 = LN1(t + 1, hn_v)
            segment("A", QKV(t), [(att, *AA), (l1, *AL), COPY(hn_v, hc_v, ACN[0], 48 - QT, 47, l1, 0, HK),
                                 COPY(hn_v, hc_v, ACN[1], 47 + 1 / AN, 48 + 1 / AN, l1, HK, D)], dl=ADL, nrel=AN, lns=ALS)
            return carry

        with scope("loopA"):
            jax.lax.fori_loop(2, NT - 1, a_step, 0)
        wait("wmr", "wo", "fw1", "fw3", "fw2a")
        q7, nq = QKV(NT - 1), AFP[0]
        mg, msc, l2 = MOD(2, mg=MG), MOD(3, mg=MG) + MOD(4, mg=MG), LN2(0, hn_v)
        done_rows = (NT - 3) * NPC * G
        att = [attn_task(True, done_rows, SA - done_rows, g, AFQ) for g in range((SA - done_rows) // G)]
        segment("AF", q7[:nq] + WO(0) + q7[nq:] + FFN(0, 0, C0),
                [(mg, 0, AFP[1]), (msc, AFP[1], AFP[2]), (l2, max(AFP[3], nq + 16), AFP[4], msc),
                 (MOD(5, mg=MG), AFP[5], AFP[6]), (att, AFP[7], AFP[8]), ([halo_task()], 1, 2)]
                + [COPY(hn_v, h2_v, 16, *AFC, l2)], need={nq: mg, 64: l2}, dl=AFDL, nrel=AFN, lns=AFL)
        wait("fw2b")

        nch = F // HK
        nf = (nch - C0) * 24

        def b_step(i, carry):
            att = [attn_task(False, jnp.minimum(i, NT - 3) * TM, TM, g, BQ) for g in range(NG)]
            l2 = LN2(i + 1, hn_v)
            ffn = FFN(i, C0, nch)
            cpy = [COPY(hn_v, h2_v, 16, nf + 16 - 8 + BCP[0], nf + 16 - 8 + BCP[1], l2)]
            assert BA[0] >= 16 + BW and BL[0] >= 16 + BW and min(BCP) >= 0
            segment("F", ffn[:BW] + WO(i + 1) + ffn[BW:] + FFN(i + 1, 0, C0), ([(att, *BA)] if NOV < 1 else []) + ([(l2, *BL)] + cpy if NOV < 2 else []),
                    need={nf + 16: l2}, dl=BDL, nrel=BN, lns=BLS)
            return carry

        with scope("B"):
            jax.lax.fori_loop(0, NT - 1, b_step, 0)
        for t in range(NT - 2):
            out_wait(t)
        segment("FL", FFN(NT - 1, C0, nch))
        with scope("fin"):
            for t in range(NT - 2, NT):
                out_wait(t)

    @jax.jit
    def fn(A_x, A_wqkv, A_wo, B_x, B_w1, B_w3, B_w2, c, w_mod):
        V = pltpu.VMEM
        scratch = [
            V((S, D), BF16), V((3, D, D), BF16), V((D // 2, 3 * D), U32), V((D, D), BF16),
            V((D, F), BF16), V((D, F), BF16), V((F, D), BF16), V((2 * NC, D, 128), BF16), V((D, 4 * D), BF16),
            V((8, D), F32), V((D, 128), F32), V((2, SA, 128), F32), V((2, TM // 2, D), U32),
            V((NC, SA, 128), F32), V((NC, PAD + SA, 128), F32), V((NC, PAD + SA, 128), F32),
            V((NC, SB, 128), F32), V((NC, PAD + SB, 128), F32), V((NC, PAD + SB, 128), F32),
            V((S // 2, D), U32), V((NC, S, 128), F32), V((TM // 2, D), U32), V((NC, S, 128), BF16),
            V((TM // 2, D), U32), V((TM // 2, D), U32), V((NC, TM, 128), F32), V((32, 128), F32), V((1, D), BF16),
            pltpu.SemaphoreType.DMA((5 * NC + 12,)), pltpu.SemaphoreType.DMA((NT,)), pltpu.SemaphoreType.REGULAR,
        ]
        out = pl.pallas_call(
            kernel,
            in_specs=[pl.BlockSpec(memory_space=pl.ANY)] * 8,
            out_specs=pl.BlockSpec(memory_space=pl.ANY),
            out_shape=jax.ShapeDtypeStruct((S, D), BF16),
            scratch_shapes=scratch,
            compiler_params=pltpu.CompilerParams(vmem_limit_bytes=124 * 1024 * 1024, disable_bounds_checks=True,
                                                 disable_semaphore_checks=True),
        )(A_x.reshape(S, D), A_wqkv, A_wo, B_w1, B_w3, B_w2, c, w_mod)
        return out.reshape(1, S, D)

    return fn


_impl = make_kernel()


@jax.jit
def pallas_adaLN_cond__sliding_local_dilated__glu_gated_swiglu__prompt_kernel(A_x, A_wqkv, A_wo, B_x, B_w1, B_w3, B_w2, c, w_mod):
    return _impl(A_x, A_wqkv, A_wo, B_x, B_w1, B_w3, B_w2, c, w_mod)
```

```python
import contextlib
import functools
import math

import jax
import jax.numpy as jnp
import jax.experimental.pallas as pl
import jax.experimental.pallas.tpu as pltpu

S, D, F = 2048, 1024, 3584
DH, WIN, DIL = 32, 8, 2
NC = D // 128
PAD = 16
EPS = 1e-5
SCALE = DH ** -0.5
EXP2_C = SCALE * math.log2(math.e)
MASKED = -1e9 / SCALE
F32, BF16, U32 = jnp.float32, jnp.bfloat16, jnp.uint32
TM = 256
NT = S // TM
G = 16
NG = TM // G
HK = D // 2
SA = 2 * TM
SB = S - SA


def _xor_network(xs):
    lane = jax.lax.broadcasted_iota(jnp.int32, xs[0].shape, 1)
    for b in range(3):
        m = ((lane >> (2 + b)) & 1) == 1
        xs = [jnp.where(m, xs[i ^ (1 << b)], xs[i]) for i in range(NC)]
    return xs


def _gather_fwd(z, j):
    lane = jax.lax.broadcasted_iota(jnp.int32, z.shape, 1)
    e, g, p = lane >> 5, (lane >> 3) & 3, lane & 7
    return jnp.take_along_axis(z, g * 32 + (p ^ j) * 4 + e, axis=1)


def _gather_inv(y, j):
    lane = jax.lax.broadcasted_iota(jnp.int32, y.shape, 1)
    g, q, e = lane >> 5, (lane >> 2) & 7, lane & 3
    return jnp.take_along_axis(y, e * 32 + g * 8 + (q ^ j), axis=1)


def _pack(x):
    return pltpu.bitcast(x.astype(BF16), U32)


def _or_all(vs):
    parts = [v[r:r + 8, c:c + 128] for v in vs for r in range(0, v.shape[0], 8) for c in range(0, v.shape[1], 128)]
    while len(parts) > 1:
        parts = [parts[i] | parts[i + 1] if i + 1 < len(parts) else parts[i] for i in range(0, len(parts), 2)]
    return parts[0]


def _gate(x, g):
    if g is None:
        return x
    xb = x if x.dtype == U32 else pltpu.bitcast(x, U32)
    y = xb | jnp.tile(g, (x.shape[0] // 8, x.shape[1] // 128))
    return y if x.dtype == U32 else pltpu.bitcast(y, x.dtype)


def _rows(start, n, mult):
    if isinstance(start, int):
        return pl.ds(start, n)
    return pl.ds(pl.multiple_of(start, mult), n)


def _stats(x):
    mu = jnp.mean(x, axis=-1, keepdims=True)
    xc = x - mu
    var = jnp.mean(xc * xc, axis=-1, keepdims=True)
    return mu, xc, jax.lax.rsqrt(var + EPS)


def make_kernel(NREL=2, DL=4,
                W0=(4, 10, 3), WA=(9, 10, 7, 6, 6, 6, 6), WP=(2.5, 1, 0.25, 1, 2, 6), X2AT=5, PR=16, X2S=(2, 9),
                X2F=((6, 9.5, 10.5), (7, 2, 3), (7, 4, 5), (7, 7, 8), (7, 9, 10), (7, 12, 13), (7, 13, 14), (7, 14, 15)),
                AQ=(2, 2, 13, 4), AA=(1, 38), AL=(2, 38), ADL=4,
                NOV=0, DSH=1, QKJ=True, PVW=2, C0=1, NPC=6, AFQ=(1, 1, 12, 3), AFP=(20, 15, 36, 38, 58, 60, 84, 0, 16), AFDL=5,
                BW=2, BQ=(1, 1, 20, 5), BA=(18, 170), BL=(20, 149), BCP=(8, 28), AFC=(66, 86), QT=4, ACN=(4, 2), BDL=6,
                MG=1, AFN=4, AFL=(0, 0), AN=4, ALS=(2, 4), BN=4, BLS=(2, 4), TMG=2, TN=4, TLS=(1, 3), scopes=False, only=None):

    def scope(name):
        return jax.named_scope(name) if scopes else contextlib.nullcontext()

    def kernel(x_hbm, wqkv_hbm, wo_hbm, w1_hbm, w3_hbm, w2_hbm, c_hbm, wm_hbm, out_hbm,
               x_v, wraw_v, wp_v, wo_v, w1_v, w3_v, w2_v, wmc_v, wmr_v,
               mod_v, scol_v, st_v, h1_v, qa_v, ka_v, va_v, qb_v, kb_v, vb_v, o_v, x1_v, h2_v, out_v,
               hc_v, hn_v, acc_v, z_v, c_v, sems, sem_out, bar):
        cp = pltpu.make_async_copy

        dmas = {}

        def add(name, src, dst):
            dmas[name] = cp(src, dst, sems.at[len(dmas)])

        def add_x(name, t0, n):
            add(name, x_hbm.at[pl.ds(t0 * TM, n * TM), :], x_v.at[pl.ds(t0 * TM, n * TM), :])

        add("c", c_hbm, c_v)
        add_x("x0", 0, 1)
        for k in range(NC):
            for m in (1, 0):
                add(f"m{m}{k}", wm_hbm.at[:, pl.ds(m * D + k * 128, 128)], wmc_v.at[m * NC + k])
            for m in range(3):
                add(f"w{m}{k}", wqkv_hbm.at[pl.ds(k * 128, 128), pl.ds(m * D, D)], wraw_v.at[m, pl.ds(k * 128, 128), :])
            if k == 0:
                add_x("x1", 1, 1)
            if k == X2AT:
                add_x("x2", 2, 1)
        add_x("xr", 3, NT - 3)
        add("wmr", wm_hbm.at[:, pl.ds(2 * D, 4 * D)], wmr_v)
        add("wo", wo_hbm, wo_v)
        add("fw1", w1_hbm, w1_v)
        add("fw3", w3_hbm, w3_v)
        add("fw2a", w2_hbm.at[pl.ds(0, C0 * HK), :], w2_v.at[pl.ds(0, C0 * HK), :])
        add("fw2b", w2_hbm.at[pl.ds(C0 * HK, F - C0 * HK), :], w2_v.at[pl.ds(C0 * HK, F - C0 * HK), :])
        for d in dmas.values():
            d.start()
            pl.semaphore_signal(bar, 1)
            pl.semaphore_wait(bar, 1)
        for j in range(NC):
            ka_v[j, 0:PAD, :] = jnp.zeros((PAD, 128), F32)
            va_v[j, 0:PAD, :] = jnp.zeros((PAD, 128), F32)
        add("z", ka_v.at[0, pl.ds(0, 8), :], z_v.at[pl.ds(0, 8), :])
        dmas["z"].start()

        def wait(*names):
            with scope("w_" + names[0]):
                for n in names:
                    dmas[n].wait()

        def zero():
            return pltpu.bitcast(z_v[0:8, :], U32)

        cur = {"nrel": NREL, "lns": (0, 0)}

        def mod_task(m, j, mg=2):
            src = wmc_v.at[m * NC + j] if m < 2 else wmr_v.at[:, pl.ds((m - 2) * D + j * 128, 128)]
            acc = None
            for kb in range(D // 128):
                if kb % mg == 0:
                    rel = yield
                p = src[kb * 128:(kb + 1) * 128, :].astype(F32) * scol_v[kb * 128:(kb + 1) * 128, :]
                parts = [p[r:r + 8] for r in range(0, 128, 8)]
                a0, a1 = parts[0], parts[1]
                if kb % mg == 0:
                    a0, a1 = _gate(a0, rel), _gate(a1, rel)
                for r in range(2, 16, 2):
                    a0, a1 = a0 + parts[r], a1 + parts[r + 1]
                a0 = a0 + a1
                acc = a0 if acc is None else acc + a0
            r = jnp.sum(acc, axis=0, keepdims=True)
            if m in (1, 4):
                r = r + 1.0
            mod_v[m:m + 1, j * 128:(j + 1) * 128] = r
            return pltpu.bitcast(jnp.broadcast_to(r, (8, 128)), U32)

        def modulate(xn, ms, dst, g, c0, c1):
            hb = _pack(xn * mod_v[ms + 1:ms + 2, c0:c1] + mod_v[ms:ms + 1, c0:c1])
            dst[g * 8:(g + 1) * 8, c0:c1] = hb
            return _or_all([hb])

        def ln_tail(xc, rs, ms, dst, g):
            ns, skip = cur["lns"]
            if ns == 0:
                return modulate(xc * rs, ms, dst, g, 0, D)
            for _ in range(skip):
                yield
            rs = jnp.broadcast_to(rs, (G, 128))
            toks = []
            cw = D // ns
            for p in range(ns):
                rel = yield
                r = jnp.tile(_gate(rs, rel), (1, cw // 128))
                toks.append(modulate(xc[:, p * cw:(p + 1) * cw] * r, ms, dst, g, p * cw, (p + 1) * cw))
            return _or_all(toks)

        def ln1_task(t, g, dst):
            rel = yield
            xt = x_v.at[_rows(t * TM, TM, TM), :]
            _, xc, rs = _stats(_gate(xt[g * G:(g + 1) * G, :].astype(F32), rel))
            return (yield from ln_tail(xc, rs, 0, dst, g))

        def stats_task(t, g):
            rel = yield
            rows = slice(t * TM + g * G, t * TM + (g + 1) * G)
            mu, _, rs = _stats(_gate(x_v[rows, :].astype(F32), rel))
            st_v[0, rows, :] = jnp.broadcast_to(mu, (G, 128))
            st_v[1, rows, :] = jnp.broadcast_to(rs, (G, 128))

        def fin_task(t, k, g0, ng):
            rel = yield
            for g in range(g0, g0 + ng):
                rows = slice(t * TM + g * G, t * TM + (g + 1) * G)
                x = _gate(x_v[rows, k * 128:(k + 1) * 128].astype(F32), rel)
                modulate((x - st_v[0, rows, :]) * st_v[1, rows, :], 0, h1_v.at[t] if t < 2 else hc_v, g, k * 128, (k + 1) * 128)

        def ln2_task(t, g, dst):
            rel = yield
            xv = x1_v.at[:, _rows(t * TM, TM, TM), :]
            x = jnp.concatenate([_gate(xv[j, g * G:(g + 1) * G, :], rel) for j in range(NC)], axis=1)
            _, xc, rs = _stats(x)
            return (yield from ln_tail(xc, rs, 3, dst, g))

        def perm_select_task(m, r0, n):
            rel = yield
            xs = [_gate(pltpu.bitcast(wraw_v[m, r0:r0 + n, j * 128:(j + 1) * 128], U32), rel) for j in range(NC)]
            zs = _xor_network(xs)
            for j in range(NC):
                wp_v[r0 // 2:(r0 + n) // 2, m * D + j * 128:m * D + (j + 1) * 128] = zs[j]

        def perm_gather_task(m, j, r0, n):
            rel = yield
            sl = (slice(r0 // 2, (r0 + n) // 2), slice(m * D + j * 128, m * D + (j + 1) * 128))
            wp_v[sl] = _gather_fwd(_gate(wp_v[sl], rel), j)

        def copy_task(src, dst, r0, nr, c0, c1):
            rel = yield
            dst[r0:r0 + nr, c0:c1] = _gate(src[r0:r0 + nr, c0:c1], rel)

        def halo_task():
            yield
            for j in range(NC):
                kb_v[j, 0:PAD, :] = ka_v[j, SA:SA + PAD, :]
                vb_v[j, 0:PAD, :] = va_v[j, SA:SA + PAD, :]

        def attn_task(first, base, span, g, pace, masked=False):
            qkg, pvg, skip, smd = pace
            q_v, k_v, v_v = (qa_v, ka_v, va_v) if first else (qb_v, kb_v, vb_v)
            qv = q_v.at[:, _rows(base, span, 32), :]
            kv = k_v.at[:, _rows(base, span + PAD, 32), :]
            vv = v_v.at[:, _rows(base, span + PAD, 32), :]

            def shifted(ref, j, w):
                return ref[j, pl.ds(g * G + PAD - DIL * w, G), :]

            if QKJ:
                ls = [None] * WIN
                for j in range(NC):
                    if j % qkg == 0:
                        rel = yield
                    q = _gate(qv[j, g * G:(g + 1) * G, :], rel)
                    for w in range(WIN):
                        p = q * shifted(kv, j, w)
                        ls[w] = p if j == 0 else ls[w] + p
            else:
                q = [qv[j, g * G:(g + 1) * G, :] for j in range(NC)]
                ls = []
                for w in range(WIN):
                    if w % qkg == 0:
                        rel = yield
                    acc = _gate(q[0], rel) * shifted(kv, 0, w)
                    for j in range(1, NC):
                        acc = acc + q[j] * shifted(kv, j, w)
                    ls.append(acc)
            ls = [l + pltpu.roll(l, 64, 1) for l in ls]
            ls = [l + pltpu.roll(l, 32, 1) for l in ls]
            if masked:
                rows = base + g * G + jax.lax.broadcasted_iota(jnp.int32, (G, 128), 0)
                ls = [ls[0]] + [jnp.where(rows >= DIL * w, ls[w], MASKED) for w in range(1, WIN)]
            mx = ls[0]
            for w in range(1, WIN):
                mx = jnp.maximum(mx, ls[w])
            ps = [jnp.exp2((l - mx) * EXP2_C) for l in ls]
            den = ps[0]
            for w in range(1, WIN):
                den = den + ps[w]
            inv = 1.0 / den
            ps = [pw * inv for pw in ps]
            if smd:
                yield _or_all([pltpu.bitcast(ps[0], U32)]), smd
            for _ in range(skip - (1 if smd else 0)):
                yield
            zs = []
            if PVW == 1:
                os_ = [None] * NC
                for w in range(WIN):
                    if w % pvg == 0:
                        rel = yield
                    p = _gate(ps[w], rel)
                    for j in range(NC):
                        pv = p * shifted(vv, j, w)
                        os_[j] = pv if w == 0 else os_[j] + pv
                for j in range(NC):
                    if j % 4 == 0:
                        rel = yield
                    zs.append(_gather_inv(_pack(_gate(os_[j], rel)), j))
            else:
                for j in range(NC):
                    if j % pvg == 0:
                        rel = yield
                        pg = [_gate(p, rel) for p in ps] if PVW == 2 else [_gate(ps[0], rel)] + ps[1:]
                    acc = pg[0] * shifted(vv, j, 0)
                    for w in range(1, WIN):
                        acc = acc + pg[w] * shifted(vv, j, w)
                    zs.append(_gather_inv(_pack(acc), j))
            xs = _xor_network(zs)
            half = (base // 2 if isinstance(base, int) else jax.lax.shift_right_logical(base, 1)) + (0 if first else SA // 2)
            ov = o_v.at[_rows(half, span // 2, 16), :]
            for j in range(NC):
                ov[g * 8:(g + 1) * 8, j * 128:(j + 1) * 128] = xs[j]
            return _or_all(xs)

        def LN1(t, dst):
            return [ln1_task(t, g, dst) for g in range(NG)]

        def LN2(t, dst):
            return [ln2_task(t, g, dst) for g in range(NG)]

        def STATS(t):
            return [stats_task(t, g) for g in range(NG)]

        def FIN(t, k):
            return [fin_task(t, k, g0, 4) for g0 in range(0, NG, 4)]

        def MOD(m, j0=0, j1=NC, mg=2):
            return [mod_task(m, j, mg) for j in range(j0, j1)]

        def PERM(m, k):
            r0 = k * 128
            return ([perm_select_task(m, r, PR) for r in range(r0, r0 + 128, PR)]
                    + [perm_gather_task(m, j, r0, 128) for j in range(NC)])

        def COPY(src, dst, n, lo, hi, pre, c0=0, c1=D):
            nr = TM // 2 // n
            return ([copy_task(src, dst, r, nr, c0, c1) for r in range(0, TM // 2, nr)], lo, hi, pre)

        def run_now(tasks):
            for tk in tasks:
                try:
                    next(tk)
                    while True:
                        tk.send(None)
                except StopIteration:
                    pass

        def tie(a, tok):
            if tok is not None:
                top = a[0:8, 0:128] | (tok & zero())
                if a.shape[1] > 128:
                    top = jnp.concatenate([top, a[0:8, 128:]], axis=1)
                a = jnp.concatenate([top, a[8:]], axis=0)
            return pltpu.bitcast(a, BF16)


        def releases(res):
            return [pltpu.bitcast(res[r:r + 8, 0:128], U32) & zero() for r in range(0, TM, TM // cur["nrel"])]

        def wave_pass(k, t, nb, tok):
            m, j0 = nb // 2, (nb % 2) * 4
            dst = (qa_v, ka_v, va_v)[m]
            rows = slice(t * TM + (PAD if m else 0), (t + 1) * TM + (PAD if m else 0))
            w = pltpu.bitcast(wp_v[k * 64:(k + 1) * 64, nb * 512:(nb + 1) * 512], BF16)
            res = jnp.dot(tie(h1_v[t, :, k * 128:(k + 1) * 128], tok), w, preferred_element_type=F32)
            for jj in range(4):
                r = res[:, jj * 128:(jj + 1) * 128]
                if k > 0:
                    r = dst[j0 + jj, rows, :] + r
                dst[j0 + jj, rows, :] = r
            return releases(res)

        def qkv_pass(t, m, j, hf, st, tok):
            w = pltpu.bitcast(wp_v[hf * HK // 2:(hf + 1) * HK // 2, m * D + j * 128:m * D + (j + 1) * 128], BF16)
            res = jnp.dot(tie(hc_v[:, hf * HK:(hf + 1) * HK], tok), w, preferred_element_type=F32)
            if hf == 0:
                st[m, j] = res
            else:
                res = st.pop((m, j)) + res
                off = PAD if m else 0
                dst = (qb_v, kb_v, vb_v)[m].at[:, _rows((t - 2) * TM, TM + off, TM), :]
                dst[j, off:off + TM, :] = res
            return releases(res)

        def wo_pass(t, j, hf, st, tok):
            h = tie(o_v[_rows(t * (TM // 2), TM // 2, TM // 2), hf * HK:(hf + 1) * HK], tok)
            res = jnp.dot(h, wo_v[hf * HK:(hf + 1) * HK, j * 128:(j + 1) * 128], preferred_element_type=F32)
            if hf == 0:
                st["a"] = res
            else:
                rows, cs = _rows(t * TM, TM, TM), slice(j * 128, (j + 1) * 128)
                res = x_v[rows, cs].astype(F32) + mod_v[2:3, cs] * (st.pop("a") + res)
                x1_v[j, rows, :] = res
            return releases(res)

        def out_copy(t, j):
            rows = _rows(t * TM, TM, TM)
            return cp(out_v.at[j, rows, :], out_hbm.at[rows, pl.ds(j * 128, 128)], sem_out.at[t])

        def out_wait(t):
            if only is not None and ("FL" if t == NT - 1 else "F") not in only:
                return
            rows = pl.ds(t * TM, TM)
            cp(out_hbm.at[rows, :], out_hbm.at[rows, :], sem_out.at[t]).wait()

        def WAVE(k):
            return [functools.partial(wave_pass, k, t, nb) for m in range(3) for t in range(2) for nb in (2 * m, 2 * m + 1)]

        def QKV(t):
            order = [(m, j, hf) for m in range(3) for j in range(NC) for hf in range(2)]
            order = order[:-2 * QT] + order[-2 * QT::2] + order[-2 * QT + 1::2]
            st = {}
            return [functools.partial(qkv_pass, t, m, j, hf, st) for m, j, hf in order]

        def WO(t):
            st = {}
            return [functools.partial(wo_pass, t, j, hf, st) for j in range(NC) for hf in range(2)]

        def FFN(t, c0, c1):
            st = {"acc": [None] * NC, "act": []}
            h_v = hn_v if c0 == 0 else h2_v

            def gate_up_pass(which, n, hf, tok):
                w = (w1_v, w3_v)[which][hf * HK:(hf + 1) * HK, n * 128:(n + 1) * 128]
                res = jnp.dot(tie(h_v[:, hf * HK:(hf + 1) * HK], tok), w, preferred_element_type=F32)
                if hf == 0:
                    st["a"] = res
                else:
                    res = st.pop("a") + res
                    if which == 0:
                        hg = 0.5 * res
                        st["g"] = hg + hg * jnp.tanh(hg)
                    else:
                        st["act"].append((st.pop("g") * res).astype(BF16))
                return releases(res)

            def down_pass(c, j, last, tok):
                if j == 0:
                    st["lhs"], st["act"] = jnp.concatenate(st["act"], axis=1), []
                w = w2_v[c * HK:(c + 1) * HK, j * 128:(j + 1) * 128]
                if tok is not None:
                    w = tie(pltpu.bitcast(w, U32), tok)
                res = jnp.dot(st["lhs"], w, preferred_element_type=F32)
                if c > 0:
                    res = (acc_v[j] if c == c0 else st["acc"][j]) + res
                st["acc"][j] = res
                if c == c1 - 1 and not last:
                    acc_v[j] = res
                if last:
                    rows = _rows(t * TM, TM, TM)
                    out_v[j, rows, :] = (x1_v[j, rows, :] + mod_v[5:6, j * 128:(j + 1) * 128] * res).astype(BF16)
                    out_copy(t, j).start()
                return releases(res)

            out = []
            nch = F // HK
            for c in range(c0, c1):
                for n in range(c * 4, c * 4 + 4):
                    out += [functools.partial(gate_up_pass, which, n, hf) for which in range(2) for hf in range(2)]
                out += [functools.partial(down_pass, c, j, c == nch - 1) for j in range(NC)]
            return out

        def segment(name, passes, groups=(), dl=DL, need=None, nrel=NREL, lns=(0, 0)):
            if only is not None and name not in only:
                return
            with scope(name):
                n = len(passes)
                cur["nrel"], cur["lns"] = nrel, lns
                active = []
                for tasks, lo, hi, *pre in groups:
                    for k, tk in enumerate(tasks):
                        active.append((int((lo + k * (hi - lo) / len(tasks)) * nrel), tk, pre[0] if pre else ()))
                        next(tk)
                deadlines = [[] for _ in range(n + dl + 8)]

                def due(p):
                    return p + DSH if p < n and passes[p].func.__name__ == "down_pass" else p

                def done(tasks):
                    return all(ent[1] is not tk for tk in tasks for ent in active)

                def feed(rel, slot, i):
                    for ent in list(active):
                        if ent[0] <= slot:
                            assert done(ent[2]), (name, i)
                            try:
                                mid = ent[1].send(rel)
                                if mid is not None:
                                    deadlines[due(i + mid[1])].append(mid[0])
                            except StopIteration as e:
                                if e.value is not None:
                                    deadlines[due(i + dl)].append(e.value)
                                active.remove(ent)

                feed(None, 0, 0)
                slot = 1
                for i, ps in enumerate(passes):
                    assert done((need or {}).get(i, ())), (name, i)
                    for rel in ps(_or_all(deadlines[i]) if deadlines[i] else None):
                        feed(rel, slot, i)
                        slot += 1
                while active:
                    feed(None, 1 << 30, n)

        with scope("S0"):
            wait("c", "z")
            c = c_v[...].astype(F32)
            s = (c * jax.nn.sigmoid(c)).astype(BF16).astype(F32)
            eye = (jax.lax.broadcasted_iota(jnp.int32, (128, 128), 0)
                   == jax.lax.broadcasted_iota(jnp.int32, (128, 128), 1))
            ones = jnp.ones((128, 128), BF16)
            for j in range(NC):
                dg = jnp.where(eye, jnp.broadcast_to(s[:, j * 128:(j + 1) * 128], (128, 128)), 0.0).astype(BF16)
                scol_v[j * 128:(j + 1) * 128, :] = jnp.dot(dg, ones, preferred_element_type=F32)
            wait("x0")
            run_now(STATS(0))
            wait("m10", "m00")
            run_now(MOD(1, 0, 1) + MOD(0, 0, 1) + FIN(0, 0))
            wait("w00")
            run_now(PERM(0, 0))
            wait("w10", "w20")

        m0 = [functools.partial(wave_pass, 0, t, nb) for t in range(2) for nb in range(6)]
        m1 = WAVE(1)
        n0, n1, n2 = W0
        p1, p2 = PERM(1, 0), PERM(2, 0)
        segment("T0a", m0[:n0], [(p1, 0, 1), (p2, 1, n0 - 0.5)], need={2: p1})
        wait("x1")
        s1, f1, u = STATS(1), FIN(1, 0), 6 - n0
        segment("T0b", m0[n0:n1], [(s1, 0, max(0.4, u - 1)), (f1, u - 0.5 if u < 3 else u - 1, u - 0.4, s1)], need={u: s1 + f1})
        wait("m11", "m01", "w01")
        mods, f0, f1, pq, u = MOD(1, 1, 2) + MOD(0, 1, 2), FIN(0, 1), FIN(1, 1), PERM(0, 1), 12 - n1
        segment("T0c", m0[n1:] + m1[:n2],
                [(mods, 0, 0.4), (f0, max(1.5, u - 1), max(1.5, u - 1) + 0.4, mods), (f1, u - 0.5, u + 0.5, mods), (pq, 0, u - 1)],
                need={u: mods + f0 + pq, u + 2: f1})
        wait("w11", "w21")
        p1, p2 = PERM(1, 1), PERM(2, 1)
        segment("T1", m1[n2:WA[1]], [(p1, 0, 3 - n2), (p2, 3 - n2, 6.5 - n2)], need={4 - n2: p1, 8 - n2: p2})
        for k in range(2, NC):
            last = k == NC - 1
            wait(f"m1{k}", f"m0{k}", f"w0{k}", f"w1{k}", f"w2{k}", *(["x2"] if k == X2AT + 1 else []))
            u = 12 - WA[k - 1]
            mods = MOD(1, k, k + 1, TMG) + MOD(0, k, k + 1, TMG)
            fins = [FIN(t, k) for t in range(2)]
            perms = [PERM(m, k) for m in range(3)]
            mend = max(0.5, u - WP[0])
            fmin = (8 // TMG - 1) / TN + (mend - 0.5 if mend > 2 else 0)
            groups = [(mods[:1], 0, 1), (mods[1:], mend - 0.5 if mend > 2 else 0, mend),
                      (fins[0], max(fmin, u - WP[1]), max(fmin + 0.2, u - WP[2]), mods), (fins[1], max(fmin + 0.2, u - WP[2]), u + 1, mods),
                      (perms[0], 0, max(0.9, u - WP[3])), (perms[1], max(0.9, u - WP[3]), u + WP[4]), (perms[2], u + WP[4], u + WP[5])]
            if k == X2AT + 1:
                s2 = STATS(2)
                groups.append((s2, *X2S))
            for kk in range(NC):
                if X2F[kk][0] == k:
                    assert kk <= k
                    groups.append((FIN(2, kk), *X2F[kk][1:], (s2 if k == X2AT + 1 else []) + (mods if kk == k else [])))
            segment(f"T{k}", WAVE(k - 1)[WA[k - 1]:] + (WAVE(k) if last else WAVE(k)[:WA[k]]), groups,
                    need={u: mods + fins[0] + perms[0], u + 2: fins[1], u + 4: perms[1], u + 8: perms[2]}, nrel=TN, lns=TLS)
        wait("xr")

        def a_step(t, carry):
            base = jnp.minimum((t - 2) * (NPC // 2), NG) * (2 * G)
            att = [attn_task(True, base, NPC * G, g, AQ, masked=(g == 0)) for g in range(NPC)]
            l1 = LN1(t + 1, hn_v)
            segment("A", QKV(t), [(att, *AA), (l1, *AL), COPY(hn_v, hc_v, ACN[0], 48 - QT, 47, l1, 0, HK),
                                 COPY(hn_v, hc_v, ACN[1], 47 + 1 / AN, 48 + 1 / AN, l1, HK, D)], dl=ADL, nrel=AN, lns=ALS)
            return carry

        with scope("loopA"):
            jax.lax.fori_loop(2, NT - 1, a_step, 0)
        wait("wmr", "wo", "fw1", "fw3", "fw2a")
        q7, nq = QKV(NT - 1), AFP[0]
        mg, msc, l2 = MOD(2, mg=MG), MOD(3, mg=MG) + MOD(4, mg=MG), LN2(0, hn_v)
        done_rows = (NT - 3) * NPC * G
        att = [attn_task(True, done_rows, SA - done_rows, g, AFQ) for g in range((SA - done_rows) // G)]
        segment("AF", q7[:nq] + WO(0) + q7[nq:] + FFN(0, 0, C0),
                [(mg, 0, AFP[1]), (msc, AFP[1], AFP[2]), (l2, max(AFP[3], nq + 16), AFP[4], msc),
                 (MOD(5, mg=MG), AFP[5], AFP[6]), (att, AFP[7], AFP[8]), ([halo_task()], 1, 2)]
                + [COPY(hn_v, h2_v, 16, *AFC, l2)], need={nq: mg, 64: l2}, dl=AFDL, nrel=AFN, lns=AFL)
        wait("fw2b")

        nch = F // HK
        nf = (nch - C0) * 24

        def b_step(i, carry):
            att = [attn_task(False, jnp.minimum(i, NT - 3) * TM, TM, g, BQ) for g in range(NG)]
            l2 = LN2(i + 1, hn_v)
            ffn = FFN(i, C0, nch)
            cpy = [COPY(hn_v, h2_v, 16, nf + 16 - 8 + BCP[0], nf + 16 - 8 + BCP[1], l2)]
            assert BA[0] >= 16 + BW and BL[0] >= 16 + BW and min(BCP) >= 0
            segment("F", ffn[:BW] + WO(i + 1) + ffn[BW:] + FFN(i + 1, 0, C0), ([(att, *BA)] if NOV < 1 else []) + ([(l2, *BL)] + cpy if NOV < 2 else []),
                    need={nf + 16: l2}, dl=BDL, nrel=BN, lns=BLS)
            return carry

        with scope("B"):
            jax.lax.fori_loop(0, NT - 1, b_step, 0)
        for t in range(NT - 2):
            out_wait(t)
        segment("FL", FFN(NT - 1, C0, nch))
        with scope("fin"):
            for t in range(NT - 2, NT):
                out_wait(t)

    @jax.jit
    def fn(A_x, A_wqkv, A_wo, B_x, B_w1, B_w3, B_w2, c, w_mod):
        V = pltpu.VMEM
        scratch = [
            V((S, D), BF16), V((3, D, D), BF16), V((D // 2, 3 * D), U32), V((D, D), BF16),
            V((D, F), BF16), V((D, F), BF16), V((F, D), BF16), V((2 * NC, D, 128), BF16), V((D, 4 * D), BF16),
            V((8, D), F32), V((D, 128), F32), V((2, SA + TM, 128), F32), V((2, TM // 2, D), U32),
            V((NC, SA, 128), F32), V((NC, PAD + SA, 128), F32), V((NC, PAD + SA, 128), F32),
            V((NC, SB, 128), F32), V((NC, PAD + SB, 128), F32), V((NC, PAD + SB, 128), F32),
            V((S // 2, D), U32), V((NC, S, 128), F32), V((TM // 2, D), U32), V((NC, S, 128), BF16),
            V((TM // 2, D), U32), V((TM // 2, D), U32), V((NC, TM, 128), F32), V((32, 128), F32), V((1, D), BF16),
            pltpu.SemaphoreType.DMA((5 * NC + 12,)), pltpu.SemaphoreType.DMA((NT,)), pltpu.SemaphoreType.REGULAR,
        ]
        out = pl.pallas_call(
            kernel,
            in_specs=[pl.BlockSpec(memory_space=pl.ANY)] * 8,
            out_specs=pl.BlockSpec(memory_space=pl.ANY),
            out_shape=jax.ShapeDtypeStruct((S, D), BF16),
            scratch_shapes=scratch,
            compiler_params=pltpu.CompilerParams(vmem_limit_bytes=124 * 1024 * 1024, disable_bounds_checks=True,
                                                 disable_semaphore_checks=True),
        )(A_x.reshape(S, D), A_wqkv, A_wo, B_w1, B_w3, B_w2, c, w_mod)
        return out.reshape(1, S, D)

    return fn


_impl = make_kernel()


@jax.jit
def pallas_adaLN_cond__sliding_local_dilated__glu_gated_swiglu__prompt_kernel(A_x, A_wqkv, A_wo, B_x, B_w1, B_w3, B_w2, c, w_mod):
    return _impl(A_x, A_wqkv, A_wo, B_x, B_w1, B_w3, B_w2, c, w_mod)
```

```python
import contextlib
import functools
import math

import jax
import jax.numpy as jnp
import jax.experimental.pallas as pl
import jax.experimental.pallas.tpu as pltpu

S, D, F = 2048, 1024, 3584
DH, WIN, DIL = 32, 8, 2
NC = D // 128
PAD = 16
EPS = 1e-5
SCALE = DH ** -0.5
EXP2_C = SCALE * math.log2(math.e)
MASKED = -1e9 / SCALE
F32, BF16, U32 = jnp.float32, jnp.bfloat16, jnp.uint32
TM = 256
NT = S // TM
G = 16
NG = TM // G
HK = D // 2
SA = 2 * TM
SB = S - SA


def _xor_network(xs):
    lane = jax.lax.broadcasted_iota(jnp.int32, xs[0].shape, 1)
    for b in range(3):
        m = ((lane >> (2 + b)) & 1) == 1
        xs = [jnp.where(m, xs[i ^ (1 << b)], xs[i]) for i in range(NC)]
    return xs


def _gather_fwd(z, j):
    lane = jax.lax.broadcasted_iota(jnp.int32, z.shape, 1)
    e, g, p = lane >> 5, (lane >> 3) & 3, lane & 7
    return jnp.take_along_axis(z, g * 32 + (p ^ j) * 4 + e, axis=1)


def _gather_inv(y, j):
    lane = jax.lax.broadcasted_iota(jnp.int32, y.shape, 1)
    g, q, e = lane >> 5, (lane >> 2) & 7, lane & 3
    return jnp.take_along_axis(y, e * 32 + g * 8 + (q ^ j), axis=1)


def _pack(x):
    return pltpu.bitcast(x.astype(BF16), U32)


def _or_all(vs):
    parts = [v[r:r + 8, c:c + 128] for v in vs for r in range(0, v.shape[0], 8) for c in range(0, v.shape[1], 128)]
    while len(parts) > 1:
        parts = [parts[i] | parts[i + 1] if i + 1 < len(parts) else parts[i] for i in range(0, len(parts), 2)]
    return parts[0]


def _gate(x, g):
    if g is None:
        return x
    xb = x if x.dtype == U32 else pltpu.bitcast(x, U32)
    y = xb | jnp.tile(g, (x.shape[0] // 8, x.shape[1] // 128))
    return y if x.dtype == U32 else pltpu.bitcast(y, x.dtype)


def _rows(start, n, mult):
    if isinstance(start, int):
        return pl.ds(start, n)
    return pl.ds(pl.multiple_of(start, mult), n)


def _stats(x):
    mu = jnp.mean(x, axis=-1, keepdims=True)
    xc = x - mu
    var = jnp.mean(xc * xc, axis=-1, keepdims=True)
    return mu, xc, jax.lax.rsqrt(var + EPS)


def make_kernel(NREL=2, DL=4,
                W0=(4, 10, 3), T0N=(2, 2, 4, 2), T0P=(1, 1, 0.5, 0.5, 1, 0.5), WA=(9, 10, 8, 7, 7, 6, 6), WP=(2.5, 1, 0.25, 1, 2, 6), X2AT=5, PR=16, X2S=(2, 9),
                X2F=((6, 9.5, 10.5), (7, 2, 3), (7, 4, 5), (7, 7, 8), (7, 9, 10), (7, 12, 13), (7, 13, 14), (7, 14, 15)),
                AQ=(2, 2, 13, 4), AA=(1, 38), AL=(2, 38), ADL=4,
                NOV=0, DSH=1, QKJ=True, PVW=2, C0=1, NPC=6, AFQ=(1, 1, 12, 3), AFP=(20, 15, 36, 38, 58, 60, 84, 0, 16), AFDL=5,
                BW=2, BQ=(1, 1, 20, 5), BA=(18, 170), BL=(20, 149), BCP=(8, 28), AFC=(66, 86), QT=4, ACN=(4, 2), BDL=6,
                MG=1, AFN=4, AFL=(0, 0), AN=4, ALS=(2, 4), BN=4, BLS=(2, 4), TMG=2, TN=4, TLS=(1, 3), scopes=False, only=None):

    def scope(name):
        return jax.named_scope(name) if scopes else contextlib.nullcontext()

    def kernel(x_hbm, wqkv_hbm, wo_hbm, w1_hbm, w3_hbm, w2_hbm, c_hbm, wm_hbm, out_hbm,
               x_v, wraw_v, wp_v, wo_v, w1_v, w3_v, w2_v, wmc_v, wmr_v,
               mod_v, scol_v, st_v, h1_v, qa_v, ka_v, va_v, qb_v, kb_v, vb_v, o_v, x1_v, h2_v, out_v,
               hc_v, hn_v, acc_v, z_v, c_v, sems, sem_out, bar):
        cp = pltpu.make_async_copy

        dmas = {}

        def add(name, src, dst):
            dmas[name] = cp(src, dst, sems.at[len(dmas)])

        def add_x(name, t0, n):
            add(name, x_hbm.at[pl.ds(t0 * TM, n * TM), :], x_v.at[pl.ds(t0 * TM, n * TM), :])

        add("c", c_hbm, c_v)
        add_x("x0", 0, 1)
        for k in range(NC):
            for m in (1, 0):
                add(f"m{m}{k}", wm_hbm.at[:, pl.ds(m * D + k * 128, 128)], wmc_v.at[m * NC + k])
            for m in range(3):
                add(f"w{m}{k}", wqkv_hbm.at[pl.ds(k * 128, 128), pl.ds(m * D, D)], wraw_v.at[m, pl.ds(k * 128, 128), :])
            if k == 0:
                add_x("x1", 1, 1)
            if k == X2AT:
                add_x("x2", 2, 1)
        add_x("xr", 3, NT - 3)
        add("wmr", wm_hbm.at[:, pl.ds(2 * D, 4 * D)], wmr_v)
        add("wo", wo_hbm, wo_v)
        add("fw1", w1_hbm, w1_v)
        add("fw3", w3_hbm, w3_v)
        add("fw2a", w2_hbm.at[pl.ds(0, C0 * HK), :], w2_v.at[pl.ds(0, C0 * HK), :])
        add("fw2b", w2_hbm.at[pl.ds(C0 * HK, F - C0 * HK), :], w2_v.at[pl.ds(C0 * HK, F - C0 * HK), :])
        for d in dmas.values():
            d.start()
            pl.semaphore_signal(bar, 1)
            pl.semaphore_wait(bar, 1)
        for j in range(NC):
            ka_v[j, 0:PAD, :] = jnp.zeros((PAD, 128), F32)
            va_v[j, 0:PAD, :] = jnp.zeros((PAD, 128), F32)
        add("z", ka_v.at[0, pl.ds(0, 8), :], z_v.at[pl.ds(0, 8), :])
        dmas["z"].start()

        def wait(*names):
            with scope("w_" + names[0]):
                for n in names:
                    dmas[n].wait()

        def zero():
            return pltpu.bitcast(z_v[0:8, :], U32)

        cur = {"nrel": NREL, "lns": (0, 0)}

        def mod_task(m, j, mg=2):
            src = wmc_v.at[m * NC + j] if m < 2 else wmr_v.at[:, pl.ds((m - 2) * D + j * 128, 128)]
            acc = None
            for kb in range(D // 128):
                if kb % mg == 0:
                    rel = yield
                p = src[kb * 128:(kb + 1) * 128, :].astype(F32) * scol_v[kb * 128:(kb + 1) * 128, :]
                parts = [p[r:r + 8] for r in range(0, 128, 8)]
                a0, a1 = parts[0], parts[1]
                if kb % mg == 0:
                    a0, a1 = _gate(a0, rel), _gate(a1, rel)
                for r in range(2, 16, 2):
                    a0, a1 = a0 + parts[r], a1 + parts[r + 1]
                a0 = a0 + a1
                acc = a0 if acc is None else acc + a0
            r = jnp.sum(acc, axis=0, keepdims=True)
            if m in (1, 4):
                r = r + 1.0
            mod_v[m:m + 1, j * 128:(j + 1) * 128] = r
            return pltpu.bitcast(jnp.broadcast_to(r, (8, 128)), U32)

        def modulate(xn, ms, dst, g, c0, c1):
            hb = _pack(xn * mod_v[ms + 1:ms + 2, c0:c1] + mod_v[ms:ms + 1, c0:c1])
            dst[g * 8:(g + 1) * 8, c0:c1] = hb
            return _or_all([hb])

        def ln_tail(xc, rs, ms, dst, g):
            ns, skip = cur["lns"]
            if ns == 0:
                return modulate(xc * rs, ms, dst, g, 0, D)
            for _ in range(skip):
                yield
            rs = jnp.broadcast_to(rs, (G, 128))
            toks = []
            cw = D // ns
            for p in range(ns):
                rel = yield
                r = jnp.tile(_gate(rs, rel), (1, cw // 128))
                toks.append(modulate(xc[:, p * cw:(p + 1) * cw] * r, ms, dst, g, p * cw, (p + 1) * cw))
            return _or_all(toks)

        def ln1_task(t, g, dst):
            rel = yield
            xt = x_v.at[_rows(t * TM, TM, TM), :]
            _, xc, rs = _stats(_gate(xt[g * G:(g + 1) * G, :].astype(F32), rel))
            return (yield from ln_tail(xc, rs, 0, dst, g))

        def stats_task(t, g):
            rel = yield
            rows = slice(t * TM + g * G, t * TM + (g + 1) * G)
            mu, _, rs = _stats(_gate(x_v[rows, :].astype(F32), rel))
            rs = jnp.broadcast_to(rs, (G, 128))
            st_v[0, rows, :] = jnp.broadcast_to(mu, (G, 128))
            st_v[1, rows, :] = rs
            return _or_all([pltpu.bitcast(rs, U32)]) if t == 2 else None

        def fin_task(t, k, g0, ng):
            rel = yield
            toks = []
            for g in range(g0, g0 + ng):
                rows = slice(t * TM + g * G, t * TM + (g + 1) * G)
                x = _gate(x_v[rows, k * 128:(k + 1) * 128].astype(F32), rel)
                xn = (x - st_v[0, rows, :]) * st_v[1, rows, :]
                toks.append(modulate(xn, 0, h1_v.at[t] if t < 2 else hc_v, g, k * 128, (k + 1) * 128))
            return _or_all(toks) if t == 2 else None

        def ln2_task(t, g, dst):
            rel = yield
            xv = x1_v.at[:, _rows(t * TM, TM, TM), :]
            x = jnp.concatenate([_gate(xv[j, g * G:(g + 1) * G, :], rel) for j in range(NC)], axis=1)
            _, xc, rs = _stats(x)
            return (yield from ln_tail(xc, rs, 3, dst, g))

        def perm_select_task(m, r0, n):
            rel = yield
            xs = [_gate(pltpu.bitcast(wraw_v[m, r0:r0 + n, j * 128:(j + 1) * 128], U32), rel) for j in range(NC)]
            zs = _xor_network(xs)
            for j in range(NC):
                wp_v[r0 // 2:(r0 + n) // 2, m * D + j * 128:m * D + (j + 1) * 128] = zs[j]

        def perm_gather_task(m, j, r0, n):
            rel = yield
            sl = (slice(r0 // 2, (r0 + n) // 2), slice(m * D + j * 128, m * D + (j + 1) * 128))
            wp_v[sl] = _gather_fwd(_gate(wp_v[sl], rel), j)

        def copy_task(src, dst, r0, nr, c0, c1):
            rel = yield
            dst[r0:r0 + nr, c0:c1] = _gate(src[r0:r0 + nr, c0:c1], rel)

        def halo_task():
            yield
            for j in range(NC):
                kb_v[j, 0:PAD, :] = ka_v[j, SA:SA + PAD, :]
                vb_v[j, 0:PAD, :] = va_v[j, SA:SA + PAD, :]

        def attn_task(first, base, span, g, pace, masked=False):
            qkg, pvg, skip, smd = pace
            q_v, k_v, v_v = (qa_v, ka_v, va_v) if first else (qb_v, kb_v, vb_v)
            qv = q_v.at[:, _rows(base, span, 32), :]
            kv = k_v.at[:, _rows(base, span + PAD, 32), :]
            vv = v_v.at[:, _rows(base, span + PAD, 32), :]

            def shifted(ref, j, w):
                return ref[j, pl.ds(g * G + PAD - DIL * w, G), :]

            if QKJ:
                ls = [None] * WIN
                for j in range(NC):
                    if j % qkg == 0:
                        rel = yield
                    q = _gate(qv[j, g * G:(g + 1) * G, :], rel)
                    for w in range(WIN):
                        p = q * shifted(kv, j, w)
                        ls[w] = p if j == 0 else ls[w] + p
            else:
                q = [qv[j, g * G:(g + 1) * G, :] for j in range(NC)]
                ls = []
                for w in range(WIN):
                    if w % qkg == 0:
                        rel = yield
                    acc = _gate(q[0], rel) * shifted(kv, 0, w)
                    for j in range(1, NC):
                        acc = acc + q[j] * shifted(kv, j, w)
                    ls.append(acc)
            ls = [l + pltpu.roll(l, 64, 1) for l in ls]
            ls = [l + pltpu.roll(l, 32, 1) for l in ls]
            if masked:
                rows = base + g * G + jax.lax.broadcasted_iota(jnp.int32, (G, 128), 0)
                ls = [ls[0]] + [jnp.where(rows >= DIL * w, ls[w], MASKED) for w in range(1, WIN)]
            mx = ls[0]
            for w in range(1, WIN):
                mx = jnp.maximum(mx, ls[w])
            ps = [jnp.exp2((l - mx) * EXP2_C) for l in ls]
            den = ps[0]
            for w in range(1, WIN):
                den = den + ps[w]
            inv = 1.0 / den
            ps = [pw * inv for pw in ps]
            if smd:
                yield _or_all([pltpu.bitcast(ps[0], U32)]), smd
            for _ in range(skip - (1 if smd else 0)):
                yield
            zs = []
            if PVW == 1:
                os_ = [None] * NC
                for w in range(WIN):
                    if w % pvg == 0:
                        rel = yield
                    p = _gate(ps[w], rel)
                    for j in range(NC):
                        pv = p * shifted(vv, j, w)
                        os_[j] = pv if w == 0 else os_[j] + pv
                for j in range(NC):
                    if j % 4 == 0:
                        rel = yield
                    zs.append(_gather_inv(_pack(_gate(os_[j], rel)), j))
            else:
                for j in range(NC):
                    if j % pvg == 0:
                        rel = yield
                        pg = [_gate(p, rel) for p in ps] if PVW == 2 else [_gate(ps[0], rel)] + ps[1:]
                    acc = pg[0] * shifted(vv, j, 0)
                    for w in range(1, WIN):
                        acc = acc + pg[w] * shifted(vv, j, w)
                    zs.append(_gather_inv(_pack(acc), j))
            xs = _xor_network(zs)
            half = (base // 2 if isinstance(base, int) else jax.lax.shift_right_logical(base, 1)) + (0 if first else SA // 2)
            ov = o_v.at[_rows(half, span // 2, 16), :]
            for j in range(NC):
                ov[g * 8:(g + 1) * 8, j * 128:(j + 1) * 128] = xs[j]
            return _or_all(xs)

        def LN1(t, dst):
            return [ln1_task(t, g, dst) for g in range(NG)]

        def LN2(t, dst):
            return [ln2_task(t, g, dst) for g in range(NG)]

        def STATS(t):
            return [stats_task(t, g) for g in range(NG)]

        def FIN(t, k):
            return [fin_task(t, k, g0, 4) for g0 in range(0, NG, 4)]

        def MOD(m, j0=0, j1=NC, mg=2):
            return [mod_task(m, j, mg) for j in range(j0, j1)]

        def PERM(m, k):
            r0 = k * 128
            return ([perm_select_task(m, r, PR) for r in range(r0, r0 + 128, PR)]
                    + [perm_gather_task(m, j, r0, 128) for j in range(NC)])

        def COPY(src, dst, n, lo, hi, pre, c0=0, c1=D):
            nr = TM // 2 // n
            return ([copy_task(src, dst, r, nr, c0, c1) for r in range(0, TM // 2, nr)], lo, hi, pre)

        def run_now(tasks):
            for tk in tasks:
                try:
                    next(tk)
                    while True:
                        tk.send(None)
                except StopIteration:
                    pass

        def tie(a, tok):
            if tok is not None:
                top = a[0:8, 0:128] | (tok & zero())
                if a.shape[1] > 128:
                    top = jnp.concatenate([top, a[0:8, 128:]], axis=1)
                a = jnp.concatenate([top, a[8:]], axis=0)
            return pltpu.bitcast(a, BF16)


        def releases(res):
            return [pltpu.bitcast(res[r:r + 8, 0:128], U32) & zero() for r in range(0, TM, TM // cur["nrel"])]

        def wave_pass(k, t, nb, tok):
            m, j0 = nb // 2, (nb % 2) * 4
            dst = (qa_v, ka_v, va_v)[m]
            rows = slice(t * TM + (PAD if m else 0), (t + 1) * TM + (PAD if m else 0))
            w = pltpu.bitcast(wp_v[k * 64:(k + 1) * 64, nb * 512:(nb + 1) * 512], BF16)
            res = jnp.dot(tie(h1_v[t, :, k * 128:(k + 1) * 128], tok), w, preferred_element_type=F32)
            for jj in range(4):
                r = res[:, jj * 128:(jj + 1) * 128]
                if k > 0:
                    r = dst[j0 + jj, rows, :] + r
                dst[j0 + jj, rows, :] = r
            return releases(res)

        def qkv_pass(t, m, j, hf, st, tok):
            w = pltpu.bitcast(wp_v[hf * HK // 2:(hf + 1) * HK // 2, m * D + j * 128:m * D + (j + 1) * 128], BF16)
            res = jnp.dot(tie(hc_v[:, hf * HK:(hf + 1) * HK], tok), w, preferred_element_type=F32)
            if hf == 0:
                st[m, j] = res
            else:
                res = st.pop((m, j)) + res
                off = PAD if m else 0
                dst = (qb_v, kb_v, vb_v)[m].at[:, _rows((t - 2) * TM, TM + off, TM), :]
                dst[j, off:off + TM, :] = res
            return releases(res)

        def wo_pass(t, j, hf, st, tok):
            h = tie(o_v[_rows(t * (TM // 2), TM // 2, TM // 2), hf * HK:(hf + 1) * HK], tok)
            res = jnp.dot(h, wo_v[hf * HK:(hf + 1) * HK, j * 128:(j + 1) * 128], preferred_element_type=F32)
            if hf == 0:
                st["a"] = res
            else:
                rows, cs = _rows(t * TM, TM, TM), slice(j * 128, (j + 1) * 128)
                res = x_v[rows, cs].astype(F32) + mod_v[2:3, cs] * (st.pop("a") + res)
                x1_v[j, rows, :] = res
            return releases(res)

        def out_copy(t, j):
            rows = _rows(t * TM, TM, TM)
            return cp(out_v.at[j, rows, :], out_hbm.at[rows, pl.ds(j * 128, 128)], sem_out.at[t])

        def out_wait(t):
            if only is not None and ("FL" if t == NT - 1 else "F") not in only:
                return
            rows = pl.ds(t * TM, TM)
            cp(out_hbm.at[rows, :], out_hbm.at[rows, :], sem_out.at[t]).wait()

        def WAVE(k):
            return [functools.partial(wave_pass, k, t, nb) for m in range(3) for t in range(2) for nb in (2 * m, 2 * m + 1)]

        def QKV(t):
            order = [(m, j, hf) for m in range(3) for j in range(NC) for hf in range(2)]
            order = order[:-2 * QT] + order[-2 * QT::2] + order[-2 * QT + 1::2]
            st = {}
            return [functools.partial(qkv_pass, t, m, j, hf, st) for m, j, hf in order]

        def WO(t):
            st = {}
            return [functools.partial(wo_pass, t, j, hf, st) for j in range(NC) for hf in range(2)]

        def FFN(t, c0, c1):
            st = {"acc": [None] * NC, "act": []}
            h_v = hn_v if c0 == 0 else h2_v

            def gate_up_pass(which, n, hf, tok):
                w = (w1_v, w3_v)[which][hf * HK:(hf + 1) * HK, n * 128:(n + 1) * 128]
                res = jnp.dot(tie(h_v[:, hf * HK:(hf + 1) * HK], tok), w, preferred_element_type=F32)
                if hf == 0:
                    st["a"] = res
                else:
                    res = st.pop("a") + res
                    if which == 0:
                        hg = 0.5 * res
                        st["g"] = hg + hg * jnp.tanh(hg)
                    else:
                        st["act"].append((st.pop("g") * res).astype(BF16))
                return releases(res)

            def down_pass(c, j, last, tok):
                if j == 0:
                    st["lhs"], st["act"] = jnp.concatenate(st["act"], axis=1), []
                w = w2_v[c * HK:(c + 1) * HK, j * 128:(j + 1) * 128]
                if tok is not None:
                    w = tie(pltpu.bitcast(w, U32), tok)
                res = jnp.dot(st["lhs"], w, preferred_element_type=F32)
                if c > 0:
                    res = (acc_v[j] if c == c0 else st["acc"][j]) + res
                st["acc"][j] = res
                if c == c1 - 1 and not last:
                    acc_v[j] = res
                if last:
                    rows = _rows(t * TM, TM, TM)
                    out_v[j, rows, :] = (x1_v[j, rows, :] + mod_v[5:6, j * 128:(j + 1) * 128] * res).astype(BF16)
                    out_copy(t, j).start()
                return releases(res)

            out = []
            nch = F // HK
            for c in range(c0, c1):
                for n in range(c * 4, c * 4 + 4):
                    out += [functools.partial(gate_up_pass, which, n, hf) for which in range(2) for hf in range(2)]
                out += [functools.partial(down_pass, c, j, c == nch - 1) for j in range(NC)]
            return out

        def segment(name, passes, groups=(), dl=DL, need=None, nrel=NREL, lns=(0, 0)):
            if only is not None and name not in only:
                return
            with scope(name):
                n = len(passes)
                cur["nrel"], cur["lns"] = nrel, lns
                active = []
                for tasks, lo, hi, *pre in groups:
                    for k, tk in enumerate(tasks):
                        active.append((int((lo + k * (hi - lo) / len(tasks)) * nrel), tk, pre[0] if pre else ()))
                        next(tk)
                deadlines = [[] for _ in range(n + dl + 8)]

                def due(p):
                    return p + DSH if p < n and passes[p].func.__name__ == "down_pass" else p

                def done(tasks):
                    return all(ent[1] is not tk for tk in tasks for ent in active)

                def feed(rel, slot, i):
                    for ent in list(active):
                        if ent[0] <= slot:
                            assert done(ent[2]), (name, i)
                            try:
                                mid = ent[1].send(rel)
                                if mid is not None:
                                    deadlines[due(i + mid[1])].append(mid[0])
                            except StopIteration as e:
                                if e.value is not None:
                                    deadlines[due(i + dl)].append(e.value)
                                active.remove(ent)

                feed(None, 0, 0)
                slot = 1
                for i, ps in enumerate(passes):
                    assert done((need or {}).get(i, ())), (name, i)
                    for rel in ps(_or_all(deadlines[i]) if deadlines[i] else None):
                        feed(rel, slot, i)
                        slot += 1
                while active:
                    feed(None, 1 << 30, n)

        with scope("S0"):
            wait("c", "z")
            c = c_v[...].astype(F32)
            s = (c * jax.nn.sigmoid(c)).astype(BF16).astype(F32)
            eye = (jax.lax.broadcasted_iota(jnp.int32, (128, 128), 0)
                   == jax.lax.broadcasted_iota(jnp.int32, (128, 128), 1))
            ones = jnp.ones((128, 128), BF16)
            for j in range(NC):
                dg = jnp.where(eye, jnp.broadcast_to(s[:, j * 128:(j + 1) * 128], (128, 128)), 0.0).astype(BF16)
                scol_v[j * 128:(j + 1) * 128, :] = jnp.dot(dg, ones, preferred_element_type=F32)
            wait("x0")
            run_now(STATS(0))
            wait("m10", "m00")
            run_now(MOD(1, 0, 1) + MOD(0, 0, 1) + FIN(0, 0))
            wait("w00")
            run_now(PERM(0, 0))
            wait("w10", "w20")

        m0 = [functools.partial(wave_pass, 0, t, nb) for t in range(2) for nb in range(6)]
        m1 = WAVE(1)
        n0, n1, n2 = W0
        p1, p2 = PERM(1, 0), PERM(2, 0)
        segment("T0a", m0[:n0], [(p1, 0, T0P[0]), (p2, T0P[0], n0 - 0.5)], need={2: p1}, nrel=T0N[0])
        wait("x1")
        s1, f1, u = STATS(1), FIN(1, 0), 6 - n0
        segment("T0b", m0[n0:n1], [(s1, 0, max(0.2, u - T0P[1])), (f1, u - T0P[2], u - 0.01, s1)], need={u: s1 + f1},
                nrel=T0N[1])
        wait("m11", "m01", "w01")
        mods, f0, f1, pq, u = MOD(1, 1, 2) + MOD(0, 1, 2), FIN(0, 1), FIN(1, 1), PERM(0, 1), 12 - n1
        fmin = max(3 / T0N[2], u - T0P[3])
        segment("T0c", m0[n1:] + m1[:n2],
                [(mods, 0, 0.2), (f0, fmin, u - 0.01, mods), (f1, u, u + 1, mods), (pq, 0, max(0.5, u - T0P[4]))],
                need={u: mods + f0 + pq, u + 2: f1}, nrel=T0N[2])
        wait("w11", "w21")
        p1, p2 = PERM(1, 1), PERM(2, 1)
        e1 = max(0.5, 4 - n2 - T0P[5])
        segment("T1", m1[n2:WA[1]], [(p1, 0, e1), (p2, e1, 8 - n2 - 1.5)], need={4 - n2: p1, 8 - n2: p2}, nrel=T0N[3])
        for k in range(2, NC):
            last = k == NC - 1
            wait(f"m1{k}", f"m0{k}", f"w0{k}", f"w1{k}", f"w2{k}", *(["x2"] if k == X2AT + 1 else []))
            u = 12 - WA[k - 1]
            mods = MOD(1, k, k + 1, TMG) + MOD(0, k, k + 1, TMG)
            fins = [FIN(t, k) for t in range(2)]
            perms = [PERM(m, k) for m in range(3)]
            mend = max(0.5, u - WP[0])
            fmin = (8 // TMG - 1) / TN + (mend - 0.5 if mend > 2 else 0)
            groups = [(mods[:1], 0, 1), (mods[1:], mend - 0.5 if mend > 2 else 0, mend),
                      (fins[0], max(fmin, u - WP[1]), max(fmin + 0.2, u - WP[2]), mods), (fins[1], max(fmin + 0.2, u - WP[2]), u + 1, mods),
                      (perms[0], 0, max(0.9, u - WP[3])), (perms[1], max(0.9, u - WP[3]), u + WP[4]), (perms[2], u + WP[4], u + WP[5])]
            if k == X2AT + 1:
                s2 = STATS(2)
                groups.append((s2, *X2S))
            for kk in range(NC):
                if X2F[kk][0] == k:
                    assert kk <= k
                    groups.append((FIN(2, kk), *X2F[kk][1:], (s2 if k == X2AT + 1 else []) + (mods if kk == k else [])))
            segment(f"T{k}", WAVE(k - 1)[WA[k - 1]:] + (WAVE(k) if last else WAVE(k)[:WA[k]]), groups,
                    need={u: mods + fins[0] + perms[0], u + 2: fins[1], u + 4: perms[1], u + 8: perms[2]}, nrel=TN, lns=TLS)
        wait("xr")

        def a_step(t, carry):
            base = jnp.minimum((t - 2) * (NPC // 2), NG) * (2 * G)
            att = [attn_task(True, base, NPC * G, g, AQ, masked=(g == 0)) for g in range(NPC)]
            l1 = LN1(t + 1, hn_v)
            segment("A", QKV(t), [(att, *AA), (l1, *AL), COPY(hn_v, hc_v, ACN[0], 48 - QT, 47, l1, 0, HK),
                                 COPY(hn_v, hc_v, ACN[1], 47 + 1 / AN, 48 + 1 / AN, l1, HK, D)], dl=ADL, nrel=AN, lns=ALS)
            return carry

        with scope("loopA"):
            jax.lax.fori_loop(2, NT - 1, a_step, 0)
        wait("wmr", "wo", "fw1", "fw3", "fw2a")
        q7, nq = QKV(NT - 1), AFP[0]
        mg, msc, l2 = MOD(2, mg=MG), MOD(3, mg=MG) + MOD(4, mg=MG), LN2(0, hn_v)
        done_rows = (NT - 3) * NPC * G
        att = [attn_task(True, done_rows, SA - done_rows, g, AFQ) for g in range((SA - done_rows) // G)]
        segment("AF", q7[:nq] + WO(0) + q7[nq:] + FFN(0, 0, C0),
                [(mg, 0, AFP[1]), (msc, AFP[1], AFP[2]), (l2, max(AFP[3], nq + 16), AFP[4], msc),
                 (MOD(5, mg=MG), AFP[5], AFP[6]), (att, AFP[7], AFP[8]), ([halo_task()], 1, 2)]
                + [COPY(hn_v, h2_v, 16, *AFC, l2)], need={nq: mg, 64: l2}, dl=AFDL, nrel=AFN, lns=AFL)
        wait("fw2b")

        nch = F // HK
        nf = (nch - C0) * 24

        def b_step(i, carry):
            att = [attn_task(False, jnp.minimum(i, NT - 3) * TM, TM, g, BQ) for g in range(NG)]
            l2 = LN2(i + 1, hn_v)
            ffn = FFN(i, C0, nch)
            cpy = [COPY(hn_v, h2_v, 16, nf + 16 - 8 + BCP[0], nf + 16 - 8 + BCP[1], l2)]
            assert BA[0] >= 16 + BW and BL[0] >= 16 + BW and min(BCP) >= 0
            segment("F", ffn[:BW] + WO(i + 1) + ffn[BW:] + FFN(i + 1, 0, C0), ([(att, *BA)] if NOV < 1 else []) + ([(l2, *BL)] + cpy if NOV < 2 else []),
                    need={nf + 16: l2}, dl=BDL, nrel=BN, lns=BLS)
            return carry

        with scope("B"):
            jax.lax.fori_loop(0, NT - 1, b_step, 0)
        for t in range(NT - 2):
            out_wait(t)
        segment("FL", FFN(NT - 1, C0, nch))
        with scope("fin"):
            for t in range(NT - 2, NT):
                out_wait(t)

    @jax.jit
    def fn(A_x, A_wqkv, A_wo, B_x, B_w1, B_w3, B_w2, c, w_mod):
        V = pltpu.VMEM
        scratch = [
            V((S, D), BF16), V((3, D, D), BF16), V((D // 2, 3 * D), U32), V((D, D), BF16),
            V((D, F), BF16), V((D, F), BF16), V((F, D), BF16), V((2 * NC, D, 128), BF16), V((D, 4 * D), BF16),
            V((8, D), F32), V((D, 128), F32), V((2, SA + TM, 128), F32), V((2, TM // 2, D), U32),
            V((NC, SA, 128), F32), V((NC, PAD + SA, 128), F32), V((NC, PAD + SA, 128), F32),
            V((NC, SB, 128), F32), V((NC, PAD + SB, 128), F32), V((NC, PAD + SB, 128), F32),
            V((S // 2, D), U32), V((NC, S, 128), F32), V((TM // 2, D), U32), V((NC, S, 128), BF16),
            V((TM // 2, D), U32), V((TM // 2, D), U32), V((NC, TM, 128), F32), V((32, 128), F32), V((1, D), BF16),
            pltpu.SemaphoreType.DMA((5 * NC + 12,)), pltpu.SemaphoreType.DMA((NT,)), pltpu.SemaphoreType.REGULAR,
        ]
        out = pl.pallas_call(
            kernel,
            in_specs=[pl.BlockSpec(memory_space=pl.ANY)] * 8,
            out_specs=pl.BlockSpec(memory_space=pl.ANY),
            out_shape=jax.ShapeDtypeStruct((S, D), BF16),
            scratch_shapes=scratch,
            compiler_params=pltpu.CompilerParams(vmem_limit_bytes=124 * 1024 * 1024, disable_bounds_checks=True,
                                                 disable_semaphore_checks=True),
        )(A_x.reshape(S, D), A_wqkv, A_wo, B_w1, B_w3, B_w2, c, w_mod)
        return out.reshape(1, S, D)

    return fn


_impl = make_kernel()


@jax.jit
def pallas_adaLN_cond__sliding_local_dilated__glu_gated_swiglu__prompt_kernel(A_x, A_wqkv, A_wo, B_x, B_w1, B_w3, B_w2, c, w_mod):
    return _impl(A_x, A_wqkv, A_wo, B_x, B_w1, B_w3, B_w2, c, w_mod)
```

```python
import contextlib
import functools
import math

import jax
import jax.numpy as jnp
import jax.experimental.pallas as pl
import jax.experimental.pallas.tpu as pltpu

S, D, F = 2048, 1024, 3584
DH, WIN, DIL = 32, 8, 2
NC = D // 128
PAD = 16
EPS = 1e-5
SCALE = DH ** -0.5
EXP2_C = SCALE * math.log2(math.e)
MASKED = -1e9 / SCALE
F32, BF16, U32 = jnp.float32, jnp.bfloat16, jnp.uint32
TM = 256
NT = S // TM
G = 16
NG = TM // G
HK = D // 2
SA = 2 * TM
SB = S - SA


def _xor_network(xs):
    lane = jax.lax.broadcasted_iota(jnp.int32, xs[0].shape, 1)
    for b in range(3):
        m = ((lane >> (2 + b)) & 1) == 1
        xs = [jnp.where(m, xs[i ^ (1 << b)], xs[i]) for i in range(NC)]
    return xs


def _gather_fwd(z, j):
    lane = jax.lax.broadcasted_iota(jnp.int32, z.shape, 1)
    e, g, p = lane >> 5, (lane >> 3) & 3, lane & 7
    return jnp.take_along_axis(z, g * 32 + (p ^ j) * 4 + e, axis=1)


def _gather_inv(y, j):
    lane = jax.lax.broadcasted_iota(jnp.int32, y.shape, 1)
    g, q, e = lane >> 5, (lane >> 2) & 7, lane & 3
    return jnp.take_along_axis(y, e * 32 + g * 8 + (q ^ j), axis=1)


def _pack(x):
    return pltpu.bitcast(x.astype(BF16), U32)


def _or_all(vs):
    parts = [v[r:r + 8, c:c + 128] for v in vs for r in range(0, v.shape[0], 8) for c in range(0, v.shape[1], 128)]
    while len(parts) > 1:
        parts = [parts[i] | parts[i + 1] if i + 1 < len(parts) else parts[i] for i in range(0, len(parts), 2)]
    return parts[0]


def _gate(x, g):
    if g is None:
        return x
    xb = x if x.dtype == U32 else pltpu.bitcast(x, U32)
    y = xb | jnp.tile(g, (x.shape[0] // 8, x.shape[1] // 128))
    return y if x.dtype == U32 else pltpu.bitcast(y, x.dtype)


def _rows(start, n, mult):
    if isinstance(start, int):
        return pl.ds(start, n)
    return pl.ds(pl.multiple_of(start, mult), n)


def _stats(x):
    mu = jnp.mean(x, axis=-1, keepdims=True)
    xc = x - mu
    var = jnp.mean(xc * xc, axis=-1, keepdims=True)
    return mu, xc, jax.lax.rsqrt(var + EPS)


def make_kernel(NREL=2, DL=4,
                W0=(4, 10, 3), T0N=(2, 2, 4, 2), T0P=(1, 1, 0.5, 0.5, 1, 0.5), WA=(9, 10, 8, 7, 7, 6, 6), WP=(2.5, 1, 0.25, 1, 2, 6), ND=2, SAT=(4, 5), SBP=(2, 3.5, 5, 9), X2AT=5, PR=16, X2S=(2, 9),
                X2F=((6, 9.5, 10.5), (7, 2, 3), (7, 4, 5), (7, 7, 8), (7, 9, 10), (7, 12, 13), (7, 13, 14), (7, 14, 15)),
                AQ=(2, 2, 13, 4), AA=(1, 38), AL=(2, 38), ADL=4,
                NOV=0, DSH=1, QKJ=True, PVW=2, C0=1, NPC=6, AFQ=(1, 1, 12, 3), AFP=(20, 15, 36, 38, 58, 60, 84, 0, 16), AFDL=5,
                BW=2, BQ=(1, 1, 20, 5), BA=(18, 170), BL=(20, 149), BCP=(8, 28), AFC=(66, 86), QT=4, ACN=(4, 2), BDL=6,
                MG=1, AFN=4, AFL=(0, 0), AN=4, ALS=(2, 4), BN=4, BLS=(2, 4), TMG=2, TN=4, TLS=(1, 3), scopes=False, only=None):

    def scope(name):
        return jax.named_scope(name) if scopes else contextlib.nullcontext()

    def kernel(x_hbm, wqkv_hbm, wo_hbm, w1_hbm, w3_hbm, w2_hbm, c_hbm, wm_hbm, out_hbm,
               x_v, wraw_v, wp_v, wo_v, w1_v, w3_v, w2_v, wmc_v, wmr_v,
               mod_v, scol_v, st_v, h1_v, qa_v, ka_v, va_v, qb_v, kb_v, vb_v, o_v, x1_v, h2_v, out_v,
               hc_v, hn_v, acc_v, sac_v, bias_v, z_v, c_v, sems, sem_out, bar):
        cp = pltpu.make_async_copy

        dmas = {}

        def add(name, src, dst):
            dmas[name] = cp(src, dst, sems.at[len(dmas)])

        def add_x(name, t0, n):
            add(name, x_hbm.at[pl.ds(t0 * TM, n * TM), :], x_v.at[pl.ds(t0 * TM, n * TM), :])

        add("c", c_hbm, c_v)
        add_x("x0", 0, 1)
        for k in range(NC):
            for m, kk in [(1, k)] + ([(0, k)] if k >= ND else []):
                add(f"m{m}{kk}", wm_hbm.at[:, pl.ds(m * D + kk * 128, 128)], wmc_v.at[m * NC + kk])
            for m in range(3):
                add(f"w{m}{k}", wqkv_hbm.at[pl.ds(k * 128, 128), pl.ds(m * D, D)], wraw_v.at[m, pl.ds(k * 128, 128), :])
            if k == 0:
                add_x("x1", 1, 1)
            for kk in range(ND):
                if SAT[kk] - 1 == k:
                    add(f"m0{kk}", wm_hbm.at[:, pl.ds(kk * 128, 128)], wmc_v.at[kk])
            if k == X2AT:
                add_x("x2", 2, 1)
        add_x("xr", 3, NT - 3)
        add("wmr", wm_hbm.at[:, pl.ds(2 * D, 4 * D)], wmr_v)
        add("wo", wo_hbm, wo_v)
        add("fw1", w1_hbm, w1_v)
        add("fw3", w3_hbm, w3_v)
        add("fw2a", w2_hbm.at[pl.ds(0, C0 * HK), :], w2_v.at[pl.ds(0, C0 * HK), :])
        add("fw2b", w2_hbm.at[pl.ds(C0 * HK, F - C0 * HK), :], w2_v.at[pl.ds(C0 * HK, F - C0 * HK), :])
        for d in dmas.values():
            d.start()
            pl.semaphore_signal(bar, 1)
            pl.semaphore_wait(bar, 1)
        for j in range(NC):
            ka_v[j, 0:PAD, :] = jnp.zeros((PAD, 128), F32)
            va_v[j, 0:PAD, :] = jnp.zeros((PAD, 128), F32)
        add("z", ka_v.at[0, pl.ds(0, 8), :], z_v.at[pl.ds(0, 8), :])
        dmas["z"].start()

        def wait(*names):
            with scope("w_" + names[0]):
                for n in names:
                    dmas[n].wait()

        def zero():
            return pltpu.bitcast(z_v[0:8, :], U32)

        cur = {"nrel": NREL, "lns": (0, 0)}

        def mod_task(m, j, mg=2):
            src = wmc_v.at[m * NC + j] if m < 2 else wmr_v.at[:, pl.ds((m - 2) * D + j * 128, 128)]
            acc = None
            for kb in range(D // 128):
                if kb % mg == 0:
                    rel = yield
                p = src[kb * 128:(kb + 1) * 128, :].astype(F32) * scol_v[kb * 128:(kb + 1) * 128, :]
                parts = [p[r:r + 8] for r in range(0, 128, 8)]
                a0, a1 = parts[0], parts[1]
                if kb % mg == 0:
                    a0, a1 = _gate(a0, rel), _gate(a1, rel)
                for r in range(2, 16, 2):
                    a0, a1 = a0 + parts[r], a1 + parts[r + 1]
                a0 = a0 + a1
                acc = a0 if acc is None else acc + a0
            r = jnp.sum(acc, axis=0, keepdims=True)
            if m in (1, 4):
                r = r + 1.0
            mod_v[m:m + 1, j * 128:(j + 1) * 128] = r
            return pltpu.bitcast(jnp.broadcast_to(r, (8, 128)), U32)

        def modulate(xn, ms, dst, g, c0, c1, shift=True):
            h = xn * mod_v[ms + 1:ms + 2, c0:c1]
            hb = _pack(h + mod_v[ms:ms + 1, c0:c1] if shift else h)
            dst[g * 8:(g + 1) * 8, c0:c1] = hb
            return _or_all([hb])

        def ln_tail(xc, rs, ms, dst, g):
            ns, skip = cur["lns"]
            if ns == 0:
                return modulate(xc * rs, ms, dst, g, 0, D)
            for _ in range(skip):
                yield
            rs = jnp.broadcast_to(rs, (G, 128))
            toks = []
            cw = D // ns
            for p in range(ns):
                rel = yield
                r = jnp.tile(_gate(rs, rel), (1, cw // 128))
                toks.append(modulate(xc[:, p * cw:(p + 1) * cw] * r, ms, dst, g, p * cw, (p + 1) * cw))
            return _or_all(toks)

        def ln1_task(t, g, dst):
            rel = yield
            xt = x_v.at[_rows(t * TM, TM, TM), :]
            _, xc, rs = _stats(_gate(xt[g * G:(g + 1) * G, :].astype(F32), rel))
            return (yield from ln_tail(xc, rs, 0, dst, g))

        def stats_task(t, g):
            rel = yield
            rows = slice(t * TM + g * G, t * TM + (g + 1) * G)
            mu, _, rs = _stats(_gate(x_v[rows, :].astype(F32), rel))
            rs = jnp.broadcast_to(rs, (G, 128))
            st_v[0, rows, :] = jnp.broadcast_to(mu, (G, 128))
            st_v[1, rows, :] = rs
            return _or_all([pltpu.bitcast(rs, U32)]) if t == 2 else None

        def fin_task(t, k, g0, ng):
            rel = yield
            toks = []
            for g in range(g0, g0 + ng):
                rows = slice(t * TM + g * G, t * TM + (g + 1) * G)
                x = _gate(x_v[rows, k * 128:(k + 1) * 128].astype(F32), rel)
                xn = (x - st_v[0, rows, :]) * st_v[1, rows, :]
                toks.append(modulate(xn, 0, h1_v.at[t] if t < 2 else hc_v, g, k * 128, (k + 1) * 128, t == 2 or k >= ND))
            return _or_all(toks) if t == 2 else None

        def ln2_task(t, g, dst):
            rel = yield
            xv = x1_v.at[:, _rows(t * TM, TM, TM), :]
            x = jnp.concatenate([_gate(xv[j, g * G:(g + 1) * G, :], rel) for j in range(NC)], axis=1)
            _, xc, rs = _stats(x)
            return (yield from ln_tail(xc, rs, 3, dst, g))

        def perm_select_task(m, r0, n):
            rel = yield
            xs = [_gate(pltpu.bitcast(wraw_v[m, r0:r0 + n, j * 128:(j + 1) * 128], U32), rel) for j in range(NC)]
            zs = _xor_network(xs)
            for j in range(NC):
                wp_v[r0 // 2:(r0 + n) // 2, m * D + j * 128:m * D + (j + 1) * 128] = zs[j]

        def perm_gather_task(m, j, r0, n):
            rel = yield
            sl = (slice(r0 // 2, (r0 + n) // 2), slice(m * D + j * 128, m * D + (j + 1) * 128))
            wp_v[sl] = _gather_fwd(_gate(wp_v[sl], rel), j)

        def shift_col_task(k):
            rel = yield
            row = _gate(jnp.broadcast_to(mod_v[0:1, k * 128:(k + 1) * 128], (128, 128)), rel)
            sac_v[...] = row.T

        def bias_task(k, c):
            rel = yield
            cs = slice(c * 128, (c + 1) * 128)
            w = pltpu.bitcast(_gate(wp_v[k * 64:(k + 1) * 64, cs], rel), BF16).astype(F32) * sac_v[...]
            parts = [w[r:r + 8] for r in range(0, 128, 8)]
            while len(parts) > 1:
                parts = [parts[i] + parts[i + 1] for i in range(0, len(parts), 2)]
            acc = parts[0] if k == 0 else bias_v[:, cs] + parts[0]
            if k == ND - 1:
                acc = jnp.broadcast_to(jnp.sum(acc, axis=0, keepdims=True), (8, 128))
            bias_v[:, cs] = acc
            return pltpu.bitcast(acc, U32)

        def copy_task(src, dst, r0, nr, c0, c1):
            rel = yield
            dst[r0:r0 + nr, c0:c1] = _gate(src[r0:r0 + nr, c0:c1], rel)

        def halo_task():
            yield
            for j in range(NC):
                kb_v[j, 0:PAD, :] = ka_v[j, SA:SA + PAD, :]
                vb_v[j, 0:PAD, :] = va_v[j, SA:SA + PAD, :]

        def attn_task(first, base, span, g, pace, masked=False):
            qkg, pvg, skip, smd = pace
            q_v, k_v, v_v = (qa_v, ka_v, va_v) if first else (qb_v, kb_v, vb_v)
            qv = q_v.at[:, _rows(base, span, 32), :]
            kv = k_v.at[:, _rows(base, span + PAD, 32), :]
            vv = v_v.at[:, _rows(base, span + PAD, 32), :]

            def shifted(ref, j, w):
                return ref[j, pl.ds(g * G + PAD - DIL * w, G), :]

            if QKJ:
                ls = [None] * WIN
                for j in range(NC):
                    if j % qkg == 0:
                        rel = yield
                    q = _gate(qv[j, g * G:(g + 1) * G, :], rel)
                    for w in range(WIN):
                        p = q * shifted(kv, j, w)
                        ls[w] = p if j == 0 else ls[w] + p
            else:
                q = [qv[j, g * G:(g + 1) * G, :] for j in range(NC)]
                ls = []
                for w in range(WIN):
                    if w % qkg == 0:
                        rel = yield
                    acc = _gate(q[0], rel) * shifted(kv, 0, w)
                    for j in range(1, NC):
                        acc = acc + q[j] * shifted(kv, j, w)
                    ls.append(acc)
            ls = [l + pltpu.roll(l, 64, 1) for l in ls]
            ls = [l + pltpu.roll(l, 32, 1) for l in ls]
            if masked:
                rows = base + g * G + jax.lax.broadcasted_iota(jnp.int32, (G, 128), 0)
                ls = [ls[0]] + [jnp.where(rows >= DIL * w, ls[w], MASKED) for w in range(1, WIN)]
            mx = ls[0]
            for w in range(1, WIN):
                mx = jnp.maximum(mx, ls[w])
            ps = [jnp.exp2((l - mx) * EXP2_C) for l in ls]
            den = ps[0]
            for w in range(1, WIN):
                den = den + ps[w]
            inv = 1.0 / den
            ps = [pw * inv for pw in ps]
            if smd:
                yield _or_all([pltpu.bitcast(ps[0], U32)]), smd
            for _ in range(skip - (1 if smd else 0)):
                yield
            zs = []
            if PVW == 1:
                os_ = [None] * NC
                for w in range(WIN):
                    if w % pvg == 0:
                        rel = yield
                    p = _gate(ps[w], rel)
                    for j in range(NC):
                        pv = p * shifted(vv, j, w)
                        os_[j] = pv if w == 0 else os_[j] + pv
                for j in range(NC):
                    if j % 4 == 0:
                        rel = yield
                    zs.append(_gather_inv(_pack(_gate(os_[j], rel)), j))
            else:
                for j in range(NC):
                    if j % pvg == 0:
                        rel = yield
                        pg = [_gate(p, rel) for p in ps] if PVW == 2 else [_gate(ps[0], rel)] + ps[1:]
                    acc = pg[0] * shifted(vv, j, 0)
                    for w in range(1, WIN):
                        acc = acc + pg[w] * shifted(vv, j, w)
                    zs.append(_gather_inv(_pack(acc), j))
            xs = _xor_network(zs)
            half = (base // 2 if isinstance(base, int) else jax.lax.shift_right_logical(base, 1)) + (0 if first else SA // 2)
            ov = o_v.at[_rows(half, span // 2, 16), :]
            for j in range(NC):
                ov[g * 8:(g + 1) * 8, j * 128:(j + 1) * 128] = xs[j]
            return _or_all(xs)

        def LN1(t, dst):
            return [ln1_task(t, g, dst) for g in range(NG)]

        def LN2(t, dst):
            return [ln2_task(t, g, dst) for g in range(NG)]

        def STATS(t):
            return [stats_task(t, g) for g in range(NG)]

        def FIN(t, k):
            return [fin_task(t, k, g0, 4) for g0 in range(0, NG, 4)]

        def MOD(m, j0=0, j1=NC, mg=2):
            return [mod_task(m, j, mg) for j in range(j0, j1)]

        def PERM(m, k):
            r0 = k * 128
            return ([perm_select_task(m, r, PR) for r in range(r0, r0 + 128, PR)]
                    + [perm_gather_task(m, j, r0, 128) for j in range(NC)])

        def COPY(src, dst, n, lo, hi, pre, c0=0, c1=D):
            nr = TM // 2 // n
            return ([copy_task(src, dst, r, nr, c0, c1) for r in range(0, TM // 2, nr)], lo, hi, pre)

        def run_now(tasks):
            for tk in tasks:
                try:
                    next(tk)
                    while True:
                        tk.send(None)
                except StopIteration:
                    pass

        def tie(a, tok):
            if tok is not None:
                top = a[0:8, 0:128] | (tok & zero())
                if a.shape[1] > 128:
                    top = jnp.concatenate([top, a[0:8, 128:]], axis=1)
                a = jnp.concatenate([top, a[8:]], axis=0)
            return pltpu.bitcast(a, BF16)


        def releases(res):
            return [pltpu.bitcast(res[r:r + 8, 0:128], U32) & zero() for r in range(0, TM, TM // cur["nrel"])]

        def wave_pass(k, t, nb, tok):
            m, j0 = nb // 2, (nb % 2) * 4
            dst = (qa_v, ka_v, va_v)[m]
            rows = slice(t * TM + (PAD if m else 0), (t + 1) * TM + (PAD if m else 0))
            w = pltpu.bitcast(wp_v[k * 64:(k + 1) * 64, nb * 512:(nb + 1) * 512], BF16)
            res = jnp.dot(tie(h1_v[t, :, k * 128:(k + 1) * 128], tok), w, preferred_element_type=F32)
            for jj in range(4):
                r = res[:, jj * 128:(jj + 1) * 128]
                if k == NC - 1 and ND:
                    c0 = nb * 512 + jj * 128
                    r = r + jnp.tile(bias_v[:, c0:c0 + 128], (TM // 8, 1))
                if k > 0:
                    r = dst[j0 + jj, rows, :] + r
                dst[j0 + jj, rows, :] = r
            return releases(res)

        def qkv_pass(t, m, j, hf, st, tok):
            w = pltpu.bitcast(wp_v[hf * HK // 2:(hf + 1) * HK // 2, m * D + j * 128:m * D + (j + 1) * 128], BF16)
            res = jnp.dot(tie(hc_v[:, hf * HK:(hf + 1) * HK], tok), w, preferred_element_type=F32)
            if hf == 0:
                st[m, j] = res
            else:
                res = st.pop((m, j)) + res
                off = PAD if m else 0
                dst = (qb_v, kb_v, vb_v)[m].at[:, _rows((t - 2) * TM, TM + off, TM), :]
                dst[j, off:off + TM, :] = res
            return releases(res)

        def wo_pass(t, j, hf, st, tok):
            h = tie(o_v[_rows(t * (TM // 2), TM // 2, TM // 2), hf * HK:(hf + 1) * HK], tok)
            res = jnp.dot(h, wo_v[hf * HK:(hf + 1) * HK, j * 128:(j + 1) * 128], preferred_element_type=F32)
            if hf == 0:
                st["a"] = res
            else:
                rows, cs = _rows(t * TM, TM, TM), slice(j * 128, (j + 1) * 128)
                res = x_v[rows, cs].astype(F32) + mod_v[2:3, cs] * (st.pop("a") + res)
                x1_v[j, rows, :] = res
            return releases(res)

        def out_copy(t, j):
            rows = _rows(t * TM, TM, TM)
            return cp(out_v.at[j, rows, :], out_hbm.at[rows, pl.ds(j * 128, 128)], sem_out.at[t])

        def out_wait(t):
            if only is not None and ("FL" if t == NT - 1 else "F") not in only:
                return
            rows = pl.ds(t * TM, TM)
            cp(out_hbm.at[rows, :], out_hbm.at[rows, :], sem_out.at[t]).wait()

        def WAVE(k):
            return [functools.partial(wave_pass, k, t, nb) for m in range(3) for t in range(2) for nb in (2 * m, 2 * m + 1)]

        def QKV(t):
            order = [(m, j, hf) for m in range(3) for j in range(NC) for hf in range(2)]
            order = order[:-2 * QT] + order[-2 * QT::2] + order[-2 * QT + 1::2]
            st = {}
            return [functools.partial(qkv_pass, t, m, j, hf, st) for m, j, hf in order]

        def WO(t):
            st = {}
            return [functools.partial(wo_pass, t, j, hf, st) for j in range(NC) for hf in range(2)]

        def FFN(t, c0, c1):
            st = {"acc": [None] * NC, "act": []}
            h_v = hn_v if c0 == 0 else h2_v

            def gate_up_pass(which, n, hf, tok):
                w = (w1_v, w3_v)[which][hf * HK:(hf + 1) * HK, n * 128:(n + 1) * 128]
                res = jnp.dot(tie(h_v[:, hf * HK:(hf + 1) * HK], tok), w, preferred_element_type=F32)
                if hf == 0:
                    st["a"] = res
                else:
                    res = st.pop("a") + res
                    if which == 0:
                        hg = 0.5 * res
                        st["g"] = hg + hg * jnp.tanh(hg)
                    else:
                        st["act"].append((st.pop("g") * res).astype(BF16))
                return releases(res)

            def down_pass(c, j, last, tok):
                if j == 0:
                    st["lhs"], st["act"] = jnp.concatenate(st["act"], axis=1), []
                w = w2_v[c * HK:(c + 1) * HK, j * 128:(j + 1) * 128]
                if tok is not None:
                    w = tie(pltpu.bitcast(w, U32), tok)
                res = jnp.dot(st["lhs"], w, preferred_element_type=F32)
                if c > 0:
                    res = (acc_v[j] if c == c0 else st["acc"][j]) + res
                st["acc"][j] = res
                if c == c1 - 1 and not last:
                    acc_v[j] = res
                if last:
                    rows = _rows(t * TM, TM, TM)
                    out_v[j, rows, :] = (x1_v[j, rows, :] + mod_v[5:6, j * 128:(j + 1) * 128] * res).astype(BF16)
                    out_copy(t, j).start()
                return releases(res)

            out = []
            nch = F // HK
            for c in range(c0, c1):
                for n in range(c * 4, c * 4 + 4):
                    out += [functools.partial(gate_up_pass, which, n, hf) for which in range(2) for hf in range(2)]
                out += [functools.partial(down_pass, c, j, c == nch - 1) for j in range(NC)]
            return out

        def segment(name, passes, groups=(), dl=DL, need=None, nrel=NREL, lns=(0, 0)):
            if only is not None and name not in only:
                return
            with scope(name):
                n = len(passes)
                cur["nrel"], cur["lns"] = nrel, lns
                active = []
                for tasks, lo, hi, *pre in groups:
                    for k, tk in enumerate(tasks):
                        active.append((int((lo + k * (hi - lo) / len(tasks)) * nrel), tk, pre[0] if pre else ()))
                        next(tk)
                deadlines = [[] for _ in range(n + dl + 8)]

                def due(p):
                    return p + DSH if p < n and passes[p].func.__name__ == "down_pass" else p

                def done(tasks):
                    return all(ent[1] is not tk for tk in tasks for ent in active)

                def feed(rel, slot, i):
                    for ent in list(active):
                        if ent[0] <= slot:
                            assert done(ent[2]), (name, i)
                            try:
                                mid = ent[1].send(rel)
                                if mid is not None:
                                    deadlines[due(i + mid[1])].append(mid[0])
                            except StopIteration as e:
                                if e.value is not None:
                                    deadlines[due(i + dl)].append(e.value)
                                active.remove(ent)

                feed(None, 0, 0)
                slot = 1
                for i, ps in enumerate(passes):
                    assert done((need or {}).get(i, ())), (name, i)
                    for rel in ps(_or_all(deadlines[i]) if deadlines[i] else None):
                        feed(rel, slot, i)
                        slot += 1
                while active:
                    feed(None, 1 << 30, n)

        def mnames(k):
            return [f"m1{k}"] + ([f"m0{k}"] if k >= ND else [])

        def MODS(k, mg=2):
            return MOD(1, k, k + 1, mg) + (MOD(0, k, k + 1, mg) if k >= ND else [])

        with scope("S0"):
            wait("c", "z")
            c = c_v[...].astype(F32)
            s = (c * jax.nn.sigmoid(c)).astype(BF16).astype(F32)
            eye = (jax.lax.broadcasted_iota(jnp.int32, (128, 128), 0)
                   == jax.lax.broadcasted_iota(jnp.int32, (128, 128), 1))
            ones = jnp.ones((128, 128), BF16)
            for j in range(NC):
                dg = jnp.where(eye, jnp.broadcast_to(s[:, j * 128:(j + 1) * 128], (128, 128)), 0.0).astype(BF16)
                scol_v[j * 128:(j + 1) * 128, :] = jnp.dot(dg, ones, preferred_element_type=F32)
            wait("x0")
            run_now(STATS(0))
            wait(*mnames(0))
            run_now(MODS(0) + FIN(0, 0))
            wait("w00")
            run_now(PERM(0, 0))
            wait("w10", "w20")

        m0 = [functools.partial(wave_pass, 0, t, nb) for t in range(2) for nb in range(6)]
        m1 = WAVE(1)
        n0, n1, n2 = W0
        p1, p2 = PERM(1, 0), PERM(2, 0)
        segment("T0a", m0[:n0], [(p1, 0, T0P[0]), (p2, T0P[0], n0 - 0.5)], need={2: p1}, nrel=T0N[0])
        wait("x1")
        s1, f1, u = STATS(1), FIN(1, 0), 6 - n0
        segment("T0b", m0[n0:n1], [(s1, 0, max(0.2, u - T0P[1])), (f1, u - T0P[2], u - 0.01, s1)], need={u: s1 + f1},
                nrel=T0N[1])
        wait(*mnames(1), "w01")
        mods, f0, f1, pq, u = MODS(1), FIN(0, 1), FIN(1, 1), PERM(0, 1), 12 - n1
        fmin = max(3 / T0N[2], u - T0P[3])
        segment("T0c", m0[n1:] + m1[:n2],
                [(mods, 0, 0.2), (f0, fmin, u - 0.01, mods), (f1, u, u + 1, mods), (pq, 0, max(0.5, u - T0P[4]))],
                need={u: mods + f0 + pq, u + 2: f1}, nrel=T0N[2])
        wait("w11", "w21")
        p1, p2 = PERM(1, 1), PERM(2, 1)
        e1 = max(0.5, 4 - n2 - T0P[5])
        segment("T1", m1[n2:WA[1]], [(p1, 0, e1), (p2, e1, 8 - n2 - 1.5)], need={4 - n2: p1, 8 - n2: p2}, nrel=T0N[3])
        for k in range(2, NC):
            last = k == NC - 1
            late = [kk for kk in range(ND) if SAT[kk] == k]
            wait(*mnames(k), f"w0{k}", f"w1{k}", f"w2{k}", *[f"m0{kk}" for kk in late], *(["x2"] if k == X2AT + 1 else []))
            u = 12 - WA[k - 1]
            mods = MODS(k, TMG)
            fins = [FIN(t, k) for t in range(2)]
            perms = [PERM(m, k) for m in range(3)]
            mend = max(0.5, u - WP[0])
            fmin = (8 // TMG - 1) / TN + (mend - 0.5 if mend > 2 else 0)
            groups = [(mods[:1], 0, 1)] + ([(mods[1:], mend - 0.5 if mend > 2 else 0, mend)] if len(mods) > 1 else []) + [
                      (fins[0], max(fmin, u - WP[1]), max(fmin + 0.2, u - WP[2]), mods), (fins[1], max(fmin + 0.2, u - WP[2]), u + 1, mods),
                      (perms[0], 0, max(0.9, u - WP[3])), (perms[1], max(0.9, u - WP[3]), u + WP[4]), (perms[2], u + WP[4], u + WP[5])]
            for kk in late:
                ms, sc = MOD(0, kk, kk + 1, TMG), [shift_col_task(kk)]
                groups += [(ms, SBP[0], SBP[0] + 1), (sc, SBP[1], SBP[1] + 1, ms),
                           ([bias_task(kk, c) for c in range(3 * NC)], SBP[2], SBP[3], sc)]
            if k == X2AT + 1:
                s2 = STATS(2)
                groups.append((s2, *X2S))
            for kk in range(NC):
                if X2F[kk][0] == k:
                    assert kk <= k
                    groups.append((FIN(2, kk), *X2F[kk][1:], (s2 if k == X2AT + 1 else []) + (mods if kk == k else [])))
            segment(f"T{k}", WAVE(k - 1)[WA[k - 1]:] + (WAVE(k) if last else WAVE(k)[:WA[k]]), groups,
                    need={u: mods + fins[0] + perms[0], u + 2: fins[1], u + 4: perms[1], u + 8: perms[2]}, nrel=TN, lns=TLS)
        wait("xr")

        def a_step(t, carry):
            base = jnp.minimum((t - 2) * (NPC // 2), NG) * (2 * G)
            att = [attn_task(True, base, NPC * G, g, AQ, masked=(g == 0)) for g in range(NPC)]
            l1 = LN1(t + 1, hn_v)
            segment("A", QKV(t), [(att, *AA), (l1, *AL), COPY(hn_v, hc_v, ACN[0], 48 - QT, 47, l1, 0, HK),
                                 COPY(hn_v, hc_v, ACN[1], 47 + 1 / AN, 48 + 1 / AN, l1, HK, D)], dl=ADL, nrel=AN, lns=ALS)
            return carry

        with scope("loopA"):
            jax.lax.fori_loop(2, NT - 1, a_step, 0)
        wait("wmr", "wo", "fw1", "fw3", "fw2a")
        q7, nq = QKV(NT - 1), AFP[0]
        mg, msc, l2 = MOD(2, mg=MG), MOD(3, mg=MG) + MOD(4, mg=MG), LN2(0, hn_v)
        done_rows = (NT - 3) * NPC * G
        att = [attn_task(True, done_rows, SA - done_rows, g, AFQ) for g in range((SA - done_rows) // G)]
        segment("AF", q7[:nq] + WO(0) + q7[nq:] + FFN(0, 0, C0),
                [(mg, 0, AFP[1]), (msc, AFP[1], AFP[2]), (l2, max(AFP[3], nq + 16), AFP[4], msc),
                 (MOD(5, mg=MG), AFP[5], AFP[6]), (att, AFP[7], AFP[8]), ([halo_task()], 1, 2)]
                + [COPY(hn_v, h2_v, 16, *AFC, l2)], need={nq: mg, 64: l2}, dl=AFDL, nrel=AFN, lns=AFL)
        wait("fw2b")

        nch = F // HK
        nf = (nch - C0) * 24

        def b_step(i, carry):
            att = [attn_task(False, jnp.minimum(i, NT - 3) * TM, TM, g, BQ) for g in range(NG)]
            l2 = LN2(i + 1, hn_v)
            ffn = FFN(i, C0, nch)
            cpy = [COPY(hn_v, h2_v, 16, nf + 16 - 8 + BCP[0], nf + 16 - 8 + BCP[1], l2)]
            assert BA[0] >= 16 + BW and BL[0] >= 16 + BW and min(BCP) >= 0
            segment("F", ffn[:BW] + WO(i + 1) + ffn[BW:] + FFN(i + 1, 0, C0), ([(att, *BA)] if NOV < 1 else []) + ([(l2, *BL)] + cpy if NOV < 2 else []),
                    need={nf + 16: l2}, dl=BDL, nrel=BN, lns=BLS)
            return carry

        with scope("B"):
            jax.lax.fori_loop(0, NT - 1, b_step, 0)
        for t in range(NT - 2):
            out_wait(t)
        segment("FL", FFN(NT - 1, C0, nch))
        with scope("fin"):
            for t in range(NT - 2, NT):
                out_wait(t)

    @jax.jit
    def fn(A_x, A_wqkv, A_wo, B_x, B_w1, B_w3, B_w2, c, w_mod):
        V = pltpu.VMEM
        scratch = [
            V((S, D), BF16), V((3, D, D), BF16), V((D // 2, 3 * D), U32), V((D, D), BF16),
            V((D, F), BF16), V((D, F), BF16), V((F, D), BF16), V((2 * NC, D, 128), BF16), V((D, 4 * D), BF16),
            V((8, D), F32), V((D, 128), F32), V((2, SA + TM, 128), F32), V((2, TM // 2, D), U32),
            V((NC, SA, 128), F32), V((NC, PAD + SA, 128), F32), V((NC, PAD + SA, 128), F32),
            V((NC, SB, 128), F32), V((NC, PAD + SB, 128), F32), V((NC, PAD + SB, 128), F32),
            V((S // 2, D), U32), V((NC, S, 128), F32), V((TM // 2, D), U32), V((NC, S, 128), BF16),
            V((TM // 2, D), U32), V((TM // 2, D), U32), V((NC, TM, 128), F32), V((128, 128), F32), V((8, 3 * D), F32), V((32, 128), F32), V((1, D), BF16),
            pltpu.SemaphoreType.DMA((5 * NC + 12,)), pltpu.SemaphoreType.DMA((NT,)), pltpu.SemaphoreType.REGULAR,
        ]
        out = pl.pallas_call(
            kernel,
            in_specs=[pl.BlockSpec(memory_space=pl.ANY)] * 8,
            out_specs=pl.BlockSpec(memory_space=pl.ANY),
            out_shape=jax.ShapeDtypeStruct((S, D), BF16),
            scratch_shapes=scratch,
            compiler_params=pltpu.CompilerParams(vmem_limit_bytes=124 * 1024 * 1024, disable_bounds_checks=True,
                                                 disable_semaphore_checks=True),
        )(A_x.reshape(S, D), A_wqkv, A_wo, B_w1, B_w3, B_w2, c, w_mod)
        return out.reshape(1, S, D)

    return fn


_impl = make_kernel()


@jax.jit
def pallas_adaLN_cond__sliding_local_dilated__glu_gated_swiglu__prompt_kernel(A_x, A_wqkv, A_wo, B_x, B_w1, B_w3, B_w2, c, w_mod):
    return _impl(A_x, A_wqkv, A_wo, B_x, B_w1, B_w3, B_w2, c, w_mod)
```

```python
import contextlib
import functools
import math

import jax
import jax.numpy as jnp
import jax.experimental.pallas as pl
import jax.experimental.pallas.tpu as pltpu

S, D, F = 2048, 1024, 3584
DH, WIN, DIL = 32, 8, 2
NC = D // 128
PAD = 16
EPS = 1e-5
SCALE = DH ** -0.5
EXP2_C = SCALE * math.log2(math.e)
MASKED = -1e9 / SCALE
F32, BF16, U32 = jnp.float32, jnp.bfloat16, jnp.uint32
TM = 256
NT = S // TM
G = 16
NG = TM // G
HK = D // 2
SA = 2 * TM
SB = S - SA


def _xor_network(xs):
    lane = jax.lax.broadcasted_iota(jnp.int32, xs[0].shape, 1)
    for b in range(3):
        m = ((lane >> (2 + b)) & 1) == 1
        xs = [jnp.where(m, xs[i ^ (1 << b)], xs[i]) for i in range(NC)]
    return xs


def _gather_fwd(z, j):
    lane = jax.lax.broadcasted_iota(jnp.int32, z.shape, 1)
    e, g, p = lane >> 5, (lane >> 3) & 3, lane & 7
    return jnp.take_along_axis(z, g * 32 + (p ^ j) * 4 + e, axis=1)


def _gather_inv(y, j):
    lane = jax.lax.broadcasted_iota(jnp.int32, y.shape, 1)
    g, q, e = lane >> 5, (lane >> 2) & 7, lane & 3
    return jnp.take_along_axis(y, e * 32 + g * 8 + (q ^ j), axis=1)


def _pack(x):
    return pltpu.bitcast(x.astype(BF16), U32)


def _or_all(vs):
    parts = [v[r:r + 8, c:c + 128] for v in vs for r in range(0, v.shape[0], 8) for c in range(0, v.shape[1], 128)]
    while len(parts) > 1:
        parts = [parts[i] | parts[i + 1] if i + 1 < len(parts) else parts[i] for i in range(0, len(parts), 2)]
    return parts[0]


def _gate(x, g):
    if g is None:
        return x
    xb = x if x.dtype == U32 else pltpu.bitcast(x, U32)
    y = xb | jnp.tile(g, (x.shape[0] // 8, x.shape[1] // 128))
    return y if x.dtype == U32 else pltpu.bitcast(y, x.dtype)


def _rows(start, n, mult):
    if isinstance(start, int):
        return pl.ds(start, n)
    return pl.ds(pl.multiple_of(start, mult), n)


def _stats(x):
    mu = jnp.mean(x, axis=-1, keepdims=True)
    xc = x - mu
    var = jnp.mean(xc * xc, axis=-1, keepdims=True)
    return mu, xc, jax.lax.rsqrt(var + EPS)


def make_kernel(
        NREL=2, DL=4, DSH=1, MG=1, TMG=2, PR=16,
        ND=2, SAT=(4, 5), SBP=(1.5, 3, 4.5, 8), W0=(4, 10, 3), WA=(9, 10, 8, 7, 7, 6, 6),
        T0N=(2, 4, 2, 2), T0P=(1.25, 0.75, 0.5, 0.25, 1.25, 0.5), TN=4, WP=(3, 1, 0.5, 1.5, 2, 5.5),
        X2AT=5, X2S=(2, 9),
        X2F=((6, 9.5, 10.5), (7, 2, 3), (7, 4, 5), (7, 7, 8), (7, 9, 10), (7, 12, 13), (7, 13, 14), (7, 14, 15)),
        NPC=6, QT=4, AN=4, AQ=(2, 2, 13, 4), AA=(1, 38), AL=(2, 38), ALS=(2, 4), ACN=(4, 2), ADL=4,
        C0=1, AFN=4, AFQ=(1, 1, 12, 3), AFP=(20, 15, 36, 38, 58, 60, 84, 0, 16), AFL=(0, 0), AFC=(66, 86), AFDL=5,
        BW=2, BN=4, BQ=(1, 1, 20, 5), BA=(18, 170), BL=(20, 149), BLS=(2, 4), BCP=(8, 28), BDL=6,
        scopes=False, only=None):

    def scope(name):
        return jax.named_scope(name) if scopes else contextlib.nullcontext()

    def kernel(x_hbm, wqkv_hbm, wo_hbm, w1_hbm, w3_hbm, w2_hbm, c_hbm, wm_hbm, out_hbm,
               x_v, wraw_v, wp_v, wo_v, w1_v, w3_v, w2_v, wmc_v, wmr_v,
               mod_v, scol_v, st_v, h1_v, qa_v, ka_v, va_v, qb_v, kb_v, vb_v, o_v, x1_v, h2_v, out_v,
               hc_v, hn_v, acc_v, sac_v, bias_v, z_v, c_v, sems, sem_out, bar):
        cp = pltpu.make_async_copy

        dmas = {}

        def add(name, src, dst):
            dmas[name] = cp(src, dst, sems.at[len(dmas)])

        def add_x(name, t0, n):
            add(name, x_hbm.at[pl.ds(t0 * TM, n * TM), :], x_v.at[pl.ds(t0 * TM, n * TM), :])

        add("c", c_hbm, c_v)
        add_x("x0", 0, 1)
        for k in range(NC):
            for m, kk in [(1, k)] + ([(0, k)] if k >= ND else []):
                add(f"m{m}{kk}", wm_hbm.at[:, pl.ds(m * D + kk * 128, 128)], wmc_v.at[m * NC + kk])
            for m in range(3):
                add(f"w{m}{k}", wqkv_hbm.at[pl.ds(k * 128, 128), pl.ds(m * D, D)], wraw_v.at[m, pl.ds(k * 128, 128), :])
            if k == 0:
                add_x("x1", 1, 1)
            for kk in range(ND):
                if SAT[kk] - 1 == k:
                    add(f"m0{kk}", wm_hbm.at[:, pl.ds(kk * 128, 128)], wmc_v.at[kk])
            if k == X2AT:
                add_x("x2", 2, 1)
        add_x("xr", 3, NT - 3)
        add("wmr", wm_hbm.at[:, pl.ds(2 * D, 4 * D)], wmr_v)
        add("wo", wo_hbm, wo_v)
        add("fw1", w1_hbm, w1_v)
        add("fw3", w3_hbm, w3_v)
        add("fw2a", w2_hbm.at[pl.ds(0, C0 * HK), :], w2_v.at[pl.ds(0, C0 * HK), :])
        add("fw2b", w2_hbm.at[pl.ds(C0 * HK, F - C0 * HK), :], w2_v.at[pl.ds(C0 * HK, F - C0 * HK), :])
        for d in dmas.values():
            d.start()
            pl.semaphore_signal(bar, 1)
            pl.semaphore_wait(bar, 1)
        for j in range(NC):
            ka_v[j, 0:PAD, :] = jnp.zeros((PAD, 128), F32)
            va_v[j, 0:PAD, :] = jnp.zeros((PAD, 128), F32)
        add("z", ka_v.at[0, pl.ds(0, 8), :], z_v.at[pl.ds(0, 8), :])
        dmas["z"].start()

        def wait(*names):
            with scope("w_" + names[0]):
                for n in names:
                    dmas[n].wait()

        def zero():
            return pltpu.bitcast(z_v[0:8, :], U32)

        cur = {"nrel": NREL, "lns": (0, 0)}

        def mod_task(m, j, mg=2):
            src = wmc_v.at[m * NC + j] if m < 2 else wmr_v.at[:, pl.ds((m - 2) * D + j * 128, 128)]
            acc = None
            for kb in range(D // 128):
                if kb % mg == 0:
                    rel = yield
                p = src[kb * 128:(kb + 1) * 128, :].astype(F32) * scol_v[kb * 128:(kb + 1) * 128, :]
                parts = [p[r:r + 8] for r in range(0, 128, 8)]
                a0, a1 = parts[0], parts[1]
                if kb % mg == 0:
                    a0, a1 = _gate(a0, rel), _gate(a1, rel)
                for r in range(2, 16, 2):
                    a0, a1 = a0 + parts[r], a1 + parts[r + 1]
                a0 = a0 + a1
                acc = a0 if acc is None else acc + a0
            r = jnp.sum(acc, axis=0, keepdims=True)
            if m in (1, 4):
                r = r + 1.0
            mod_v[m:m + 1, j * 128:(j + 1) * 128] = r
            return pltpu.bitcast(jnp.broadcast_to(r, (8, 128)), U32)

        def modulate(xn, ms, dst, g, c0, c1, shift=True):
            h = xn * mod_v[ms + 1:ms + 2, c0:c1]
            hb = _pack(h + mod_v[ms:ms + 1, c0:c1] if shift else h)
            dst[g * 8:(g + 1) * 8, c0:c1] = hb
            return _or_all([hb])

        def ln_tail(xc, rs, ms, dst, g):
            ns, skip = cur["lns"]
            if ns == 0:
                return modulate(xc * rs, ms, dst, g, 0, D)
            for _ in range(skip):
                yield
            rs = jnp.broadcast_to(rs, (G, 128))
            toks = []
            cw = D // ns
            for p in range(ns):
                rel = yield
                r = jnp.tile(_gate(rs, rel), (1, cw // 128))
                toks.append(modulate(xc[:, p * cw:(p + 1) * cw] * r, ms, dst, g, p * cw, (p + 1) * cw))
            return _or_all(toks)

        def ln1_task(t, g, dst):
            rel = yield
            xt = x_v.at[_rows(t * TM, TM, TM), :]
            _, xc, rs = _stats(_gate(xt[g * G:(g + 1) * G, :].astype(F32), rel))
            return (yield from ln_tail(xc, rs, 0, dst, g))

        def stats_task(t, g):
            rel = yield
            rows = slice(t * TM + g * G, t * TM + (g + 1) * G)
            mu, _, rs = _stats(_gate(x_v[rows, :].astype(F32), rel))
            rs = jnp.broadcast_to(rs, (G, 128))
            st_v[0, rows, :] = jnp.broadcast_to(mu, (G, 128))
            st_v[1, rows, :] = rs
            return _or_all([pltpu.bitcast(rs, U32)]) if t == 2 else None

        def fin_task(t, k, g0, ng):
            rel = yield
            toks = []
            for g in range(g0, g0 + ng):
                rows = slice(t * TM + g * G, t * TM + (g + 1) * G)
                x = _gate(x_v[rows, k * 128:(k + 1) * 128].astype(F32), rel)
                xn = (x - st_v[0, rows, :]) * st_v[1, rows, :]
                toks.append(modulate(xn, 0, h1_v.at[t] if t < 2 else hc_v, g, k * 128, (k + 1) * 128, t == 2 or k >= ND))
            return _or_all(toks) if t == 2 else None

        def ln2_task(t, g, dst):
            rel = yield
            xv = x1_v.at[:, _rows(t * TM, TM, TM), :]
            x = jnp.concatenate([_gate(xv[j, g * G:(g + 1) * G, :], rel) for j in range(NC)], axis=1)
            _, xc, rs = _stats(x)
            return (yield from ln_tail(xc, rs, 3, dst, g))

        def perm_select_task(m, r0, n):
            rel = yield
            xs = [_gate(pltpu.bitcast(wraw_v[m, r0:r0 + n, j * 128:(j + 1) * 128], U32), rel) for j in range(NC)]
            zs = _xor_network(xs)
            for j in range(NC):
                wp_v[r0 // 2:(r0 + n) // 2, m * D + j * 128:m * D + (j + 1) * 128] = zs[j]

        def perm_gather_task(m, j, r0, n):
            rel = yield
            sl = (slice(r0 // 2, (r0 + n) // 2), slice(m * D + j * 128, m * D + (j + 1) * 128))
            wp_v[sl] = _gather_fwd(_gate(wp_v[sl], rel), j)

        def shift_col_task(k):
            rel = yield
            row = _gate(jnp.broadcast_to(mod_v[0:1, k * 128:(k + 1) * 128], (128, 128)), rel)
            sac_v[...] = row.T

        def bias_task(k, c):
            rel = yield
            cs = slice(c * 128, (c + 1) * 128)
            w = pltpu.bitcast(_gate(wp_v[k * 64:(k + 1) * 64, cs], rel), BF16).astype(F32) * sac_v[...]
            parts = [w[r:r + 8] for r in range(0, 128, 8)]
            while len(parts) > 1:
                parts = [parts[i] + parts[i + 1] for i in range(0, len(parts), 2)]
            acc = parts[0] if k == 0 else bias_v[:, cs] + parts[0]
            if k == ND - 1:
                acc = jnp.broadcast_to(jnp.sum(acc, axis=0, keepdims=True), (8, 128))
            bias_v[:, cs] = acc
            return pltpu.bitcast(acc, U32)

        def copy_task(src, dst, r0, nr, c0, c1):
            rel = yield
            dst[r0:r0 + nr, c0:c1] = _gate(src[r0:r0 + nr, c0:c1], rel)

        def halo_task():
            yield
            for j in range(NC):
                kb_v[j, 0:PAD, :] = ka_v[j, SA:SA + PAD, :]
                vb_v[j, 0:PAD, :] = va_v[j, SA:SA + PAD, :]

        def attn_task(first, base, span, g, pace, masked=False):
            qkg, pvg, skip, smd = pace
            q_v, k_v, v_v = (qa_v, ka_v, va_v) if first else (qb_v, kb_v, vb_v)
            qv = q_v.at[:, _rows(base, span, 32), :]
            kv = k_v.at[:, _rows(base, span + PAD, 32), :]
            vv = v_v.at[:, _rows(base, span + PAD, 32), :]

            def shifted(ref, j, w):
                return ref[j, pl.ds(g * G + PAD - DIL * w, G), :]

            ls = [None] * WIN
            for j in range(NC):
                if j % qkg == 0:
                    rel = yield
                q = _gate(qv[j, g * G:(g + 1) * G, :], rel)
                for w in range(WIN):
                    p = q * shifted(kv, j, w)
                    ls[w] = p if j == 0 else ls[w] + p
            ls = [l + pltpu.roll(l, 64, 1) for l in ls]
            ls = [l + pltpu.roll(l, 32, 1) for l in ls]
            if masked:
                rows = base + g * G + jax.lax.broadcasted_iota(jnp.int32, (G, 128), 0)
                ls = [ls[0]] + [jnp.where(rows >= DIL * w, ls[w], MASKED) for w in range(1, WIN)]
            mx = ls[0]
            for w in range(1, WIN):
                mx = jnp.maximum(mx, ls[w])
            ps = [jnp.exp2((l - mx) * EXP2_C) for l in ls]
            den = ps[0]
            for w in range(1, WIN):
                den = den + ps[w]
            inv = 1.0 / den
            ps = [pw * inv for pw in ps]
            if smd:
                yield _or_all([pltpu.bitcast(ps[0], U32)]), smd
            for _ in range(skip - (1 if smd else 0)):
                yield
            zs = []
            for j in range(NC):
                if j % pvg == 0:
                    rel = yield
                    pg = [_gate(p, rel) for p in ps]
                acc = pg[0] * shifted(vv, j, 0)
                for w in range(1, WIN):
                    acc = acc + pg[w] * shifted(vv, j, w)
                zs.append(_gather_inv(_pack(acc), j))
            xs = _xor_network(zs)
            half = (base // 2 if isinstance(base, int) else jax.lax.shift_right_logical(base, 1)) + (0 if first else SA // 2)
            ov = o_v.at[_rows(half, span // 2, 16), :]
            for j in range(NC):
                ov[g * 8:(g + 1) * 8, j * 128:(j + 1) * 128] = xs[j]
            return _or_all(xs)

        def LN1(t, dst):
            return [ln1_task(t, g, dst) for g in range(NG)]

        def LN2(t, dst):
            return [ln2_task(t, g, dst) for g in range(NG)]

        def STATS(t):
            return [stats_task(t, g) for g in range(NG)]

        def FIN(t, k):
            return [fin_task(t, k, g0, 4) for g0 in range(0, NG, 4)]

        def MOD(m, j0=0, j1=NC, mg=2):
            return [mod_task(m, j, mg) for j in range(j0, j1)]

        def PERM(m, k):
            r0 = k * 128
            return ([perm_select_task(m, r, PR) for r in range(r0, r0 + 128, PR)]
                    + [perm_gather_task(m, j, r0, 128) for j in range(NC)])

        def COPY(src, dst, n, lo, hi, pre, c0=0, c1=D):
            nr = TM // 2 // n
            return ([copy_task(src, dst, r, nr, c0, c1) for r in range(0, TM // 2, nr)], lo, hi, pre)

        def run_now(tasks):
            for tk in tasks:
                try:
                    next(tk)
                    while True:
                        tk.send(None)
                except StopIteration:
                    pass

        def tie(a, tok):
            if tok is not None:
                top = a[0:8, 0:128] | (tok & zero())
                if a.shape[1] > 128:
                    top = jnp.concatenate([top, a[0:8, 128:]], axis=1)
                a = jnp.concatenate([top, a[8:]], axis=0)
            return pltpu.bitcast(a, BF16)


        def releases(res):
            return [pltpu.bitcast(res[r:r + 8, 0:128], U32) & zero() for r in range(0, TM, TM // cur["nrel"])]

        def wave_pass(k, t, nb, tok):
            m, j0 = nb // 2, (nb % 2) * 4
            dst = (qa_v, ka_v, va_v)[m]
            rows = slice(t * TM + (PAD if m else 0), (t + 1) * TM + (PAD if m else 0))
            w = pltpu.bitcast(wp_v[k * 64:(k + 1) * 64, nb * 512:(nb + 1) * 512], BF16)
            res = jnp.dot(tie(h1_v[t, :, k * 128:(k + 1) * 128], tok), w, preferred_element_type=F32)
            for jj in range(4):
                r = res[:, jj * 128:(jj + 1) * 128]
                if k == NC - 1 and ND:
                    c0 = nb * 512 + jj * 128
                    r = r + jnp.tile(bias_v[:, c0:c0 + 128], (TM // 8, 1))
                if k > 0:
                    r = dst[j0 + jj, rows, :] + r
                dst[j0 + jj, rows, :] = r
            return releases(res)

        def qkv_pass(t, m, j, hf, st, tok):
            w = pltpu.bitcast(wp_v[hf * HK // 2:(hf + 1) * HK // 2, m * D + j * 128:m * D + (j + 1) * 128], BF16)
            res = jnp.dot(tie(hc_v[:, hf * HK:(hf + 1) * HK], tok), w, preferred_element_type=F32)
            if hf == 0:
                st[m, j] = res
            else:
                res = st.pop((m, j)) + res
                off = PAD if m else 0
                dst = (qb_v, kb_v, vb_v)[m].at[:, _rows((t - 2) * TM, TM + off, TM), :]
                dst[j, off:off + TM, :] = res
            return releases(res)

        def wo_pass(t, j, hf, st, tok):
            h = tie(o_v[_rows(t * (TM // 2), TM // 2, TM // 2), hf * HK:(hf + 1) * HK], tok)
            res = jnp.dot(h, wo_v[hf * HK:(hf + 1) * HK, j * 128:(j + 1) * 128], preferred_element_type=F32)
            if hf == 0:
                st["a"] = res
            else:
                rows, cs = _rows(t * TM, TM, TM), slice(j * 128, (j + 1) * 128)
                res = x_v[rows, cs].astype(F32) + mod_v[2:3, cs] * (st.pop("a") + res)
                x1_v[j, rows, :] = res
            return releases(res)

        def out_copy(t, j):
            rows = _rows(t * TM, TM, TM)
            return cp(out_v.at[j, rows, :], out_hbm.at[rows, pl.ds(j * 128, 128)], sem_out.at[t])

        def out_wait(t):
            if only is not None and ("FL" if t == NT - 1 else "F") not in only:
                return
            rows = pl.ds(t * TM, TM)
            cp(out_hbm.at[rows, :], out_hbm.at[rows, :], sem_out.at[t]).wait()

        def WAVE(k):
            return [functools.partial(wave_pass, k, t, nb) for m in range(3) for t in range(2) for nb in (2 * m, 2 * m + 1)]

        def QKV(t):
            order = [(m, j, hf) for m in range(3) for j in range(NC) for hf in range(2)]
            order = order[:-2 * QT] + order[-2 * QT::2] + order[-2 * QT + 1::2]
            st = {}
            return [functools.partial(qkv_pass, t, m, j, hf, st) for m, j, hf in order]

        def WO(t):
            st = {}
            return [functools.partial(wo_pass, t, j, hf, st) for j in range(NC) for hf in range(2)]

        def FFN(t, c0, c1):
            st = {"acc": [None] * NC, "act": []}
            h_v = hn_v if c0 == 0 else h2_v

            def gate_up_pass(which, n, hf, tok):
                w = (w1_v, w3_v)[which][hf * HK:(hf + 1) * HK, n * 128:(n + 1) * 128]
                res = jnp.dot(tie(h_v[:, hf * HK:(hf + 1) * HK], tok), w, preferred_element_type=F32)
                if hf == 0:
                    st["a"] = res
                else:
                    res = st.pop("a") + res
                    if which == 0:
                        hg = 0.5 * res
                        st["g"] = hg + hg * jnp.tanh(hg)
                    else:
                        st["act"].append((st.pop("g") * res).astype(BF16))
                return releases(res)

            def down_pass(c, j, last, tok):
                if j == 0:
                    st["lhs"], st["act"] = jnp.concatenate(st["act"], axis=1), []
                w = w2_v[c * HK:(c + 1) * HK, j * 128:(j + 1) * 128]
                if tok is not None:
                    w = tie(pltpu.bitcast(w, U32), tok)
                res = jnp.dot(st["lhs"], w, preferred_element_type=F32)
                if c > 0:
                    res = (acc_v[j] if c == c0 else st["acc"][j]) + res
                st["acc"][j] = res
                if c == c1 - 1 and not last:
                    acc_v[j] = res
                if last:
                    rows = _rows(t * TM, TM, TM)
                    out_v[j, rows, :] = (x1_v[j, rows, :] + mod_v[5:6, j * 128:(j + 1) * 128] * res).astype(BF16)
                    out_copy(t, j).start()
                return releases(res)

            out = []
            nch = F // HK
            for c in range(c0, c1):
                for n in range(c * 4, c * 4 + 4):
                    out += [functools.partial(gate_up_pass, which, n, hf) for which in range(2) for hf in range(2)]
                out += [functools.partial(down_pass, c, j, c == nch - 1) for j in range(NC)]
            return out

        def segment(name, passes, groups=(), dl=DL, need=None, nrel=NREL, lns=(0, 0)):
            if only is not None and name not in only:
                return
            with scope(name):
                n = len(passes)
                cur["nrel"], cur["lns"] = nrel, lns
                active = []
                for tasks, lo, hi, *pre in groups:
                    for k, tk in enumerate(tasks):
                        active.append((int((lo + k * (hi - lo) / len(tasks)) * nrel), tk, pre[0] if pre else ()))
                        next(tk)
                deadlines = [[] for _ in range(n + dl + 8)]

                def due(p):
                    return p + DSH if p < n and passes[p].func.__name__ == "down_pass" else p

                def done(tasks):
                    return all(ent[1] is not tk for tk in tasks for ent in active)

                def feed(rel, slot, i):
                    for ent in list(active):
                        if ent[0] <= slot:
                            assert done(ent[2]), (name, i)
                            try:
                                mid = ent[1].send(rel)
                                if mid is not None:
                                    deadlines[due(i + mid[1])].append(mid[0])
                            except StopIteration as e:
                                if e.value is not None:
                                    deadlines[due(i + dl)].append(e.value)
                                active.remove(ent)

                feed(None, 0, 0)
                slot = 1
                for i, ps in enumerate(passes):
                    assert done((need or {}).get(i, ())), (name, i)
                    for rel in ps(_or_all(deadlines[i]) if deadlines[i] else None):
                        feed(rel, slot, i)
                        slot += 1
                while active:
                    feed(None, 1 << 30, n)

        def mnames(k):
            return [f"m1{k}"] + ([f"m0{k}"] if k >= ND else [])

        def MODS(k, mg=2):
            return MOD(1, k, k + 1, mg) + (MOD(0, k, k + 1, mg) if k >= ND else [])

        with scope("S0"):
            wait("c", "z")
            c = c_v[...].astype(F32)
            s = (c * jax.nn.sigmoid(c)).astype(BF16).astype(F32)
            eye = (jax.lax.broadcasted_iota(jnp.int32, (128, 128), 0)
                   == jax.lax.broadcasted_iota(jnp.int32, (128, 128), 1))
            ones = jnp.ones((128, 128), BF16)
            for j in range(NC):
                dg = jnp.where(eye, jnp.broadcast_to(s[:, j * 128:(j + 1) * 128], (128, 128)), 0.0).astype(BF16)
                scol_v[j * 128:(j + 1) * 128, :] = jnp.dot(dg, ones, preferred_element_type=F32)
            wait("x0")
            run_now(STATS(0))
            wait(*mnames(0))
            run_now(MODS(0) + FIN(0, 0))
            wait("w00")
            run_now(PERM(0, 0))
            wait("w10", "w20")

        m0 = [functools.partial(wave_pass, 0, t, nb) for t in range(2) for nb in range(6)]
        m1 = WAVE(1)
        n0, n1, n2 = W0
        p1, p2 = PERM(1, 0), PERM(2, 0)
        segment("T0a", m0[:n0], [(p1, 0, T0P[0]), (p2, T0P[0], n0 - 0.5)], need={2: p1}, nrel=T0N[0])
        wait("x1")
        s1, f1, u = STATS(1), FIN(1, 0), 6 - n0
        segment("T0b", m0[n0:n1], [(s1, 0, max(0.2, u - T0P[1])), (f1, u - T0P[2], u - 0.01, s1)], need={u: s1 + f1},
                nrel=T0N[1])
        wait(*mnames(1), "w01")
        mods, f0, f1, pq, u = MODS(1), FIN(0, 1), FIN(1, 1), PERM(0, 1), 12 - n1
        fmin = max(3 / T0N[2], u - T0P[3])
        segment("T0c", m0[n1:] + m1[:n2],
                [(mods, 0, 0.2), (f0, fmin, u - 0.01, mods), (f1, u, u + 1, mods), (pq, 0, max(0.5, u - T0P[4]))],
                need={u: mods + f0 + pq, u + 2: f1}, nrel=T0N[2])
        wait("w11", "w21")
        p1, p2 = PERM(1, 1), PERM(2, 1)
        e1 = max(0.5, 4 - n2 - T0P[5])
        segment("T1", m1[n2:WA[1]], [(p1, 0, e1), (p2, e1, 8 - n2 - 1.5)], need={4 - n2: p1, 8 - n2: p2}, nrel=T0N[3])
        for k in range(2, NC):
            last = k == NC - 1
            late = [kk for kk in range(ND) if SAT[kk] == k]
            wait(*mnames(k), f"w0{k}", f"w1{k}", f"w2{k}", *[f"m0{kk}" for kk in late], *(["x2"] if k == X2AT + 1 else []))
            u = 12 - WA[k - 1]
            mods = MODS(k, TMG)
            fins = [FIN(t, k) for t in range(2)]
            perms = [PERM(m, k) for m in range(3)]
            mend = max(0.5, u - WP[0])
            fmin = (8 // TMG - 1) / TN + (mend - 0.5 if mend > 2 else 0)
            groups = [(mods[:1], 0, 1)] + ([(mods[1:], mend - 0.5 if mend > 2 else 0, mend)] if len(mods) > 1 else []) + [
                      (fins[0], max(fmin, u - WP[1]), max(fmin + 0.2, u - WP[2]), mods), (fins[1], max(fmin + 0.2, u - WP[2]), u + 1, mods),
                      (perms[0], 0, max(0.9, u - WP[3])), (perms[1], max(0.9, u - WP[3]), u + WP[4]), (perms[2], u + WP[4], u + WP[5])]
            for kk in late:
                ms, sc = MOD(0, kk, kk + 1, TMG), [shift_col_task(kk)]
                groups += [(ms, SBP[0], SBP[0] + 1), (sc, SBP[1], SBP[1] + 1, ms),
                           ([bias_task(kk, c) for c in range(3 * NC)], SBP[2], SBP[3], sc)]
            if k == X2AT + 1:
                s2 = STATS(2)
                groups.append((s2, *X2S))
            for kk in range(NC):
                if X2F[kk][0] == k:
                    assert kk <= k
                    groups.append((FIN(2, kk), *X2F[kk][1:], (s2 if k == X2AT + 1 else []) + (mods if kk == k else [])))
            segment(f"T{k}", WAVE(k - 1)[WA[k - 1]:] + (WAVE(k) if last else WAVE(k)[:WA[k]]), groups,
                    need={u: mods + fins[0] + perms[0], u + 2: fins[1], u + 4: perms[1], u + 8: perms[2]}, nrel=TN)
        wait("xr")

        def a_step(t, carry):
            base = jnp.minimum((t - 2) * (NPC // 2), NG) * (2 * G)
            att = [attn_task(True, base, NPC * G, g, AQ, masked=(g == 0)) for g in range(NPC)]
            l1 = LN1(t + 1, hn_v)
            segment("A", QKV(t), [(att, *AA), (l1, *AL), COPY(hn_v, hc_v, ACN[0], 48 - QT, 47, l1, 0, HK),
                                 COPY(hn_v, hc_v, ACN[1], 47 + 1 / AN, 48 + 1 / AN, l1, HK, D)], dl=ADL, nrel=AN, lns=ALS)
            return carry

        with scope("loopA"):
            jax.lax.fori_loop(2, NT - 1, a_step, 0)
        wait("wmr", "wo", "fw1", "fw3", "fw2a")
        q7, nq = QKV(NT - 1), AFP[0]
        mg, msc, l2 = MOD(2, mg=MG), MOD(3, mg=MG) + MOD(4, mg=MG), LN2(0, hn_v)
        done_rows = (NT - 3) * NPC * G
        att = [attn_task(True, done_rows, SA - done_rows, g, AFQ) for g in range((SA - done_rows) // G)]
        segment("AF", q7[:nq] + WO(0) + q7[nq:] + FFN(0, 0, C0),
                [(mg, 0, AFP[1]), (msc, AFP[1], AFP[2]), (l2, max(AFP[3], nq + 16), AFP[4], msc),
                 (MOD(5, mg=MG), AFP[5], AFP[6]), (att, AFP[7], AFP[8]), ([halo_task()], 1, 2)]
                + [COPY(hn_v, h2_v, 16, *AFC, l2)], need={nq: mg, 64: l2}, dl=AFDL, nrel=AFN, lns=AFL)
        wait("fw2b")

        nch = F // HK
        nf = (nch - C0) * 24

        def b_step(i, carry):
            att = [attn_task(False, jnp.minimum(i, NT - 3) * TM, TM, g, BQ) for g in range(NG)]
            l2 = LN2(i + 1, hn_v)
            ffn = FFN(i, C0, nch)
            cpy = [COPY(hn_v, h2_v, 16, nf + 16 - 8 + BCP[0], nf + 16 - 8 + BCP[1], l2)]
            assert BA[0] >= 16 + BW and BL[0] >= 16 + BW and min(BCP) >= 0
            segment("F", ffn[:BW] + WO(i + 1) + ffn[BW:] + FFN(i + 1, 0, C0), [(att, *BA), (l2, *BL)] + cpy,
                    need={nf + 16: l2}, dl=BDL, nrel=BN, lns=BLS)
            return carry

        with scope("B"):
            jax.lax.fori_loop(0, NT - 1, b_step, 0)
        for t in range(NT - 2):
            out_wait(t)
        segment("FL", FFN(NT - 1, C0, nch))
        with scope("fin"):
            for t in range(NT - 2, NT):
                out_wait(t)

    @jax.jit
    def fn(A_x, A_wqkv, A_wo, B_x, B_w1, B_w3, B_w2, c, w_mod):
        V = pltpu.VMEM
        scratch = [
            V((S, D), BF16), V((3, D, D), BF16), V((D // 2, 3 * D), U32), V((D, D), BF16),
            V((D, F), BF16), V((D, F), BF16), V((F, D), BF16), V((2 * NC, D, 128), BF16), V((D, 4 * D), BF16),
            V((8, D), F32), V((D, 128), F32), V((2, SA + TM, 128), F32), V((2, TM // 2, D), U32),
            V((NC, SA, 128), F32), V((NC, PAD + SA, 128), F32), V((NC, PAD + SA, 128), F32),
            V((NC, SB, 128), F32), V((NC, PAD + SB, 128), F32), V((NC, PAD + SB, 128), F32),
            V((S // 2, D), U32), V((NC, S, 128), F32), V((TM // 2, D), U32), V((NC, S, 128), BF16),
            V((TM // 2, D), U32), V((TM // 2, D), U32), V((NC, TM, 128), F32), V((128, 128), F32), V((8, 3 * D), F32), V((32, 128), F32), V((1, D), BF16),
            pltpu.SemaphoreType.DMA((5 * NC + 12,)), pltpu.SemaphoreType.DMA((NT,)), pltpu.SemaphoreType.REGULAR,
        ]
        out = pl.pallas_call(
            kernel,
            in_specs=[pl.BlockSpec(memory_space=pl.ANY)] * 8,
            out_specs=pl.BlockSpec(memory_space=pl.ANY),
            out_shape=jax.ShapeDtypeStruct((S, D), BF16),
            scratch_shapes=scratch,
            compiler_params=pltpu.CompilerParams(vmem_limit_bytes=124 * 1024 * 1024, disable_bounds_checks=True,
                                                 disable_semaphore_checks=True),
        )(A_x.reshape(S, D), A_wqkv, A_wo, B_w1, B_w3, B_w2, c, w_mod)
        return out.reshape(1, S, D)

    return fn


_impl = make_kernel()


@jax.jit
def pallas_adaLN_cond__sliding_local_dilated__glu_gated_swiglu__prompt_kernel(A_x, A_wqkv, A_wo, B_x, B_w1, B_w3, B_w2, c, w_mod):
    return _impl(A_x, A_wqkv, A_wo, B_x, B_w1, B_w3, B_w2, c, w_mod)
```

```python
import contextlib
import functools
import math

import jax
import jax.numpy as jnp
import jax.experimental.pallas as pl
import jax.experimental.pallas.tpu as pltpu

S, D, F = 2048, 1024, 3584
DH, WIN, DIL = 32, 8, 2
NC = D // 128
PAD = 16
EPS = 1e-5
SCALE = DH ** -0.5
EXP2_C = SCALE * math.log2(math.e)
MASKED = -1e9 / SCALE
F32, BF16, U32 = jnp.float32, jnp.bfloat16, jnp.uint32
TM = 256
NT = S // TM
G = 16
NG = TM // G
HK = D // 2
SA = 2 * TM
SB = S - SA


def _xor_network(xs):
    lane = jax.lax.broadcasted_iota(jnp.int32, xs[0].shape, 1)
    for b in range(3):
        m = ((lane >> (2 + b)) & 1) == 1
        xs = [jnp.where(m, xs[i ^ (1 << b)], xs[i]) for i in range(NC)]
    return xs


def _gather_fwd(z, j):
    lane = jax.lax.broadcasted_iota(jnp.int32, z.shape, 1)
    e, g, p = lane >> 5, (lane >> 3) & 3, lane & 7
    return jnp.take_along_axis(z, g * 32 + (p ^ j) * 4 + e, axis=1)


def _gather_inv(y, j):
    lane = jax.lax.broadcasted_iota(jnp.int32, y.shape, 1)
    g, q, e = lane >> 5, (lane >> 2) & 7, lane & 3
    return jnp.take_along_axis(y, e * 32 + g * 8 + (q ^ j), axis=1)


def _pack(x):
    return pltpu.bitcast(x.astype(BF16), U32)


def _or_all(vs):
    parts = [v[r:r + 8, c:c + 128] for v in vs for r in range(0, v.shape[0], 8) for c in range(0, v.shape[1], 128)]
    while len(parts) > 1:
        parts = [parts[i] | parts[i + 1] if i + 1 < len(parts) else parts[i] for i in range(0, len(parts), 2)]
    return parts[0]


def _gate(x, g):
    if g is None:
        return x
    xb = x if x.dtype == U32 else pltpu.bitcast(x, U32)
    y = xb | jnp.tile(g, (x.shape[0] // 8, x.shape[1] // 128))
    return y if x.dtype == U32 else pltpu.bitcast(y, x.dtype)


def _rows(start, n, mult):
    if isinstance(start, int):
        return pl.ds(start, n)
    return pl.ds(pl.multiple_of(start, mult), n)


def _stats(x):
    mu = jnp.mean(x, axis=-1, keepdims=True)
    xc = x - mu
    var = jnp.mean(xc * xc, axis=-1, keepdims=True)
    return mu, xc, jax.lax.rsqrt(var + EPS)


def make_kernel(
        NREL=2, DL=4, DSH=1, MG=1, TMG=2, PR=16,
        ND=2, SAT=(4, 5), SBP=(1.5, 3, 4.5, 8), W0=(4, 10, 3), WA=(9, 10, 8, 7, 7, 6, 6),
        T0N=(2, 4, 2, 2), T0P=(1.25, 0.75, 0.5, 0.25, 1.25, 0.5), TN=4, WP=(3, 1, 0.5, 1.5, 2, 5.5),
        X2AT=5, X2S=(2, 9),
        X2F=((6, 9.5, 10.5), (7, 2, 3), (7, 4, 5), (7, 7, 8), (7, 9, 10), (7, 12, 13), (7, 13, 14), (7, 14, 15)),
        NPC=6, QT=4, AN=4, AQ=(2, 2, 13, 4), AA=(1, 38), AL=(2, 38), ALS=(2, 4), ACN=(4, 2), ADL=4,
        C0=1, AFN=4, AFQ=(1, 1, 12, 3), AFP=(20, 15, 36, 38, 58, 60, 84, 0, 16), AFL=(0, 0), AFC=(66, 86), AFDL=5,
        BW=2, BN=4, BQ=(1, 1, 20, 5), BA=(18, 170), BL=(20, 149), BLS=(2, 4), BCP=(8, 28), BDL=6,
        scopes=False, only=None):

    def scope(name):
        return jax.named_scope(name) if scopes else contextlib.nullcontext()

    def kernel(x_hbm, wqkv_hbm, wo_hbm, w1_hbm, w3_hbm, w2_hbm, c_hbm, wm_hbm, out_hbm,
               x_v, wraw_v, wp_v, wo_v, w1_v, w3_v, w2_v, wmc_v, wmr_v,
               mod_v, scol_v, st_v, h1_v, qa_v, ka_v, va_v, qb_v, kb_v, vb_v, o_v, x1_v, h2_v, out_v,
               hc_v, hn_v, acc_v, sac_v, bias_v, z_v, c_v, sems, sem_out, bar):
        cp = pltpu.make_async_copy

        dmas = {}

        def add(name, src, dst):
            dmas[name] = cp(src, dst, sems.at[len(dmas)])

        def add_x(name, t0, n):
            add(name, x_hbm.at[pl.ds(t0 * TM, n * TM), :], x_v.at[pl.ds(t0 * TM, n * TM), :])

        add("c", c_hbm, c_v)
        add_x("x0", 0, 1)
        for k in range(NC):
            for m, kk in [(1, k)] + ([(0, k)] if k >= ND else []):
                add(f"m{m}{kk}", wm_hbm.at[:, pl.ds(m * D + kk * 128, 128)], wmc_v.at[m * NC + kk])
            for m in range(3):
                add(f"w{m}{k}", wqkv_hbm.at[pl.ds(k * 128, 128), pl.ds(m * D, D)], wraw_v.at[m, pl.ds(k * 128, 128), :])
            if k == 0:
                add_x("x1", 1, 1)
            for kk in range(ND):
                if SAT[kk] - 1 == k:
                    add(f"m0{kk}", wm_hbm.at[:, pl.ds(kk * 128, 128)], wmc_v.at[kk])
            if k == X2AT:
                add_x("x2", 2, 1)
        add_x("xr", 3, NT - 3)
        add("wmr", wm_hbm.at[:, pl.ds(2 * D, 4 * D)], wmr_v)
        add("wo", wo_hbm, wo_v)
        add("fw1", w1_hbm, w1_v)
        add("fw3", w3_hbm, w3_v)
        add("fw2a", w2_hbm.at[pl.ds(0, C0 * HK), :], w2_v.at[pl.ds(0, C0 * HK), :])
        add("fw2b", w2_hbm.at[pl.ds(C0 * HK, F - C0 * HK), :], w2_v.at[pl.ds(C0 * HK, F - C0 * HK), :])
        for d in dmas.values():
            d.start()
            pl.semaphore_signal(bar, 1)
            pl.semaphore_wait(bar, 1)
        for j in range(NC):
            ka_v[j, 0:PAD, :] = jnp.zeros((PAD, 128), F32)
        add("z", ka_v.at[0, pl.ds(0, 8), :], z_v.at[pl.ds(0, 8), :])
        dmas["z"].start()

        def wait(*names):
            with scope("w_" + names[0]):
                for n in names:
                    dmas[n].wait()

        def zero():
            return pltpu.bitcast(z_v[0:8, :], U32)

        cur = {"nrel": NREL, "lns": (0, 0)}

        def mod_task(m, j, mg=2):
            src = wmc_v.at[m * NC + j] if m < 2 else wmr_v.at[:, pl.ds((m - 2) * D + j * 128, 128)]
            acc = None
            for kb in range(D // 128):
                if kb % mg == 0:
                    rel = yield
                p = src[kb * 128:(kb + 1) * 128, :].astype(F32) * scol_v[kb * 128:(kb + 1) * 128, :]
                parts = [p[r:r + 8] for r in range(0, 128, 8)]
                a0, a1 = parts[0], parts[1]
                if kb % mg == 0:
                    a0, a1 = _gate(a0, rel), _gate(a1, rel)
                for r in range(2, 16, 2):
                    a0, a1 = a0 + parts[r], a1 + parts[r + 1]
                a0 = a0 + a1
                acc = a0 if acc is None else acc + a0
            r = jnp.sum(acc, axis=0, keepdims=True)
            if m in (1, 4):
                r = r + 1.0
            mod_v[m:m + 1, j * 128:(j + 1) * 128] = r
            return pltpu.bitcast(jnp.broadcast_to(r, (8, 128)), U32)

        def modulate(xn, ms, dst, g, c0, c1, shift=True):
            h = xn * mod_v[ms + 1:ms + 2, c0:c1]
            hb = _pack(h + mod_v[ms:ms + 1, c0:c1] if shift else h)
            dst[g * 8:(g + 1) * 8, c0:c1] = hb
            return _or_all([hb])

        def ln_tail(xc, rs, ms, dst, g):
            ns, skip = cur["lns"]
            if ns == 0:
                return modulate(xc * rs, ms, dst, g, 0, D)
            for _ in range(skip):
                yield
            rs = jnp.broadcast_to(rs, (G, 128))
            toks = []
            cw = D // ns
            for p in range(ns):
                rel = yield
                r = jnp.tile(_gate(rs, rel), (1, cw // 128))
                toks.append(modulate(xc[:, p * cw:(p + 1) * cw] * r, ms, dst, g, p * cw, (p + 1) * cw))
            return _or_all(toks)

        def ln1_task(t, g, dst):
            rel = yield
            xt = x_v.at[_rows(t * TM, TM, TM), :]
            _, xc, rs = _stats(_gate(xt[g * G:(g + 1) * G, :].astype(F32), rel))
            return (yield from ln_tail(xc, rs, 0, dst, g))

        def stats_task(t, g):
            rel = yield
            rows = slice(t * TM + g * G, t * TM + (g + 1) * G)
            mu, _, rs = _stats(_gate(x_v[rows, :].astype(F32), rel))
            rs = jnp.broadcast_to(rs, (G, 128))
            st_v[0, rows, :] = jnp.broadcast_to(mu, (G, 128))
            st_v[1, rows, :] = rs
            return _or_all([pltpu.bitcast(rs, U32)]) if t == 2 else None

        def fin_task(t, k, g0, ng):
            rel = yield
            toks = []
            for g in range(g0, g0 + ng):
                rows = slice(t * TM + g * G, t * TM + (g + 1) * G)
                x = _gate(x_v[rows, k * 128:(k + 1) * 128].astype(F32), rel)
                xn = (x - st_v[0, rows, :]) * st_v[1, rows, :]
                toks.append(modulate(xn, 0, h1_v.at[t] if t < 2 else hc_v, g, k * 128, (k + 1) * 128, t == 2 or k >= ND))
            return _or_all(toks) if t == 2 else None

        def ln2_task(t, g, dst):
            rel = yield
            xv = x1_v.at[:, _rows(t * TM, TM, TM), :]
            x = jnp.concatenate([_gate(xv[j, g * G:(g + 1) * G, :], rel) for j in range(NC)], axis=1)
            _, xc, rs = _stats(x)
            return (yield from ln_tail(xc, rs, 3, dst, g))

        def perm_select_task(m, r0, n):
            rel = yield
            xs = [_gate(pltpu.bitcast(wraw_v[m, r0:r0 + n, j * 128:(j + 1) * 128], U32), rel) for j in range(NC)]
            zs = _xor_network(xs)
            for j in range(NC):
                wp_v[r0 // 2:(r0 + n) // 2, m * D + j * 128:m * D + (j + 1) * 128] = zs[j]

        def perm_gather_task(m, j, r0, n):
            rel = yield
            sl = (slice(r0 // 2, (r0 + n) // 2), slice(m * D + j * 128, m * D + (j + 1) * 128))
            wp_v[sl] = _gather_fwd(_gate(wp_v[sl], rel), j)

        def shift_col_task(k):
            rel = yield
            row = _gate(jnp.broadcast_to(mod_v[0:1, k * 128:(k + 1) * 128], (128, 128)), rel)
            sac_v[...] = row.T

        def bias_task(k, c):
            rel = yield
            cs = slice(c * 128, (c + 1) * 128)
            w = pltpu.bitcast(_gate(wp_v[k * 64:(k + 1) * 64, cs], rel), BF16).astype(F32) * sac_v[...]
            parts = [w[r:r + 8] for r in range(0, 128, 8)]
            while len(parts) > 1:
                parts = [parts[i] + parts[i + 1] for i in range(0, len(parts), 2)]
            acc = parts[0] if k == 0 else bias_v[:, cs] + parts[0]
            if k == ND - 1:
                acc = jnp.broadcast_to(jnp.sum(acc, axis=0, keepdims=True), (8, 128))
            bias_v[:, cs] = acc
            return pltpu.bitcast(acc, U32)

        def copy_task(src, dst, r0, nr, c0, c1):
            rel = yield
            dst[r0:r0 + nr, c0:c1] = _gate(src[r0:r0 + nr, c0:c1], rel)

        def pad_task():
            yield
            for j in range(NC):
                va_v[j, 0:PAD, :] = jnp.broadcast_to(va_v[j, PAD:PAD + 1, :], (PAD, 128))

        def halo_task():
            yield
            for j in range(NC):
                kb_v[j, 0:PAD, :] = ka_v[j, SA:SA + PAD, :]
                vb_v[j, 0:PAD, :] = va_v[j, SA:SA + PAD, :]

        def attn_task(first, base, span, g, pace, masked=False):
            qkg, pvg, skip, smd = pace
            q_v, k_v, v_v = (qa_v, ka_v, va_v) if first else (qb_v, kb_v, vb_v)
            qv = q_v.at[:, _rows(base, span, 32), :]
            kv = k_v.at[:, _rows(base, span + PAD, 32), :]
            vv = v_v.at[:, _rows(base, span + PAD, 32), :]

            def shifted(ref, j, w):
                return ref[j, pl.ds(g * G + PAD - DIL * w, G), :]

            ls = [None] * WIN
            for j in range(NC):
                if j % qkg == 0:
                    rel = yield
                q = _gate(qv[j, g * G:(g + 1) * G, :], rel)
                for w in range(WIN):
                    p = q * shifted(kv, j, w)
                    ls[w] = p if j == 0 else ls[w] + p
            ls = [l + pltpu.roll(l, 64, 1) for l in ls]
            ls = [l + pltpu.roll(l, 32, 1) for l in ls]
            if masked:
                rows = base + g * G + jax.lax.broadcasted_iota(jnp.int32, (G, 128), 0)
                ls = [ls[0]] + [jnp.where(rows >= DIL * w, ls[w], MASKED) for w in range(1, WIN)]
            mx = ls[0]
            for w in range(1, WIN):
                mx = jnp.maximum(mx, ls[w])
            ps = [jnp.exp2((l - mx) * EXP2_C) for l in ls]
            den = ps[0]
            for w in range(1, WIN):
                den = den + ps[w]
            inv = 1.0 / den
            ps = [pw * inv for pw in ps]
            if smd:
                yield _or_all([pltpu.bitcast(ps[0], U32)]), smd
            for _ in range(skip - (1 if smd else 0)):
                yield
            zs = []
            for j in range(NC):
                if j % pvg == 0:
                    rel = yield
                    pg = [_gate(p, rel) for p in ps]
                acc = pg[0] * shifted(vv, j, 0)
                for w in range(1, WIN):
                    acc = acc + pg[w] * shifted(vv, j, w)
                zs.append(_gather_inv(_pack(acc), j))
            xs = _xor_network(zs)
            half = (base // 2 if isinstance(base, int) else jax.lax.shift_right_logical(base, 1)) + (0 if first else SA // 2)
            ov = o_v.at[_rows(half, span // 2, 16), :]
            for j in range(NC):
                ov[g * 8:(g + 1) * 8, j * 128:(j + 1) * 128] = xs[j]
            return _or_all(xs)

        def LN1(t, dst):
            return [ln1_task(t, g, dst) for g in range(NG)]

        def LN2(t, dst):
            return [ln2_task(t, g, dst) for g in range(NG)]

        def STATS(t):
            return [stats_task(t, g) for g in range(NG)]

        def FIN(t, k):
            return [fin_task(t, k, g0, 4) for g0 in range(0, NG, 4)]

        def MOD(m, j0=0, j1=NC, mg=2):
            return [mod_task(m, j, mg) for j in range(j0, j1)]

        def PERM(m, k):
            r0 = k * 128
            return ([perm_select_task(m, r, PR) for r in range(r0, r0 + 128, PR)]
                    + [perm_gather_task(m, j, r0, 128) for j in range(NC)])

        def COPY(src, dst, n, lo, hi, pre, c0=0, c1=D):
            nr = TM // 2 // n
            return ([copy_task(src, dst, r, nr, c0, c1) for r in range(0, TM // 2, nr)], lo, hi, pre)

        def run_now(tasks):
            for tk in tasks:
                try:
                    next(tk)
                    while True:
                        tk.send(None)
                except StopIteration:
                    pass

        def tie(a, tok):
            if tok is not None:
                top = a[0:8, 0:128] | (tok & zero())
                if a.shape[1] > 128:
                    top = jnp.concatenate([top, a[0:8, 128:]], axis=1)
                a = jnp.concatenate([top, a[8:]], axis=0)
            return pltpu.bitcast(a, BF16)


        def releases(res):
            return [pltpu.bitcast(res[r:r + 8, 0:128], U32) & zero() for r in range(0, TM, TM // cur["nrel"])]

        def wave_pass(k, t, nb, tok):
            m, j0 = nb // 2, (nb % 2) * 4
            dst = (qa_v, ka_v, va_v)[m]
            rows = slice(t * TM + (PAD if m else 0), (t + 1) * TM + (PAD if m else 0))
            w = pltpu.bitcast(wp_v[k * 64:(k + 1) * 64, nb * 512:(nb + 1) * 512], BF16)
            res = jnp.dot(tie(h1_v[t, :, k * 128:(k + 1) * 128], tok), w, preferred_element_type=F32)
            for jj in range(4):
                r = res[:, jj * 128:(jj + 1) * 128]
                if k == NC - 1 and ND:
                    c0 = nb * 512 + jj * 128
                    r = r + jnp.tile(bias_v[:, c0:c0 + 128], (TM // 8, 1))
                if k > 0:
                    r = dst[j0 + jj, rows, :] + r
                dst[j0 + jj, rows, :] = r
            return releases(res)

        def qkv_pass(t, m, j, hf, st, tok):
            w = pltpu.bitcast(wp_v[hf * HK // 2:(hf + 1) * HK // 2, m * D + j * 128:m * D + (j + 1) * 128], BF16)
            res = jnp.dot(tie(hc_v[:, hf * HK:(hf + 1) * HK], tok), w, preferred_element_type=F32)
            if hf == 0:
                st[m, j] = res
            else:
                res = st.pop((m, j)) + res
                off = PAD if m else 0
                dst = (qb_v, kb_v, vb_v)[m].at[:, _rows((t - 2) * TM, TM + off, TM), :]
                dst[j, off:off + TM, :] = res
            return releases(res)

        def wo_pass(t, j, hf, st, tok):
            h = tie(o_v[_rows(t * (TM // 2), TM // 2, TM // 2), hf * HK:(hf + 1) * HK], tok)
            res = jnp.dot(h, wo_v[hf * HK:(hf + 1) * HK, j * 128:(j + 1) * 128], preferred_element_type=F32)
            if hf == 0:
                st["a"] = res
            else:
                rows, cs = _rows(t * TM, TM, TM), slice(j * 128, (j + 1) * 128)
                res = x_v[rows, cs].astype(F32) + mod_v[2:3, cs] * (st.pop("a") + res)
                x1_v[j, rows, :] = res
            return releases(res)

        def out_copy(t, j):
            rows = _rows(t * TM, TM, TM)
            return cp(out_v.at[j, rows, :], out_hbm.at[rows, pl.ds(j * 128, 128)], sem_out.at[t])

        def out_wait(t):
            if only is not None and ("FL" if t == NT - 1 else "F") not in only:
                return
            rows = pl.ds(t * TM, TM)
            cp(out_hbm.at[rows, :], out_hbm.at[rows, :], sem_out.at[t]).wait()

        def WAVE(k):
            return [functools.partial(wave_pass, k, t, nb) for m in range(3) for t in range(2) for nb in (2 * m, 2 * m + 1)]

        def QKV(t):
            order = [(m, j, hf) for m in range(3) for j in range(NC) for hf in range(2)]
            order = order[:-2 * QT] + order[-2 * QT::2] + order[-2 * QT + 1::2]
            st = {}
            return [functools.partial(qkv_pass, t, m, j, hf, st) for m, j, hf in order]

        def WO(t):
            st = {}
            return [functools.partial(wo_pass, t, j, hf, st) for j in range(NC) for hf in range(2)]

        def FFN(t, c0, c1):
            st = {"acc": [None] * NC, "act": []}
            h_v = hn_v if c0 == 0 else h2_v

            def gate_up_pass(which, n, hf, tok):
                w = (w1_v, w3_v)[which][hf * HK:(hf + 1) * HK, n * 128:(n + 1) * 128]
                res = jnp.dot(tie(h_v[:, hf * HK:(hf + 1) * HK], tok), w, preferred_element_type=F32)
                if hf == 0:
                    st["a"] = res
                else:
                    res = st.pop("a") + res
                    if which == 0:
                        hg = 0.5 * res
                        st["g"] = hg + hg * jnp.tanh(hg)
                    else:
                        st["act"].append((st.pop("g") * res).astype(BF16))
                return releases(res)

            def down_pass(c, j, last, tok):
                if j == 0:
                    st["lhs"], st["act"] = jnp.concatenate(st["act"], axis=1), []
                w = w2_v[c * HK:(c + 1) * HK, j * 128:(j + 1) * 128]
                if tok is not None:
                    w = tie(pltpu.bitcast(w, U32), tok)
                res = jnp.dot(st["lhs"], w, preferred_element_type=F32)
                if c > 0:
                    res = (acc_v[j] if c == c0 else st["acc"][j]) + res
                st["acc"][j] = res
                if c == c1 - 1 and not last:
                    acc_v[j] = res
                if last:
                    rows = _rows(t * TM, TM, TM)
                    out_v[j, rows, :] = (x1_v[j, rows, :] + mod_v[5:6, j * 128:(j + 1) * 128] * res).astype(BF16)
                    out_copy(t, j).start()
                return releases(res)

            out = []
            nch = F // HK
            for c in range(c0, c1):
                for n in range(c * 4, c * 4 + 4):
                    out += [functools.partial(gate_up_pass, which, n, hf) for which in range(2) for hf in range(2)]
                out += [functools.partial(down_pass, c, j, c == nch - 1) for j in range(NC)]
            return out

        def segment(name, passes, groups=(), dl=DL, need=None, nrel=NREL, lns=(0, 0)):
            if only is not None and name not in only:
                return
            with scope(name):
                n = len(passes)
                cur["nrel"], cur["lns"] = nrel, lns
                active = []
                for tasks, lo, hi, *pre in groups:
                    for k, tk in enumerate(tasks):
                        active.append((int((lo + k * (hi - lo) / len(tasks)) * nrel), tk, pre[0] if pre else ()))
                        next(tk)
                deadlines = [[] for _ in range(n + dl + 8)]

                def due(p):
                    return p + DSH if p < n and passes[p].func.__name__ == "down_pass" else p

                def done(tasks):
                    return all(ent[1] is not tk for tk in tasks for ent in active)

                def feed(rel, slot, i):
                    for ent in list(active):
                        if ent[0] <= slot:
                            assert done(ent[2]), (name, i)
                            try:
                                mid = ent[1].send(rel)
                                if mid is not None:
                                    deadlines[due(i + mid[1])].append(mid[0])
                            except StopIteration as e:
                                if e.value is not None:
                                    deadlines[due(i + dl)].append(e.value)
                                active.remove(ent)

                feed(None, 0, 0)
                slot = 1
                for i, ps in enumerate(passes):
                    assert done((need or {}).get(i, ())), (name, i)
                    for rel in ps(_or_all(deadlines[i]) if deadlines[i] else None):
                        feed(rel, slot, i)
                        slot += 1
                while active:
                    feed(None, 1 << 30, n)

        def mnames(k):
            return [f"m1{k}"] + ([f"m0{k}"] if k >= ND else [])

        def MODS(k, mg=2):
            return MOD(1, k, k + 1, mg) + (MOD(0, k, k + 1, mg) if k >= ND else [])

        with scope("S0"):
            wait("c", "z")
            c = c_v[...].astype(F32)
            s = (c * jax.nn.sigmoid(c)).astype(BF16).astype(F32)
            eye = (jax.lax.broadcasted_iota(jnp.int32, (128, 128), 0)
                   == jax.lax.broadcasted_iota(jnp.int32, (128, 128), 1))
            ones = jnp.ones((128, 128), BF16)
            for j in range(NC):
                dg = jnp.where(eye, jnp.broadcast_to(s[:, j * 128:(j + 1) * 128], (128, 128)), 0.0).astype(BF16)
                scol_v[j * 128:(j + 1) * 128, :] = jnp.dot(dg, ones, preferred_element_type=F32)
            wait("x0")
            run_now(STATS(0))
            wait(*mnames(0))
            run_now(MODS(0) + FIN(0, 0))
            wait("w00")
            run_now(PERM(0, 0))
            wait("w10", "w20")

        m0 = [functools.partial(wave_pass, 0, t, nb) for t in range(2) for nb in range(6)]
        m1 = WAVE(1)
        n0, n1, n2 = W0
        p1, p2 = PERM(1, 0), PERM(2, 0)
        segment("T0a", m0[:n0], [(p1, 0, T0P[0]), (p2, T0P[0], n0 - 0.5)], need={2: p1}, nrel=T0N[0])
        wait("x1")
        s1, f1, u = STATS(1), FIN(1, 0), 6 - n0
        segment("T0b", m0[n0:n1], [(s1, 0, max(0.2, u - T0P[1])), (f1, u - T0P[2], u - 0.01, s1)], need={u: s1 + f1},
                nrel=T0N[1])
        wait(*mnames(1), "w01")
        mods, f0, f1, pq, u = MODS(1), FIN(0, 1), FIN(1, 1), PERM(0, 1), 12 - n1
        fmin = max(3 / T0N[2], u - T0P[3])
        segment("T0c", m0[n1:] + m1[:n2],
                [(mods, 0, 0.2), (f0, fmin, u - 0.01, mods), (f1, u, u + 1, mods), (pq, 0, max(0.5, u - T0P[4]))],
                need={u: mods + f0 + pq, u + 2: f1}, nrel=T0N[2])
        wait("w11", "w21")
        p1, p2 = PERM(1, 1), PERM(2, 1)
        e1 = max(0.5, 4 - n2 - T0P[5])
        segment("T1", m1[n2:WA[1]], [(p1, 0, e1), (p2, e1, 8 - n2 - 1.5)], need={4 - n2: p1, 8 - n2: p2}, nrel=T0N[3])
        for k in range(2, NC):
            last = k == NC - 1
            late = [kk for kk in range(ND) if SAT[kk] == k]
            wait(*mnames(k), f"w0{k}", f"w1{k}", f"w2{k}", *[f"m0{kk}" for kk in late], *(["x2"] if k == X2AT + 1 else []))
            u = 12 - WA[k - 1]
            mods = MODS(k, TMG)
            fins = [FIN(t, k) for t in range(2)]
            perms = [PERM(m, k) for m in range(3)]
            mend = max(0.5, u - WP[0])
            fmin = (8 // TMG - 1) / TN + (mend - 0.5 if mend > 2 else 0)
            groups = [(mods[:1], 0, 1)] + ([(mods[1:], mend - 0.5 if mend > 2 else 0, mend)] if len(mods) > 1 else []) + [
                      (fins[0], max(fmin, u - WP[1]), max(fmin + 0.2, u - WP[2]), mods), (fins[1], max(fmin + 0.2, u - WP[2]), u + 1, mods),
                      (perms[0], 0, max(0.9, u - WP[3])), (perms[1], max(0.9, u - WP[3]), u + WP[4]), (perms[2], u + WP[4], u + WP[5])]
            for kk in late:
                ms, sc = MOD(0, kk, kk + 1, TMG), [shift_col_task(kk)]
                assert not last and len(late) == 1
                groups += [(ms, SBP[0], SBP[0] + 1), (sc, SBP[1], SBP[1] + 1, ms),
                           ([bias_task(kk, c) for c in range(3 * NC)], SBP[2], SBP[3], sc)]
            if k == X2AT + 1:
                s2 = STATS(2)
                groups.append((s2, *X2S))
            for kk in range(NC):
                if X2F[kk][0] == k:
                    assert kk <= k
                    groups.append((FIN(2, kk), *X2F[kk][1:], (s2 if k == X2AT + 1 else []) + (mods if kk == k else [])))
            if last:
                groups.append(([pad_task()], u + 10, u + 11))
            segment(f"T{k}", WAVE(k - 1)[WA[k - 1]:] + (WAVE(k) if last else WAVE(k)[:WA[k]]), groups,
                    need={u: mods + fins[0] + perms[0], u + 2: fins[1], u + 4: perms[1], u + 8: perms[2]}, nrel=TN)
        wait("xr")

        def a_step(t, carry):
            base = jnp.minimum((t - 2) * (NPC // 2), NG) * (2 * G)
            att = [attn_task(True, base, NPC * G, g, AQ, masked=(g == 0)) for g in range(NPC)]
            l1 = LN1(t + 1, hn_v)
            segment("A", QKV(t), [(att, *AA), (l1, *AL), COPY(hn_v, hc_v, ACN[0], 48 - QT, 47, l1, 0, HK),
                                 COPY(hn_v, hc_v, ACN[1], 47 + 1 / AN, 48 + 1 / AN, l1, HK, D)], dl=ADL, nrel=AN, lns=ALS)
            return carry

        with scope("loopA"):
            jax.lax.fori_loop(2, NT - 1, a_step, 0)
        wait("wmr", "wo", "fw1", "fw3", "fw2a")
        q7, nq = QKV(NT - 1), AFP[0]
        mg, msc, l2 = MOD(2, mg=MG), MOD(3, mg=MG) + MOD(4, mg=MG), LN2(0, hn_v)
        done_rows = (NT - 3) * NPC * G
        att = [attn_task(True, done_rows, SA - done_rows, g, AFQ) for g in range((SA - done_rows) // G)]
        segment("AF", q7[:nq] + WO(0) + q7[nq:] + FFN(0, 0, C0),
                [(mg, 0, AFP[1]), (msc, AFP[1], AFP[2]), (l2, max(AFP[3], nq + 16), AFP[4], msc),
                 (MOD(5, mg=MG), AFP[5], AFP[6]), (att, AFP[7], AFP[8]), ([halo_task()], 1, 2)]
                + [COPY(hn_v, h2_v, 16, *AFC, l2)], need={nq: mg, 64: l2}, dl=AFDL, nrel=AFN, lns=AFL)
        wait("fw2b")

        nch = F // HK
        nf = (nch - C0) * 24

        def b_step(i, carry):
            att = [attn_task(False, jnp.minimum(i, NT - 3) * TM, TM, g, BQ) for g in range(NG)]
            l2 = LN2(i + 1, hn_v)
            ffn = FFN(i, C0, nch)
            cpy = [COPY(hn_v, h2_v, 16, nf + 16 - 8 + BCP[0], nf + 16 - 8 + BCP[1], l2)]
            assert BA[0] >= 16 + BW and BL[0] >= 16 + BW and min(BCP) >= 0
            segment("F", ffn[:BW] + WO(i + 1) + ffn[BW:] + FFN(i + 1, 0, C0), [(att, *BA), (l2, *BL)] + cpy,
                    need={nf + 16: l2}, dl=BDL, nrel=BN, lns=BLS)
            return carry

        with scope("B"):
            jax.lax.fori_loop(0, NT - 1, b_step, 0)
        for t in range(NT - 2):
            out_wait(t)
        segment("FL", FFN(NT - 1, C0, nch))
        with scope("fin"):
            for t in range(NT - 2, NT):
                out_wait(t)

    @jax.jit
    def fn(A_x, A_wqkv, A_wo, B_x, B_w1, B_w3, B_w2, c, w_mod):
        V = pltpu.VMEM
        scratch = [
            V((S, D), BF16), V((3, D, D), BF16), V((D // 2, 3 * D), U32), V((D, D), BF16),
            V((D, F), BF16), V((D, F), BF16), V((F, D), BF16), V((2 * NC, D, 128), BF16), V((D, 4 * D), BF16),
            V((8, D), F32), V((D, 128), F32), V((2, SA + TM, 128), F32), V((2, TM // 2, D), U32),
            V((NC, SA, 128), F32), V((NC, PAD + SA, 128), F32), V((NC, PAD + SA, 128), F32),
            V((NC, SB, 128), F32), V((NC, PAD + SB, 128), F32), V((NC, PAD + SB, 128), F32),
            V((S // 2, D), U32), V((NC, S, 128), F32), V((TM // 2, D), U32), V((NC, S, 128), BF16),
            V((TM // 2, D), U32), V((TM // 2, D), U32), V((NC, TM, 128), F32), V((128, 128), F32), V((8, 3 * D), F32), V((32, 128), F32), V((1, D), BF16),
            pltpu.SemaphoreType.DMA((5 * NC + 12,)), pltpu.SemaphoreType.DMA((NT,)), pltpu.SemaphoreType.REGULAR,
        ]
        out = pl.pallas_call(
            kernel,
            in_specs=[pl.BlockSpec(memory_space=pl.ANY)] * 8,
            out_specs=pl.BlockSpec(memory_space=pl.ANY),
            out_shape=jax.ShapeDtypeStruct((S, D), BF16),
            scratch_shapes=scratch,
            compiler_params=pltpu.CompilerParams(vmem_limit_bytes=124 * 1024 * 1024, disable_bounds_checks=True,
                                                 disable_semaphore_checks=True),
        )(A_x.reshape(S, D), A_wqkv, A_wo, B_w1, B_w3, B_w2, c, w_mod)
        return out.reshape(1, S, D)

    return fn


_impl = make_kernel()


@jax.jit
def pallas_adaLN_cond__sliding_local_dilated__glu_gated_swiglu__prompt_kernel(A_x, A_wqkv, A_wo, B_x, B_w1, B_w3, B_w2, c, w_mod):
    return _impl(A_x, A_wqkv, A_wo, B_x, B_w1, B_w3, B_w2, c, w_mod)
```
